```python
import jax
import jax.numpy as jnp

def _softmax(x, axis=-1):
    return jax.nn.softmax(x, axis=axis)

def _gelu(x):
    return jax.nn.gelu(x, approximate=True)

def _silu(x):
    return jax.nn.silu(x)

def _sigmoid(x):
    return jax.nn.sigmoid(x)

def _layernorm(x, axis=-1, eps=1e-05):
    m = jnp.mean(x, axis=axis, keepdims=True)
    v = jnp.var(x, axis=axis, keepdims=True)
    return (x - m) / jnp.sqrt(v + eps)

def _scatter_add(tgt, idx, src, axis=0):
    return tgt.at[idx].add(src)

def _segment_sum(src, seg, n):
    return jax.ops.segment_sum(src, seg, n)

class _Rng:

    def __init__(self, key):
        self._k = key

    def _next(self):
        self._k, sub = jax.random.split(self._k)
        return sub

    def normal(self, shape):
        return jax.random.normal(self._next(), shape, dtype=jnp.bfloat16)

    def randint(self, lo, hi, shape):
        return jax.random.randint(self._next(), shape, lo, hi, dtype=jnp.int32)

    def uniform(self, shape, lo=0.0, hi=1.0):
        return jax.random.uniform(self._next(), shape, jnp.bfloat16, lo, hi)

    def permutation(self, n):
        return jax.random.permutation(self._next(), n)
kernel_name = 'interleave_layers__memory_aug_recurrent_mem_tr__linear_kernel_hedgehog__prompt'

def setup_inputs():
    _rng = _Rng(jax.random.key(int.from_bytes(__import__("os").urandom(4), "little")))
    _w = lambda a: (lambda t: t.astype(jnp.bfloat16) if jnp.issubdtype(t.dtype, jnp.floating) else t)(jnp.asarray(a))

    def _A_setup():
        B, S, Dm = (1, 2048, 640)
        H, Dh = (32, 192)
        M, seg = (8, 32)
        seg = min(seg, S)
        S = S // seg * seg
        return {'x': _w((lambda *s: _rng.normal(s) * 0.05)(B, S, Dm)), 'mem0': _w((lambda *s: _rng.normal(s) * 0.05)(B, M, Dm)), 'Wq': _w((lambda *s: _rng.normal(s) * 0.05)(Dm, H, Dh) * Dm ** (-0.5)), 'Wk': _w((lambda *s: _rng.normal(s) * 0.05)(Dm, H, Dh) * Dm ** (-0.5)), 'Wv': _w((lambda *s: _rng.normal(s) * 0.05)(Dm, H, Dh) * Dm ** (-0.5)), 'Wo': _w((lambda *s: _rng.normal(s) * 0.05)(H, Dh, Dm) * (H * Dh) ** (-0.5)), 'seg_len': seg}
    _A_in = _A_setup()

    def _B_setup():
        B, S, D, H = (1, 2048, 640, 32)
        Dh = D // H
        return {'x': _w((lambda *s: _rng.normal(s) * 0.05)(B, S, D)), 'wqkv': _w((lambda *s: _rng.normal(s) * 0.05)(D, 3 * D)), 'w_phi': _w((lambda *s: _rng.normal(s) * 0.05)(H, Dh, Dh) * Dh ** (-0.5)), 'wo': _w((lambda *s: _rng.normal(s) * 0.05)(D, D))}
    _B_in = _B_setup()
    return {'A_x': _A_in['x'], 'A_mem0': _A_in['mem0'], 'A_Wq': _A_in['Wq'], 'A_Wk': _A_in['Wk'], 'A_Wv': _A_in['Wv'], 'A_Wo': _A_in['Wo'], 'A_seg_len': _A_in['seg_len'], 'B_x': _B_in['x'], 'B_wqkv': _B_in['wqkv'], 'B_w_phi': _B_in['w_phi'], 'B_wo': _B_in['wo']}

def reference(A_x, A_mem0, A_Wq, A_Wk, A_Wv, A_Wo, A_seg_len, B_x, B_wqkv, B_w_phi, B_wo):

    def _A_ref(x, mem0, Wq, Wk, Wv, Wo, seg_len):
        B, S, Dm = x.shape
        H, Dh = (Wq.shape[1], Wq.shape[2])
        M = mem0.shape[1]
        scale = Dh ** (-0.5)
        n_seg = S // seg_len
        L = M + seg_len
        idx = jnp.arange(L)
        mask = (idx[:, None] < M) | (idx[:, None] >= idx[None, :])
        mem = mem0
        outs = []
        for s in range(n_seg):
            xs = x[:, s * seg_len:(s + 1) * seg_len, :].copy()
            h = jnp.concatenate([mem, xs], axis=1)
            q = jnp.einsum('btd,dhe->bhte', h, Wq)
            k = jnp.einsum('btd,dhe->bhte', h, Wk)
            v = jnp.einsum('btd,dhe->bhte', h, Wv)
            scores = jnp.einsum('bhqe,bhke->bhqk', q, k) * scale
            scores = jnp.where(mask[None, None], scores, -1000000000.0)
            p = _softmax(scores, axis=-1)
            o = jnp.einsum('bhqk,bhke->bhqe', p, v)
            o = jnp.einsum('bhte,hed->btd', o, Wo)
            mem = o[:, :M, :].copy()
            outs.append(o[:, M:, :])
        return jnp.concatenate(outs, axis=1)

    def _B_ref(x, wqkv, w_phi, wo):
        B, S, D = x.shape
        H = 32
        Dh = D // H
        qkv = (lambda x, *d: x.transpose(*d))((x @ wqkv).reshape(B, S, 3, H, Dh), 2, 0, 3, 1, 4)
        q, k, v = (qkv[0], qkv[1], qkv[2])
        pq = jnp.einsum('bhsd,hdf->bhsf', q, w_phi)
        pk = jnp.einsum('bhsd,hdf->bhsf', k, w_phi)
        phi_q = jnp.concatenate([_softmax(pq, axis=-1), _softmax(-pq, axis=-1)], axis=-1)
        phi_k = jnp.concatenate([_softmax(pk, axis=-1), _softmax(-pk, axis=-1)], axis=-1)
        kv = jnp.einsum('bhsf,bhsd->bhfd', phi_k, v)
        z = jnp.einsum('bhsf->bhf', phi_k)
        num = jnp.einsum('bhqf,bhfd->bhqd', phi_q, kv)
        den = jnp.einsum('bhqf,bhf->bhq', phi_q, z)[..., None] + 1e-06
        o = num / den
        return (lambda x, *d: x.transpose(*d))(o, 0, 2, 1, 3).reshape(B, S, D) @ wo
    x = A_x
    x = x + _A_ref(_layernorm(x, axis=-1), A_mem0, A_Wq, A_Wk, A_Wv, A_Wo, A_seg_len)
    x = x + _B_ref(_layernorm(x, axis=-1), B_wqkv, B_w_phi, B_wo)
    x = x + _A_ref(_layernorm(x, axis=-1), A_mem0, A_Wq, A_Wk, A_Wv, A_Wo, A_seg_len)
    x = x + _B_ref(_layernorm(x, axis=-1), B_wqkv, B_w_phi, B_wo)
    return x
```

```python
import functools

import jax
import jax.numpy as jnp
from jax import lax
import jax.experimental.pallas as pl
import jax.experimental.pallas.tpu as pltpu

F32 = jnp.float32
BF16 = jnp.bfloat16
U32 = jnp.uint32
LOG2E = 1.4426950408889634
NT = (((1,), (1,)), ((), ()))
TN = (((0,), (0,)), ((), ()))
LANES = 128

NSLOT = 3
TB = 256
B_UNROLL = 2


def _layernorm(x):
    m = jnp.mean(x, axis=-1, keepdims=True)
    xc = x - m
    v = jnp.mean(xc * xc, axis=-1, keepdims=True)
    return xc * lax.rsqrt(v + 1e-5)


def _pack(w):
    return pltpu.bitcast(w, U32)


def _unpack(w):
    return pltpu.bitcast(w, BF16)


def _a_schedule(npair):
    s = [("k", 0), ("q", 0), ("v", 0)]
    for j in range(npair - 1):
        s += [("s", j), ("k", j + 1), ("q", j + 1), ("v", j + 1), ("p", j)]
    last = npair - 1
    s += [("s", last), ("o", 0), ("o", 1), ("o", 2), ("p", last)]
    s += [("o", i) for i in range(3, npair)]
    return s


def _kernel(
    x_hbm, mem_ref, wq_hbm, wk_hbm, wv_hbm, wo_hbm, bw_hbm, wphi_ref, bwo_hbm,
    out_hbm,
    xb_ref, xres_ref, xna_ref, xnb_ref, memf_ref,
    stage_ref, wqkv_ref, wo_ref,
    bw_ref, bwo_stage_ref, bwt_ref, bwo_ref,
    kv_ref, z_ref,
    wsem, sem, osem,
    *, seg, dh, hb,
):
    S, D = xres_ref.shape
    M = mem_ref.shape[0]
    L = M + seg
    nseg = S // seg
    PW = 2 * dh
    npair = wo_ref.shape[0]
    fb = D // hb
    GR = 2 * fb
    HR = D // 2
    NG = HR // GR
    NTILE = 2 * HR // LANES
    spans = []
    for i in range(NTILE):
        lo = (i * LANES) // (2 * GR)
        hi = ((i + 1) * LANES - 1) // (2 * GR) + 1
        spans.append((lo * GR, hi * GR))
    offs = [0]
    for lo, hi in spans:
        offs.append(offs[-1] + hi - lo)

    def wcopy(j, t):
        src = (wq_hbm, wk_hbm, wv_hbm, wo_hbm)[t]
        return pltpu.make_async_copy(
            src.at[pl.ds(pl.multiple_of(j * PW, PW), PW), :],
            stage_ref.at[j % NSLOT, t],
            wsem.at[j % NSLOT, t],
        )

    x_copy = pltpu.make_async_copy(x_hbm, xb_ref, sem.at[0])
    bw_copy = pltpu.make_async_copy(bw_hbm, bw_ref, sem.at[1])
    bwo_copy = pltpu.make_async_copy(bwo_hbm, bwo_stage_ref, sem.at[2])
    bw_copy.start()
    bwo_copy.start()
    x_copy.start()
    for j in range(NSLOT):
        for t in range(4):
            wcopy(j, t).start()

    wcat = None
    hh = lax.broadcasted_iota(jnp.int32, (hb, D), 0)
    cc = lax.broadcasted_iota(jnp.int32, (hb, D), 1)
    for d in range(fb):
        sel = jnp.where(cc == hh * fb + d, 1.0, 0.0).astype(BF16)
        t = jnp.dot(wphi_ref[d], sel, preferred_element_type=F32)
        wcat = t if wcat is None else wcat + t
    rr = lax.broadcasted_iota(jnp.int32, (GR, fb), 0)
    ff = lax.broadcasted_iota(jnp.int32, (GR, fb), 1)
    rep = jnp.where((rr >> 1) == ff, 1.0, 0.0).astype(BF16)
    wrep = jnp.dot(rep, wcat.astype(BF16), preferred_element_type=F32)
    rr = lax.broadcasted_iota(jnp.int32, (GR, D), 0)
    cc = lax.broadcasted_iota(jnp.int32, (GR, D), 1)
    cc = cc - (rr & 1) * fb
    blocks = [
        jnp.where((cc >= g * GR) & (cc < g * GR + fb), wrep, 0.0)
        for g in range(hb // 2)
    ]
    pmat = jnp.concatenate(blocks, axis=0).astype(BF16)
    bw_copy.wait()
    for t in range(2):
        w = lax.dot_general(
            pmat, bw_ref[:, t * D:(t + 1) * D], NT, preferred_element_type=F32
        )
        bwt_ref[t] = _pack((w * LOG2E).astype(BF16))
    bwt_ref[2] = _pack(bw_ref[:, 2 * D:3 * D].T)
    bwo_copy.wait()
    bwo_ref[...] = _pack(bwo_stage_ref[...])

    x_copy.wait()

    def widen(i, c):
        r = pl.ds(pl.multiple_of(i * 256, 256), 256)
        xres_ref[r, :] = xb_ref[r, :].astype(F32)
        return c

    lax.fori_loop(0, S // 256, widen, 0)

    def load_pair(j, c):
        slot = j % NSLOT
        for t in range(3):
            wcopy(j, t).wait()
            wqkv_ref[j, :, t * PW:(t + 1) * PW] = _pack(stage_ref[slot, t].T)
        wcopy(j, 3).wait()
        wo_ref[j] = _pack(stage_ref[slot, 3])

        @pl.when(j + NSLOT < npair)
        def _():
            for t in range(4):
                wcopy(j + NSLOT, t).start()

        return c

    lax.fori_loop(0, npair, load_pair, 0)

    def a_step(s, c):
        rows = pl.ds(pl.multiple_of(s * seg, seg), seg)
        row = lax.broadcasted_iota(jnp.int32, (L, LANES), 0)
        lane = lax.broadcasted_iota(jnp.int32, (L, LANES), 1)
        is_a = lane < L
        col = jnp.where(is_a, lane, lane - L)
        inside = col < L
        vis = ((row < M) | (row >= col)) & inside
        vis_a = vis & is_a
        vis_b = vis & jnp.logical_not(is_a)
        fill_a = jnp.where(is_a, -1e9 * LOG2E, -jnp.inf)
        fill_b = jnp.where(inside & jnp.logical_not(is_a), -1e9 * LOG2E, -jnp.inf)
        low = lane < dh - LANES
        scale = dh ** -0.5 * LOG2E

        def proj(j, t):
            h = jnp.concatenate([memf_ref[...], xna_ref[rows, :]], axis=0)
            w = _unpack(wqkv_ref[j, :, t * PW:(t + 1) * PW])
            return jnp.dot(h, w, preferred_element_type=F32)

        def blockdiag(a):
            zero = jnp.zeros((L, LANES), F32)
            mid = a[:, LANES:2 * LANES]
            top = jnp.concatenate(
                [a[:, :LANES], jnp.where(low, mid, 0.0), zero], axis=1)
            bot = jnp.concatenate(
                [zero, jnp.where(low, 0.0, mid), a[:, 2 * LANES:]], axis=1)
            pad = jnp.zeros((LANES - 2 * L, PW), F32)
            return jnp.concatenate([top, bot, pad], axis=0).astype(BF16)

        def probs(q, k):
            sc = lax.dot_general(q, blockdiag(k), NT, preferred_element_type=F32)
            sc = sc * scale
            sa = jnp.where(vis_a, sc, fill_a)
            sb = jnp.where(vis_b, sc, fill_b)
            ma = jnp.max(sa, axis=1, keepdims=True)
            mb = jnp.max(sb, axis=1, keepdims=True)
            e = jnp.exp2(jnp.where(is_a, sa - ma, sb - mb))
            la = jnp.sum(jnp.where(is_a, e, 0.0), axis=1, keepdims=True)
            lb = jnp.sum(jnp.where(is_a, 0.0, e), axis=1, keepdims=True)
            return e * (1.0 / jnp.where(is_a, la, lb))

        prv = pl.ds(pl.multiple_of(jnp.maximum(s - 1, 0) * seg, seg), seg)
        nxt = pl.ds(pl.multiple_of(jnp.minimum(s + 1, nseg - 1) * seg, seg), seg)
        xnb_ref[prv, :] = _layernorm(xres_ref[prv, :]).astype(BF16)
        xn_next = _layernorm(xres_ref[nxt, :])

        q, k, v, p, o = {}, {}, {}, {}, {}
        acc = None
        for op, j in _a_schedule(npair):
            if op == "q":
                q[j] = proj(j, 0)
            elif op == "k":
                k[j] = proj(j, 1)
            elif op == "v":
                v[j] = proj(j, 2)
            elif op == "s":
                p[j] = probs(q.pop(j), k.pop(j))
            elif op == "p":
                o[j] = jnp.dot(
                    p.pop(j), blockdiag(v.pop(j)), preferred_element_type=F32)
                if j == npair - 1:
                    xna_ref[nxt, :] = xn_next
            else:
                y = jnp.dot(
                    o.pop(j), _unpack(wo_ref[j]), preferred_element_type=F32)
                acc = y if acc is None else acc + y
        memf_ref[...] = acc[:M]
        xres_ref[rows, :] = xres_ref[rows, :] + acc[M:]
        return c

    def layer_a():
        memf_ref[...] = mem_ref[...].astype(F32)
        xna_ref[0:seg, :] = _layernorm(xres_ref[0:seg, :])
        lax.fori_loop(0, nseg, a_step, 0)
        xnb_ref[S - seg:S, :] = _layernorm(xres_ref[S - seg:S, :]).astype(BF16)

    def b_proj(t, half, rows):
        w = _unpack(bwt_ref[t, half * (HR // 2):(half + 1) * (HR // 2), :])
        return lax.dot_general(
            w, xnb_ref[rows, :], NT, preferred_element_type=F32)

    def fold(vals, op):
        r = functools.reduce(op, vals)
        r = op(r, pltpu.roll(r, 4, 0))
        return op(r, pltpu.roll(r, 2, 0))

    def exps(a, g):
        slabs = [a[g * GR + 8 * i:g * GR + 8 * i + 8] for i in range(GR // 8)]
        mx = fold(slabs, jnp.maximum)
        mn = fold(slabs, jnp.minimum)
        ep = [jnp.exp2(u - mx) for u in slabs]
        en = [jnp.exp2(mn - u) for u in slabs]
        return ep, en, 1.0 / fold(ep, jnp.add), 1.0 / fold(en, jnp.add)

    def unit_rows(i, u):
        start = (i * B_UNROLL + u) * TB
        return pl.ds(pl.multiple_of(start, TB), TB)

    units = [(u, half) for u in range(B_UNROLL) for half in range(2)]

    def b_pass1(i, c):
        def features(u, half):
            a = b_proj(1, half, unit_rows(i, u))
            phi = []
            for g in range(NG):
                ep, en, ip, im = exps(a, g)
                phi += [e * ip for e in ep] + [e * im for e in en]
            phi = jnp.concatenate(phi, axis=0)
            zsum = phi[:, :LANES]
            for n in range(1, TB // LANES):
                zsum = zsum + phi[:, n * LANES:(n + 1) * LANES]
            z_ref[half] += zsum
            return phi.astype(BF16)

        def outer(half, vt, phi):
            for n, (lo, hi) in enumerate(spans):
                kv_ref[half, offs[n]:offs[n + 1], :] += lax.dot_general(
                    vt[lo:hi], phi[n * LANES:(n + 1) * LANES], NT,
                    preferred_element_type=F32)

        phi = features(*units[0])
        for n, (u, half) in enumerate(units):
            vt = b_proj(2, half, unit_rows(i, u))
            phi_next = features(*units[n + 1]) if n + 1 < len(units) else None
            outer(half, vt, phi)
            phi = phi_next
        return c

    def b_mid():
        for half in range(2):
            zs = jnp.sum(z_ref[half], axis=1, keepdims=True)
            z_ref[half] = jnp.broadcast_to(zs, (2 * HR, LANES))
            for n, (lo, hi) in enumerate(spans):
                r = lax.broadcasted_iota(jnp.int32, (hi - lo, LANES), 0) + lo
                f = lax.broadcasted_iota(jnp.int32, (hi - lo, LANES), 1) + n * LANES
                first = (f & 1) * fb
                for g in range(lo // GR, hi // GR):
                    first = jnp.where(f >= g * 2 * GR, g * GR + (f & 1) * fb, first)
                keep = (r >= first) & (r < first + fb)
                blk = slice(offs[n], offs[n + 1])
                kv_ref[half, blk, :] = jnp.where(keep, kv_ref[half, blk, :], 0.0)

    def out_copy(i):
        r = pl.ds(pl.multiple_of(i * (B_UNROLL * TB), B_UNROLL * TB), B_UNROLL * TB)
        return pltpu.make_async_copy(xb_ref.at[r, :], out_hbm.at[r, :], osem.at[i])

    def b_pass2(layer, i, c):
        def features(u, half):
            a = b_proj(0, half, unit_rows(i, u))
            phi = []
            for g in range(NG):
                ep, en, ip, im = exps(a, g)

                def zdot(es, base):
                    terms = []
                    for n, e in enumerate(es):
                        z = z_ref[half, base + 8 * n:base + 8 * n + 8, :]
                        terms.append(e * jnp.concatenate([z] * (TB // LANES), axis=1))
                    return functools.reduce(jnp.add, terms)

                den = zdot(ep, 2 * GR * g) * ip + zdot(en, 2 * GR * g + GR) * im
                inv = 1.0 / (fold([den], jnp.add) + 1e-6)
                ip, im = ip * inv, im * inv
                phi += [e * ip for e in ep] + [e * im for e in en]
            return jnp.concatenate(phi, axis=0).astype(BF16)

        def mix(half, phi):
            parts = [None] * NG
            for n, (lo, hi) in enumerate(spans):
                y = jnp.dot(
                    kv_ref[half, offs[n]:offs[n + 1], :],
                    phi[n * LANES:(n + 1) * LANES], preferred_element_type=F32)
                for g in range(lo // GR, hi // GR):
                    piece = y[g * GR - lo:(g + 1) * GR - lo]
                    parts[g] = piece if parts[g] is None else parts[g] + piece
            return jnp.concatenate(parts, axis=0)

        def finish(u, halves):
            rows = unit_rows(i, u)
            ot = jnp.concatenate(halves, axis=0).astype(BF16)
            y = lax.dot_general(
                ot, _unpack(bwo_ref[...]), TN, preferred_element_type=F32)
            y = xres_ref[rows, :] + y
            xres_ref[rows, :] = y
            xb_ref[rows, :] = y.astype(BF16)

        phis = [features(*units[0]), features(*units[1])]
        halves, pending = [], None
        for n, (u, half) in enumerate(units):
            if n + 2 < len(units):
                phis.append(features(*units[n + 2]))
            halves.append(mix(half, phis.pop(0)))
            if pending is not None:
                finish(*pending)
                pending = None
            if half == 1:
                pending, halves = (u, halves), []
        finish(*pending)

        @pl.when(layer == 1)
        def _():
            out_copy(i).start()

        return c

    nblk = S // (B_UNROLL * TB)

    def layer(n, c):
        layer_a()
        kv_ref[...] = jnp.zeros(kv_ref.shape, F32)
        z_ref[...] = jnp.zeros(z_ref.shape, F32)
        lax.fori_loop(0, nblk, b_pass1, 0)
        b_mid()
        lax.fori_loop(0, nblk, functools.partial(b_pass2, n), 0)
        return c

    lax.fori_loop(0, 2, layer, 0)
    for i in range(nblk):
        out_copy(i).wait()


@functools.partial(jax.jit, static_argnames=("A_seg_len",))
def pallas_interleave_layers__memory_aug_recurrent_mem_tr__linear_kernel_hedgehog__prompt_kernel(
    A_x: jax.Array,
    A_mem0: jax.Array,
    A_Wq: jax.Array,
    A_Wk: jax.Array,
    A_Wv: jax.Array,
    A_Wo: jax.Array,
    A_seg_len: int,
    B_x: jax.Array,
    B_wqkv: jax.Array,
    B_w_phi: jax.Array,
    B_wo: jax.Array,
):
    del B_x
    _, S, D = A_x.shape
    M = A_mem0.shape[1]
    _, H, dh = A_Wq.shape
    hb = B_w_phi.shape[0]
    seg = int(A_seg_len)
    npair, PW = H // 2, 2 * dh
    assert A_x.shape[0] == 1 and PW == 3 * LANES and 2 * (M + seg) <= LANES
    assert D == 5 * LANES and hb == 32 and S % (B_UNROLL * TB) == 0

    def rows_first(w):
        return jnp.transpose(w, (1, 2, 0)).reshape(H * dh, D)

    hbm = pl.BlockSpec(memory_space=pl.ANY)
    vmem = pl.BlockSpec(memory_space=pltpu.VMEM)
    out = pl.pallas_call(
        functools.partial(_kernel, seg=seg, dh=dh, hb=hb),
        out_shape=jax.ShapeDtypeStruct((S, D), BF16),
        in_specs=[hbm, vmem, hbm, hbm, hbm, hbm, hbm, vmem, hbm],
        out_specs=hbm,
        scratch_shapes=[
            pltpu.VMEM((S, D), BF16),
            pltpu.VMEM((S, D), F32),
            pltpu.VMEM((S, D), F32),
            pltpu.VMEM((S, D), BF16),
            pltpu.VMEM((M, D), F32),
            pltpu.VMEM((NSLOT, 4, PW, D), BF16),
            pltpu.VMEM((npair, D // 2, 3 * PW), U32),
            pltpu.VMEM((npair, PW // 2, D), U32),
            pltpu.VMEM((D, 3 * D), BF16),
            pltpu.VMEM((D, D), BF16),
            pltpu.VMEM((3, D // 2, D), U32),
            pltpu.VMEM((D // 2, D), U32),
            pltpu.VMEM((2, 480, LANES), F32),
            pltpu.VMEM((2, D, LANES), F32),
            pltpu.SemaphoreType.DMA((NSLOT, 4)),
            pltpu.SemaphoreType.DMA((3,)),
            pltpu.SemaphoreType.DMA((S // (B_UNROLL * TB),)),
        ],
        compiler_params=pltpu.CompilerParams(vmem_limit_bytes=100 * 1024 * 1024),
    )(
        A_x.reshape(S, D),
        A_mem0.reshape(M, D),
        rows_first(A_Wq),
        rows_first(A_Wk),
        rows_first(A_Wv),
        A_Wo.reshape(H * dh, D),
        B_wqkv,
        jnp.transpose(B_w_phi, (1, 2, 0)),
        B_wo,
    )
    return out.reshape(1, S, D)
```

```python
import functools

import jax
import jax.numpy as jnp
from jax import lax
import jax.experimental.pallas as pl
import jax.experimental.pallas.tpu as pltpu

F32 = jnp.float32
BF16 = jnp.bfloat16
U32 = jnp.uint32
LOG2E = 1.4426950408889634
NT = (((1,), (1,)), ((), ()))
TN = (((0,), (0,)), ((), ()))
LANES = 128

NSLOT = 3
TB = 256
B_UNROLL = 2
NPRE = 48


def _layernorm(x):
    m = jnp.mean(x, axis=-1, keepdims=True)
    xc = x - m
    v = jnp.mean(xc * xc, axis=-1, keepdims=True)
    return xc * lax.rsqrt(v + 1e-5)


def _pack(w):
    return pltpu.bitcast(w, U32)


def _unpack(w):
    return pltpu.bitcast(w, BF16)


def _a_schedule(npair, short):
    s = [("k", 0), ("q", 0), ("v", 0)]
    n = 0
    for j in range(npair - 1):
        s += [("s", j), ("k", j + 1), ("q", j + 1)]
        if short and j > 0 and j % 4 != 0:
            s.append(("o", n))
            n += 1
        s += [("v", j + 1), ("p", j)]
    last = npair - 1
    s += [("s", last), ("o", n), ("o", n + 1), ("o", n + 2), ("p", last)]
    s += [("o", i) for i in range(n + 3, npair)]
    return s


def _kernel(
    x_hbm, x4_hbm, mem_ref, wq_hbm, wk_hbm, wv_hbm, wo_hbm, bw_hbm, wphi_ref, bwo_hbm,
    out_hbm,
    xb_ref, xres_ref, xna_ref, xnb_ref, memf_ref,
    stage_ref, wqkv_ref, wo_ref,
    bw_ref, bwo_stage_ref, bwt_ref, bwo_ref,
    kv_ref, z_ref, xsel_ref, xseln_ref, pre_ref, wrep_ref,
    wsem, sem, osem,
    *, seg, dh, hb,
):
    S, D = xres_ref.shape
    M = mem_ref.shape[0]
    L = M + seg
    nseg = S // seg
    PW = 2 * dh
    npair = wo_ref.shape[0]
    fb = D // hb
    GR = 2 * fb
    HR = D // 2
    NG = HR // GR
    NTILE = 2 * HR // LANES
    spans = []
    for i in range(NTILE):
        lo = (i * LANES) // (2 * GR)
        hi = ((i + 1) * LANES - 1) // (2 * GR) + 1
        spans.append((lo * GR, hi * GR))
    offs = [0]
    for lo, hi in spans:
        offs.append(offs[-1] + hi - lo)

    XP = S // npair

    def wcopy(j, t):
        if t == 4:
            r = pl.ds(pl.multiple_of(j * XP, XP), XP)
            return pltpu.make_async_copy(
                x_hbm.at[r, :], xb_ref.at[r, :], wsem.at[j % NSLOT, t])
        src = (wq_hbm, wk_hbm, wv_hbm, wo_hbm)[t]
        return pltpu.make_async_copy(
            src.at[pl.ds(pl.multiple_of(j * PW, PW), PW), :],
            stage_ref.at[j % NSLOT, t],
            wsem.at[j % NSLOT, t],
        )

    def start_pair(j):
        for t in range(5):
            wcopy(j, t).start()

    xsel_copy = pltpu.make_async_copy(
        x4_hbm.at[0:NPRE, seg // 8 - 1], xsel_ref, sem.at[0])
    bw_copy = pltpu.make_async_copy(bw_hbm, bw_ref, sem.at[1])
    bwo_copy = pltpu.make_async_copy(bwo_hbm, bwo_stage_ref, sem.at[2])
    xsel_copy.start()
    start_pair(0)

    wcat = None
    hh = lax.broadcasted_iota(jnp.int32, (hb, D), 0)
    cc = lax.broadcasted_iota(jnp.int32, (hb, D), 1)
    for d in range(fb):
        sel = jnp.where(cc == hh * fb + d, 1.0, 0.0).astype(BF16)
        t = jnp.dot(wphi_ref[d], sel, preferred_element_type=F32)
        wcat = t if wcat is None else wcat + t
    rr = lax.broadcasted_iota(jnp.int32, (GR, fb), 0)
    ff = lax.broadcasted_iota(jnp.int32, (GR, fb), 1)
    twice = jnp.where((rr >> 1) == ff, 1.0, 0.0).astype(BF16)
    wrep_ref[...] = jnp.dot(twice, wcat.astype(BF16), preferred_element_type=F32)

    xsel_copy.wait()
    start_pair(1)
    xsel = xsel_ref[...].astype(F32).reshape(NPRE * 8, D)
    xseln_ref[...] = _pack(_layernorm(xsel).astype(BF16))
    for j in range(2, NSLOT):
        start_pair(j)

    def load_pair(j, c):
        slot = j % NSLOT
        for t in range(5):
            wcopy(j, t).wait()
        for t in range(3):
            cols = slice(t * PW, (t + 1) * PW)
            pre_ref[j, :, cols] = lax.dot_general(
                _unpack(xseln_ref[...]), stage_ref[slot, t], NT,
                preferred_element_type=F32)
            wqkv_ref[j, :, cols] = _pack(
                stage_ref[slot, t].astype(F32).T.astype(BF16))
        wo_ref[j] = _pack(stage_ref[slot, 3])
        r = pl.ds(pl.multiple_of(j * XP, XP), XP)
        xres_ref[r, :] = xb_ref[r, :].astype(F32)

        @pl.when(j + NSLOT < npair)
        def _():
            start_pair(j + NSLOT)

        return c

    lax.fori_loop(0, npair, load_pair, 0)
    bw_copy.start()
    bwo_copy.start()

    def b_weights():
        bw_copy.wait()
        bwo_copy.wait()
        rr = lax.broadcasted_iota(jnp.int32, (GR, LANES), 0)
        cc = lax.broadcasted_iota(jnp.int32, (GR, LANES), 1) - (rr & 1) * fb
        for t in range(2):
            parts = [None] * (D // GR)
            for n in range(D // LANES):
                lo = (n * LANES) // GR
                hi = ((n + 1) * LANES - 1) // GR + 1
                col = cc + n * LANES
                wrep = wrep_ref[:, n * LANES:(n + 1) * LANES]
                lhs = jnp.concatenate([
                    jnp.where((col >= g * GR) & (col < g * GR + fb), wrep, 0.0)
                    for g in range(lo, hi)
                ], axis=0)
                y = lax.dot_general(
                    lhs, bw_ref[:, t * D + n * LANES:t * D + (n + 1) * LANES], NT,
                    preferred_element_type=F32)
                for g in range(lo, hi):
                    piece = y[(g - lo) * GR:(g - lo + 1) * GR]
                    parts[g] = piece if parts[g] is None else parts[g] + piece
            w = jnp.concatenate(parts, axis=0) * LOG2E
            bwt_ref[t] = _pack(w.astype(BF16))
        bwt_ref[2] = _pack(bw_ref[:, 2 * D:3 * D].T)
        bwo_ref[...] = _pack(bwo_stage_ref[...])

    def a_step(short, s, c):
        rows = pl.ds(pl.multiple_of(s * seg, seg), seg)
        row = lax.broadcasted_iota(jnp.int32, (L, LANES), 0)
        lane = lax.broadcasted_iota(jnp.int32, (L, LANES), 1)
        is_a = lane < L
        col = jnp.where(is_a, lane, lane - L)
        inside = col < L
        vis = ((row < M) | (row >= col)) & inside
        vis_a = vis & is_a
        vis_b = vis & jnp.logical_not(is_a)
        fill_a = jnp.where(is_a, -1e9 * LOG2E, -jnp.inf)
        fill_b = jnp.where(inside & jnp.logical_not(is_a), -1e9 * LOG2E, -jnp.inf)
        low = lane < dh - LANES
        scale = dh ** -0.5 * LOG2E

        def proj(j, t):
            cols = slice(t * PW, (t + 1) * PW)
            w = _unpack(wqkv_ref[j, :, cols])
            if not short:
                h = jnp.concatenate([memf_ref[...], xna_ref[rows, :]], axis=0)
                return jnp.dot(h, w, preferred_element_type=F32)
            head = pl.ds(pl.multiple_of(s * seg, seg), seg - 8)
            h = jnp.concatenate([memf_ref[...], xna_ref[head, :]], axis=0)
            y = jnp.dot(h.astype(BF16), w, preferred_element_type=F32)
            tail = pre_ref[j, pl.ds(pl.multiple_of(s * 8, 8), 8), cols]
            return jnp.concatenate([y, tail], axis=0)

        def blockdiag(a):
            zero = jnp.zeros((L, LANES), F32)
            mid = a[:, LANES:2 * LANES]
            top = jnp.concatenate(
                [a[:, :LANES], jnp.where(low, mid, 0.0), zero], axis=1)
            bot = jnp.concatenate(
                [zero, jnp.where(low, 0.0, mid), a[:, 2 * LANES:]], axis=1)
            pad = jnp.zeros((LANES - 2 * L, PW), F32)
            return jnp.concatenate([top, bot, pad], axis=0).astype(BF16)

        def probs(q, k):
            sc = lax.dot_general(q, blockdiag(k), NT, preferred_element_type=F32)
            sc = sc * scale
            sa = jnp.where(vis_a, sc, fill_a)
            sb = jnp.where(vis_b, sc, fill_b)
            ma = jnp.max(sa, axis=1, keepdims=True)
            mb = jnp.max(sb, axis=1, keepdims=True)
            e = jnp.exp2(jnp.where(is_a, sa - ma, sb - mb))
            la = jnp.sum(jnp.where(is_a, e, 0.0), axis=1, keepdims=True)
            lb = jnp.sum(jnp.where(is_a, 0.0, e), axis=1, keepdims=True)
            return e * (1.0 / jnp.where(is_a, la, lb))

        prv = pl.ds(pl.multiple_of(jnp.maximum(s - 1, 0) * seg, seg), seg)
        nxt = pl.ds(pl.multiple_of(jnp.minimum(s + 1, nseg - 1) * seg, seg), seg)
        xnb_ref[prv, :] = _layernorm(xres_ref[prv, :]).astype(BF16)
        xn_next = _layernorm(xres_ref[nxt, :])

        q, k, v, p, o = {}, {}, {}, {}, {}
        acc = None
        for op, j in _a_schedule(npair, short):
            if op == "q":
                q[j] = proj(j, 0)
            elif op == "k":
                k[j] = proj(j, 1)
            elif op == "v":
                v[j] = proj(j, 2)
            elif op == "s":
                p[j] = probs(q.pop(j), k.pop(j))
            elif op == "p":
                o[j] = jnp.dot(
                    p.pop(j), blockdiag(v.pop(j)), preferred_element_type=F32)
                if j == npair - 1:
                    xna_ref[nxt, :] = xn_next
            else:
                y = jnp.dot(
                    o.pop(j), _unpack(wo_ref[j]), preferred_element_type=F32)
                acc = y if acc is None else acc + y
        memf_ref[...] = acc[:M]
        xres_ref[rows, :] = xres_ref[rows, :] + acc[M:]
        return c

    def layer_a(n):
        memf_ref[...] = mem_ref[...].astype(F32)
        xna_ref[0:seg, :] = _layernorm(xres_ref[0:seg, :])
        first = jnp.where(n == 0, NPRE, 0)
        lax.fori_loop(0, first, functools.partial(a_step, True), 0)
        lax.fori_loop(first, nseg, functools.partial(a_step, False), 0)
        xnb_ref[S - seg:S, :] = _layernorm(xres_ref[S - seg:S, :]).astype(BF16)

    def b_proj(t, half, rows):
        w = _unpack(bwt_ref[t, half * (HR // 2):(half + 1) * (HR // 2), :])
        return lax.dot_general(
            w, xnb_ref[rows, :], NT, preferred_element_type=F32)

    def fold(vals, op):
        r = functools.reduce(op, vals)
        r = op(r, pltpu.roll(r, 4, 0))
        return op(r, pltpu.roll(r, 2, 0))

    def exps(a, g):
        slabs = [a[g * GR + 8 * i:g * GR + 8 * i + 8] for i in range(GR // 8)]
        mx = fold(slabs, jnp.maximum)
        mn = fold(slabs, jnp.minimum)
        ep = [jnp.exp2(u - mx) for u in slabs]
        en = [jnp.exp2(mn - u) for u in slabs]
        return ep, en, 1.0 / fold(ep, jnp.add), 1.0 / fold(en, jnp.add)

    def unit_rows(i, u):
        start = (i * B_UNROLL + u) * TB
        return pl.ds(pl.multiple_of(start, TB), TB)

    units = [(u, half) for u in range(B_UNROLL) for half in range(2)]

    def b_pass1(i, c):
        def features(u, half):
            a = b_proj(1, half, unit_rows(i, u))
            phi = []
            for g in range(NG):
                ep, en, ip, im = exps(a, g)
                phi += [e * ip for e in ep] + [e * im for e in en]
            phi = jnp.concatenate(phi, axis=0)
            zsum = phi[:, :LANES]
            for n in range(1, TB // LANES):
                zsum = zsum + phi[:, n * LANES:(n + 1) * LANES]
            z_ref[half] += zsum
            return phi.astype(BF16)

        def outer(half, vt, phi):
            for n, (lo, hi) in enumerate(spans):
                kv_ref[half, offs[n]:offs[n + 1], :] += lax.dot_general(
                    vt[lo:hi], phi[n * LANES:(n + 1) * LANES], NT,
                    preferred_element_type=F32)

        phi = features(*units[0])
        for n, (u, half) in enumerate(units):
            vt = b_proj(2, half, unit_rows(i, u))
            phi_next = features(*units[n + 1]) if n + 1 < len(units) else None
            outer(half, vt, phi)
            phi = phi_next
        return c

    def b_mid():
        for half in range(2):
            zs = jnp.sum(z_ref[half], axis=1, keepdims=True)
            z_ref[half] = jnp.broadcast_to(zs, (2 * HR, LANES))
            for n, (lo, hi) in enumerate(spans):
                r = lax.broadcasted_iota(jnp.int32, (hi - lo, LANES), 0) + lo
                f = lax.broadcasted_iota(jnp.int32, (hi - lo, LANES), 1) + n * LANES
                first = (f & 1) * fb
                for g in range(lo // GR, hi // GR):
                    first = jnp.where(f >= g * 2 * GR, g * GR + (f & 1) * fb, first)
                keep = (r >= first) & (r < first + fb)
                blk = slice(offs[n], offs[n + 1])
                kv_ref[half, blk, :] = jnp.where(keep, kv_ref[half, blk, :], 0.0)

    def out_copy(i):
        r = pl.ds(pl.multiple_of(i * (B_UNROLL * TB), B_UNROLL * TB), B_UNROLL * TB)
        return pltpu.make_async_copy(xb_ref.at[r, :], out_hbm.at[r, :], osem.at[i])

    def b_pass2(layer, i, c):
        def features(u, half):
            a = b_proj(0, half, unit_rows(i, u))
            phi = []
            for g in range(NG):
                ep, en, ip, im = exps(a, g)

                def zdot(es, base):
                    terms = []
                    for n, e in enumerate(es):
                        z = z_ref[half, base + 8 * n:base + 8 * n + 8, :]
                        terms.append(e * jnp.concatenate([z] * (TB // LANES), axis=1))
                    return functools.reduce(jnp.add, terms)

                den = zdot(ep, 2 * GR * g) * ip + zdot(en, 2 * GR * g + GR) * im
                inv = 1.0 / (fold([den], jnp.add) + 1e-6)
                ip, im = ip * inv, im * inv
                phi += [e * ip for e in ep] + [e * im for e in en]
            return jnp.concatenate(phi, axis=0).astype(BF16)

        def mix(half, phi):
            parts = [None] * NG
            for n, (lo, hi) in enumerate(spans):
                y = jnp.dot(
                    kv_ref[half, offs[n]:offs[n + 1], :],
                    phi[n * LANES:(n + 1) * LANES], preferred_element_type=F32)
                for g in range(lo // GR, hi // GR):
                    piece = y[g * GR - lo:(g + 1) * GR - lo]
                    parts[g] = piece if parts[g] is None else parts[g] + piece
            return jnp.concatenate(parts, axis=0)

        def finish(u, halves):
            rows = unit_rows(i, u)
            ot = jnp.concatenate(halves, axis=0).astype(BF16)
            y = lax.dot_general(
                ot, _unpack(bwo_ref[...]), TN, preferred_element_type=F32)
            y = xres_ref[rows, :] + y
            xres_ref[rows, :] = y
            xb_ref[rows, :] = y.astype(BF16)

        phis = [features(*units[0]), features(*units[1])]
        halves, pending = [], None
        for n, (u, half) in enumerate(units):
            if n + 2 < len(units):
                phis.append(features(*units[n + 2]))
            halves.append(mix(half, phis.pop(0)))
            if pending is not None:
                finish(*pending)
                pending = None
            if half == 1:
                pending, halves = (u, halves), []
        finish(*pending)

        @pl.when(layer == 1)
        def _():
            out_copy(i).start()

        return c

    nblk = S // (B_UNROLL * TB)

    def layer(n, c):
        layer_a(n)
        pl.when(n == 0)(b_weights)
        kv_ref[...] = jnp.zeros(kv_ref.shape, F32)
        z_ref[...] = jnp.zeros(z_ref.shape, F32)
        lax.fori_loop(0, nblk, b_pass1, 0)
        b_mid()
        lax.fori_loop(0, nblk, functools.partial(b_pass2, n), 0)
        return c

    lax.fori_loop(0, 2, layer, 0)
    for i in range(nblk):
        out_copy(i).wait()


@functools.partial(jax.jit, static_argnames=("A_seg_len",))
def pallas_interleave_layers__memory_aug_recurrent_mem_tr__linear_kernel_hedgehog__prompt_kernel(
    A_x: jax.Array,
    A_mem0: jax.Array,
    A_Wq: jax.Array,
    A_Wk: jax.Array,
    A_Wv: jax.Array,
    A_Wo: jax.Array,
    A_seg_len: int,
    B_x: jax.Array,
    B_wqkv: jax.Array,
    B_w_phi: jax.Array,
    B_wo: jax.Array,
):
    del B_x
    _, S, D = A_x.shape
    M = A_mem0.shape[1]
    _, H, dh = A_Wq.shape
    hb = B_w_phi.shape[0]
    seg = int(A_seg_len)
    npair, PW = H // 2, 2 * dh
    assert A_x.shape[0] == 1 and PW == 3 * LANES and 2 * (M + seg) <= LANES
    assert D == 5 * LANES and hb == 32 and S % (B_UNROLL * TB) == 0

    def rows_first(w):
        return jnp.transpose(w, (1, 2, 0)).reshape(H * dh, D)

    hbm = pl.BlockSpec(memory_space=pl.ANY)
    vmem = pl.BlockSpec(memory_space=pltpu.VMEM)
    out = pl.pallas_call(
        functools.partial(_kernel, seg=seg, dh=dh, hb=hb),
        out_shape=jax.ShapeDtypeStruct((S, D), BF16),
        in_specs=[hbm, hbm, vmem, hbm, hbm, hbm, hbm, hbm, vmem, hbm],
        out_specs=hbm,
        scratch_shapes=[
            pltpu.VMEM((S, D), BF16),
            pltpu.VMEM((S, D), F32),
            pltpu.VMEM((S, D), F32),
            pltpu.VMEM((S, D), BF16),
            pltpu.VMEM((M, D), F32),
            pltpu.VMEM((NSLOT, 4, PW, D), BF16),
            pltpu.VMEM((npair, D // 2, 3 * PW), U32),
            pltpu.VMEM((npair, PW // 2, D), U32),
            pltpu.VMEM((D, 3 * D), BF16),
            pltpu.VMEM((D, D), BF16),
            pltpu.VMEM((3, D // 2, D), U32),
            pltpu.VMEM((D // 2, D), U32),
            pltpu.VMEM((2, 480, LANES), F32),
            pltpu.VMEM((2, D, LANES), F32),
            pltpu.VMEM((NPRE, 8, D), BF16),
            pltpu.VMEM((NPRE * 4, D), U32),
            pltpu.VMEM((npair, NPRE * 8, 3 * PW), F32),
            pltpu.VMEM((2 * D // hb, D), F32),
            pltpu.SemaphoreType.DMA((NSLOT, 5)),
            pltpu.SemaphoreType.DMA((3,)),
            pltpu.SemaphoreType.DMA((S // (B_UNROLL * TB),)),
        ],
        compiler_params=pltpu.CompilerParams(vmem_limit_bytes=112 * 1024 * 1024),
    )(
        A_x.reshape(S, D),
        A_x.reshape(S // seg, seg // 8, 8, D),
        A_mem0.reshape(M, D),
        rows_first(A_Wq),
        rows_first(A_Wk),
        rows_first(A_Wv),
        A_Wo.reshape(H * dh, D),
        B_wqkv,
        jnp.transpose(B_w_phi, (1, 2, 0)),
        B_wo,
    )
    return out.reshape(1, S, D)
```

```python
import functools

import jax
import jax.numpy as jnp
from jax import lax
import jax.experimental.pallas as pl
import jax.experimental.pallas.tpu as pltpu

F32 = jnp.float32
BF16 = jnp.bfloat16
U32 = jnp.uint32
LOG2E = 1.4426950408889634
NT = (((1,), (1,)), ((), ()))
TN = (((0,), (0,)), ((), ()))
LANES = 128

NSLOT = 2
TB = 512
P2 = "f00 f01 f10 f11 m00 m01 m10 a0 m11 b0 a1 b1"
A_UNROLL = {False: 2, True: 2}
NPRE = 44


def _layernorm(x):
    m = jnp.mean(x, axis=-1, keepdims=True)
    xc = x - m
    v = jnp.mean(xc * xc, axis=-1, keepdims=True)
    return xc * lax.rsqrt(v + 1e-5)


def _pack(w):
    return pltpu.bitcast(w, U32)


def _unpack(w):
    return pltpu.bitcast(w, BF16)


def _a_schedule(npair, short):
    s = [("k", 0), ("q", 0), ("v", 0)]
    done = 0
    for j in range(npair - 1):
        s += [("s", j), ("k", j + 1), ("q", j + 1)]
        if short and j > 0:
            s.append(("a", done))
            done += 1
        s += [("v", j + 1), ("p", j)]
    last = npair - 1
    s += [("s", last)] + [("b", i) for i in range(7)] + [("p", last)]
    s += [("a", i) for i in range(done, last)]
    s += [("b", i) for i in range(7, 10)] + [("a", last)]
    return s + [("b", i) for i in range(10, npair)]


def _kernel(
    x_hbm, x4_hbm, mem_ref, wq_hbm, wk_hbm, wv_hbm, wo_hbm, bw_hbm, wphi_ref, bwo_hbm,
    out_hbm,
    xb_ref, xres_ref, xna_ref, xnb_ref, memf_ref,
    stage_ref, wqkv_ref, wo_ref,
    bw_ref, bwo_stage_ref, bwt_ref, bwo_ref,
    kv_ref, z_ref, xsel_ref, xseln_ref, pre_ref, wrep_ref,
    wsem, sem, osem,
    *, seg, dh, hb,
):
    S, D = xres_ref.shape
    M = mem_ref.shape[0]
    L = M + seg
    nseg = S // seg
    PW = 2 * dh
    npair = wqkv_ref.shape[0]
    fb = D // hb
    GR = 2 * fb
    HR = D // 2
    NG = HR // GR
    NTILE = 2 * HR // LANES
    spans = []
    for i in range(NTILE):
        lo = (i * LANES) // (2 * GR)
        hi = ((i + 1) * LANES - 1) // (2 * GR) + 1
        spans.append((lo * GR, hi * GR))
    offs = [0]
    for lo, hi in spans:
        offs.append(offs[-1] + hi - lo)

    XP = S // npair

    NCOPY = 5

    def wcopy(j, t):
        rows = pl.ds(pl.multiple_of(j * PW, PW), PW)
        if t < 3:
            src = (wq_hbm, wk_hbm, wv_hbm)[t].at[rows, :]
            dst = stage_ref.at[j % NSLOT, t]
        elif t == 3:
            part = pl.ds(pl.multiple_of(j * XP, XP), XP)
            src, dst = x_hbm.at[part, :], xb_ref.at[part, :]
        else:
            src, dst = wo_hbm.at[rows, :], wo_ref.at[rows, :]
        return pltpu.make_async_copy(src, dst, wsem.at[j % NSLOT, t])

    def start_pair(j):
        for t in range(NCOPY):
            wcopy(j, t).start()

    xsel_copy = pltpu.make_async_copy(
        x4_hbm.at[0:NPRE, seg // 8 - 1], xsel_ref, sem.at[0])
    bw_copy = pltpu.make_async_copy(bw_hbm, bw_ref, sem.at[1])
    bwo_copy = pltpu.make_async_copy(bwo_hbm, bwo_stage_ref, sem.at[2])
    xsel_copy.start()
    start_pair(0)

    wcat = None
    hh = lax.broadcasted_iota(jnp.int32, (hb, D), 0)
    cc = lax.broadcasted_iota(jnp.int32, (hb, D), 1)
    for d in range(fb):
        sel = jnp.where(cc == hh * fb + d, 1.0, 0.0).astype(BF16)
        t = jnp.dot(wphi_ref[d], sel, preferred_element_type=F32)
        wcat = t if wcat is None else wcat + t
    rr = lax.broadcasted_iota(jnp.int32, (GR, fb), 0)
    ff = lax.broadcasted_iota(jnp.int32, (GR, fb), 1)
    twice = jnp.where((rr >> 1) == ff, 1.0, 0.0).astype(BF16)
    wrep_ref[...] = jnp.dot(twice, wcat.astype(BF16), preferred_element_type=F32)

    xsel_copy.wait()
    start_pair(1)
    xsel = xsel_ref[...].astype(F32).reshape(NPRE * 8, D)
    xseln_ref[...] = _pack(_layernorm(xsel).astype(BF16))
    for j in range(2, NSLOT):
        start_pair(j)

    def load_pair(j, c):
        slot = j % NSLOT
        for t in range(3):
            wcopy(j, t).wait()
        for t in range(3):
            cols = slice(t * PW, (t + 1) * PW)
            wqkv_ref[j, :, cols] = _pack(
                stage_ref[slot, t].astype(F32).T.astype(BF16))
            xn = _unpack(xseln_ref[...])
            if t == 0:
                y = lax.dot_general(
                    xn, stage_ref[slot, t], NT, preferred_element_type=F32)
            else:
                y = jnp.dot(xn, _unpack(wqkv_ref[j, :, cols]),
                            preferred_element_type=F32)
            pre_ref[j, :, cols] = y
        for t in range(3, NCOPY):
            wcopy(j, t).wait()

        @pl.when(j + NSLOT < npair)
        def _():
            start_pair(j + NSLOT)

        return c

    lax.fori_loop(0, npair, load_pair, 0)
    bw_copy.start()
    bwo_copy.start()
    xres_ref[0:seg, :] = xb_ref[0:seg, :].astype(F32)

    def b_weights():
        bw_copy.wait()
        bwo_copy.wait()
        rr = lax.broadcasted_iota(jnp.int32, (GR, LANES), 0)
        cc = lax.broadcasted_iota(jnp.int32, (GR, LANES), 1) - (rr & 1) * fb
        for t in range(2):
            parts = [None] * (D // GR)
            for n in range(D // LANES):
                lo = (n * LANES) // GR
                hi = ((n + 1) * LANES - 1) // GR + 1
                col = cc + n * LANES
                wrep = wrep_ref[:, n * LANES:(n + 1) * LANES]
                lhs = jnp.concatenate([
                    jnp.where((col >= g * GR) & (col < g * GR + fb), wrep, 0.0)
                    for g in range(lo, hi)
                ], axis=0)
                y = lax.dot_general(
                    lhs, bw_ref[:, t * D + n * LANES:t * D + (n + 1) * LANES], NT,
                    preferred_element_type=F32)
                for g in range(lo, hi):
                    piece = y[(g - lo) * GR:(g - lo + 1) * GR]
                    parts[g] = piece if parts[g] is None else parts[g] + piece
            w = jnp.concatenate(parts, axis=0) * LOG2E
            bwt_ref[t] = _pack(w.astype(BF16))
        bwt_ref[2] = _pack(bw_ref[:, 2 * D:3 * D].T)
        bwo_ref[...] = _pack(bwo_stage_ref[...])

    def a_step(short, s, mem, chained_in):
        rows = pl.ds(pl.multiple_of(s * seg, seg), seg)
        row = lax.broadcasted_iota(jnp.int32, (L, LANES), 0)
        lane = lax.broadcasted_iota(jnp.int32, (L, LANES), 1)
        is_a = lane < L
        col = jnp.where(is_a, lane, lane - L)
        inside = col < L
        vis = ((row < M) | (row >= col)) & inside
        vis_a = vis & is_a
        vis_b = vis & jnp.logical_not(is_a)
        fill_a = jnp.where(is_a, -1e9 * LOG2E, -jnp.inf)
        fill_b = jnp.where(inside & jnp.logical_not(is_a), -1e9 * LOG2E, -jnp.inf)
        low = lane < dh - LANES
        scale = dh ** -0.5 * LOG2E

        def part(j, t, lo, hi):
            n = seg - 8 if short else seg
            x = xna_ref[pl.ds(pl.multiple_of(s * seg, seg), n), lo:hi]
            h = jnp.concatenate([mem[:, lo:hi], x], axis=0)
            w = _unpack(wqkv_ref[j, lo // 2:hi // 2, t * PW:(t + 1) * PW])
            return jnp.dot(h.astype(BF16) if short else h, w,
                           preferred_element_type=F32)

        def proj(j, t, head=None):
            if head is None:
                y = part(j, t, 0, D)
            else:
                y = part(j, t, PW, D) + head
            if short:
                tail = pl.ds(pl.multiple_of(s * 8, 8), 8)
                y = jnp.concatenate(
                    [y, pre_ref[j, tail, t * PW:(t + 1) * PW]], axis=0)
            return y

        def blockdiag(a):
            zero = jnp.zeros((L, LANES), F32)
            mid = a[:, LANES:2 * LANES]
            top = jnp.concatenate(
                [a[:, :LANES], jnp.where(low, mid, 0.0), zero], axis=1)
            bot = jnp.concatenate(
                [zero, jnp.where(low, 0.0, mid), a[:, 2 * LANES:]], axis=1)
            pad = jnp.zeros((LANES - 2 * L, PW), F32)
            return jnp.concatenate([top, bot, pad], axis=0).astype(BF16)

        def probs(q, k):
            sc = lax.dot_general(q, blockdiag(k), NT, preferred_element_type=F32)
            sc = sc * scale
            sa = jnp.where(vis_a, sc, fill_a)
            sb = jnp.where(vis_b, sc, fill_b)
            ma = jnp.max(sa, axis=1, keepdims=True)
            mb = jnp.max(sb, axis=1, keepdims=True)
            e = jnp.exp2(jnp.where(is_a, sa - ma, sb - mb))
            la = jnp.sum(jnp.where(is_a, e, 0.0), axis=1, keepdims=True)
            lb = jnp.sum(jnp.where(is_a, 0.0, e), axis=1, keepdims=True)
            return e * (1.0 / jnp.where(is_a, la, lb))

        prv = pl.ds(pl.multiple_of(jnp.maximum(s - 1, 0) * seg, seg), seg)
        nxt = pl.ds(pl.multiple_of(jnp.minimum(s + 1, nseg - 1) * seg, seg), seg)
        xnb_ref[prv, :] = _layernorm(xres_ref[prv, :]).astype(BF16)
        if short:
            far = pl.ds(
                pl.multiple_of(jnp.minimum(s + NPRE, nseg - 1) * seg, seg), seg)
            xres_ref[far, :] = xb_ref[far, :].astype(F32)
        xin_ref = xb_ref if short else xres_ref
        xn_next = _layernorm(xin_ref[nxt, :].astype(F32))

        q, k, v, p, o = {}, {}, {}, {}, {}
        acc = [None, None]
        head_k = head_q = None
        if chained_in:
            head_k, head_q = part(0, 1, 0, PW), part(0, 0, 0, PW)
        for op, j in _a_schedule(npair, short):
            if op == "q":
                q[j] = proj(j, 0, head_q if j == 0 else None)
            elif op == "k":
                k[j] = proj(j, 1, head_k if j == 0 else None)
            elif op == "v":
                v[j] = proj(j, 2)
            elif op == "s":
                p[j] = probs(q.pop(j), k.pop(j))
            elif op == "p":
                o[j] = jnp.dot(
                    p.pop(j), blockdiag(v.pop(j)), preferred_element_type=F32)
                if j == npair - 1:
                    xna_ref[nxt, :] = xn_next
            else:
                n = "ab".index(op)
                cols = (slice(0, PW), slice(PW, D))[n]
                y = jnp.dot(o[j], wo_ref[j * PW:(j + 1) * PW, cols],
                            preferred_element_type=F32)
                acc[n] = y if acc[n] is None else acc[n] + y
        acc = jnp.concatenate(acc, axis=1)
        xres_ref[rows, :] = xin_ref[rows, :].astype(F32) + acc[M:]
        return acc[:M]

    def a_steps(short, i, c):
        mem = memf_ref[...]
        n = A_UNROLL[short]
        for u in range(n):
            mem = a_step(short, i * n + u, mem, u > 0)
        memf_ref[...] = mem
        return c

    def layer_a(n):
        memf_ref[...] = mem_ref[...].astype(F32)
        xna_ref[0:seg, :] = _layernorm(xres_ref[0:seg, :])
        lax.fori_loop(0, jnp.where(n == 0, NPRE // A_UNROLL[True], 0),
                      functools.partial(a_steps, True), 0)
        lax.fori_loop(jnp.where(n == 0, NPRE // A_UNROLL[False], 0),
                      nseg // A_UNROLL[False],
                      functools.partial(a_steps, False), 0)
        xnb_ref[S - seg:S, :] = _layernorm(xres_ref[S - seg:S, :]).astype(BF16)

    def b_proj(t, half, rows):
        w = _unpack(bwt_ref[t, half * (HR // 2):(half + 1) * (HR // 2), :])
        return lax.dot_general(
            w, xnb_ref[rows, :], NT, preferred_element_type=F32)

    def fold(vals, op):
        r = functools.reduce(op, vals)
        r = op(r, pltpu.roll(r, 4, 0))
        return op(r, pltpu.roll(r, 2, 0))

    def exps(a, g):
        slabs = [a[g * GR + 8 * i:g * GR + 8 * i + 8] for i in range(GR // 8)]
        mx = fold(slabs, jnp.maximum)
        mn = fold(slabs, jnp.minimum)
        ep = [jnp.exp2(u - mx) for u in slabs]
        en = [jnp.exp2(mn - u) for u in slabs]
        return ep, en, fold(ep, jnp.add), fold(en, jnp.add)

    def b_pass1(i, c):
        rows = pl.ds(pl.multiple_of(i * TB, TB), TB)

        def features(half):
            a = b_proj(1, half, rows)
            phi = []
            for g in range(NG):
                ep, en, sp, sn = exps(a, g)
                inv = 1.0 / (sp * sn)
                ip, im = sn * inv, sp * inv
                phi += [e * ip for e in ep] + [e * im for e in en]
            phi = jnp.concatenate(phi, axis=0)
            zsum = phi[:, :LANES]
            for n in range(1, TB // LANES):
                zsum = zsum + phi[:, n * LANES:(n + 1) * LANES]
            z_ref[half] += zsum
            return phi.astype(BF16)

        def outer(half, vt, phi):
            for n, (lo, hi) in enumerate(spans):
                kv_ref[half, offs[n]:offs[n + 1], :] += lax.dot_general(
                    vt[lo:hi], phi[n * LANES:(n + 1) * LANES], NT,
                    preferred_element_type=F32)

        phi0 = features(0)
        phi1 = features(1)
        vt0 = b_proj(2, 0, rows)
        vt1 = b_proj(2, 1, rows)
        outer(0, vt0, phi0)
        outer(1, vt1, phi1)
        return c

    def b_mid():
        for half in range(2):
            zs = jnp.sum(z_ref[half], axis=1, keepdims=True)
            z_ref[half] = jnp.broadcast_to(zs, (2 * HR, LANES))
            for n, (lo, hi) in enumerate(spans):
                r = lax.broadcasted_iota(jnp.int32, (hi - lo, LANES), 0) + lo
                f = lax.broadcasted_iota(jnp.int32, (hi - lo, LANES), 1) + n * LANES
                first = (f & 1) * fb
                for g in range(lo // GR, hi // GR):
                    first = jnp.where(f >= g * 2 * GR, g * GR + (f & 1) * fb, first)
                keep = (r >= first) & (r < first + fb)
                blk = slice(offs[n], offs[n + 1])
                kv_ref[half, blk, :] = jnp.where(keep, kv_ref[half, blk, :], 0.0)

    def out_copy(i):
        r = pl.ds(pl.multiple_of(i * TB, TB), TB)
        return pltpu.make_async_copy(xb_ref.at[r, :], out_hbm.at[r, :], osem.at[i])

    def b_pass2(layer, i, c):
        tu = TB // 2

        def unit_rows(u):
            return pl.ds(pl.multiple_of(i * TB + u * tu, tu), tu)

        def features(u, half):
            a = b_proj(0, half, unit_rows(u))
            phi = []
            for g in range(NG):
                ep, en, sp, sn = exps(a, g)

                def zdot(es, base):
                    terms = []
                    for n, e in enumerate(es):
                        z = z_ref[half, base + 8 * n:base + 8 * n + 8, :]
                        terms.append(e * jnp.concatenate([z] * (tu // LANES), axis=1))
                    return functools.reduce(jnp.add, terms)

                den = zdot(ep, 2 * GR * g) * sn + zdot(en, 2 * GR * g + GR) * sp
                inv = 1.0 / (fold([den], jnp.add) + 1e-6 * (sp * sn))
                ip, im = sn * inv, sp * inv
                phi += [e * ip for e in ep] + [e * im for e in en]
            return jnp.concatenate(phi, axis=0).astype(BF16)

        def mix(half, phi):
            parts = [None] * NG
            for n, (lo, hi) in enumerate(spans):
                y = jnp.dot(
                    kv_ref[half, offs[n]:offs[n + 1], :],
                    phi[n * LANES:(n + 1) * LANES], preferred_element_type=F32)
                for g in range(lo // GR, hi // GR):
                    piece = y[g * GR - lo:(g + 1) * GR - lo]
                    parts[g] = piece if parts[g] is None else parts[g] + piece
            return jnp.concatenate(parts, axis=0)

        def finish(u, cols, o):
            rows = unit_rows(u)
            y = jnp.dot(o, _unpack(bwo_ref[:, cols]), preferred_element_type=F32)
            y = xres_ref[rows, cols] + y
            xres_ref[rows, cols] = y
            xb_ref[rows, cols] = y.astype(BF16)

        phi, ot, o = {}, {}, {}
        for op in P2.split():
            u = int(op[1])
            if op[0] == "f":
                phi[op[1:]] = features(u, int(op[2]))
            elif op[0] == "m":
                ot[op[1:]] = mix(int(op[2]), phi.pop(op[1:]))
                if op[2] == "1":
                    o[u] = jnp.concatenate(
                        [ot.pop(op[1] + "0"), ot.pop(op[1:])], axis=0).T
            else:
                finish(u, slice(0, PW) if op[0] == "a" else slice(PW, D), o[u])

        @pl.when(layer == 1)
        def _():
            out_copy(i).start()

        return c

    nblk = S // TB

    def layer(n, c):
        layer_a(n)
        pl.when(n == 0)(b_weights)
        kv_ref[...] = jnp.zeros(kv_ref.shape, F32)
        z_ref[...] = jnp.zeros(z_ref.shape, F32)
        lax.fori_loop(0, nblk, b_pass1, 0)
        b_mid()
        lax.fori_loop(0, nblk, functools.partial(b_pass2, n), 0)
        return c

    lax.fori_loop(0, 2, layer, 0)
    for i in range(nblk):
        out_copy(i).wait()


@functools.partial(jax.jit, static_argnames=("A_seg_len",))
def pallas_interleave_layers__memory_aug_recurrent_mem_tr__linear_kernel_hedgehog__prompt_kernel(
    A_x: jax.Array,
    A_mem0: jax.Array,
    A_Wq: jax.Array,
    A_Wk: jax.Array,
    A_Wv: jax.Array,
    A_Wo: jax.Array,
    A_seg_len: int,
    B_x: jax.Array,
    B_wqkv: jax.Array,
    B_w_phi: jax.Array,
    B_wo: jax.Array,
):
    del B_x
    _, S, D = A_x.shape
    M = A_mem0.shape[1]
    _, H, dh = A_Wq.shape
    hb = B_w_phi.shape[0]
    seg = int(A_seg_len)
    npair, PW = H // 2, 2 * dh
    assert A_x.shape[0] == 1 and PW == 3 * LANES and 2 * (M + seg) <= LANES
    assert 2 * NPRE * seg >= S and D == 5 * LANES and hb == 32 and S % TB == 0

    def rows_first(w):
        return jnp.transpose(w, (1, 2, 0)).reshape(H * dh, D)

    hbm = pl.BlockSpec(memory_space=pl.ANY)
    vmem = pl.BlockSpec(memory_space=pltpu.VMEM)
    out = pl.pallas_call(
        functools.partial(_kernel, seg=seg, dh=dh, hb=hb),
        out_shape=jax.ShapeDtypeStruct((S, D), BF16),
        in_specs=[hbm, hbm, vmem, hbm, hbm, hbm, hbm, hbm, vmem, hbm],
        out_specs=hbm,
        scratch_shapes=[
            pltpu.VMEM((S, D), BF16),
            pltpu.VMEM((S, D), F32),
            pltpu.VMEM((S, D), F32),
            pltpu.VMEM((S, D), BF16),
            pltpu.VMEM((M, D), F32),
            pltpu.VMEM((NSLOT, 3, PW, D), BF16),
            pltpu.VMEM((npair, D // 2, 3 * PW), U32),
            pltpu.VMEM((H * dh, D), BF16),
            pltpu.VMEM((D, 3 * D), BF16),
            pltpu.VMEM((D, D), BF16),
            pltpu.VMEM((3, D // 2, D), U32),
            pltpu.VMEM((D // 2, D), U32),
            pltpu.VMEM((2, 480, LANES), F32),
            pltpu.VMEM((2, D, LANES), F32),
            pltpu.VMEM((NPRE, 8, D), BF16),
            pltpu.VMEM((NPRE * 4, D), U32),
            pltpu.VMEM((npair, NPRE * 8, 3 * PW), F32),
            pltpu.VMEM((2 * D // hb, D), F32),
            pltpu.SemaphoreType.DMA((NSLOT, 5)),
            pltpu.SemaphoreType.DMA((3,)),
            pltpu.SemaphoreType.DMA((S // TB,)),
        ],
        compiler_params=pltpu.CompilerParams(vmem_limit_bytes=112 * 1024 * 1024),
    )(
        A_x.reshape(S, D),
        A_x.reshape(S // seg, seg // 8, 8, D),
        A_mem0.reshape(M, D),
        rows_first(A_Wq),
        rows_first(A_Wk),
        rows_first(A_Wv),
        A_Wo.reshape(H * dh, D),
        B_wqkv,
        jnp.transpose(B_w_phi, (1, 2, 0)),
        B_wo,
    )
    return out.reshape(1, S, D)
```

```python
import functools

import jax
import jax.numpy as jnp
from jax import lax
import jax.experimental.pallas as pl
import jax.experimental.pallas.tpu as pltpu

F32 = jnp.float32
BF16 = jnp.bfloat16
U32 = jnp.uint32
LOG2E = 1.4426950408889634
NT = (((1,), (1,)), ((), ()))
TN = (((0,), (0,)), ((), ()))
LANES = 128

TB = 512
P2 = "f00 f01 f10 f11 m00 m01 m10 a0 m11 b0 a1 b1"
A_UNROLL = {False: 2, True: 2}
NOBC = True
NSLOT = 3
NPRE = 44


def _layernorm(x):
    m = jnp.mean(x, axis=-1, keepdims=True)
    xc = x - m
    v = jnp.mean(xc * xc, axis=-1, keepdims=True)
    return xc * lax.rsqrt(v + 1e-5)


def _pack(w):
    return pltpu.bitcast(w, U32)


def _unpack(w):
    return pltpu.bitcast(w, BF16)


def _a_schedule(npair, short):
    s = [("k", 0), ("q", 0), ("v", 0)]
    done = 0
    for j in range(npair - 1):
        s += [("s", j), ("k", j + 1), ("q", j + 1)]
        if short and j > 0:
            s.append(("a", done))
            done += 1
        s += [("v", j + 1), ("p", j)]
    last = npair - 1
    s += [("s", last)] + [("b", i) for i in range(7)] + [("p", last)]
    s += [("a", i) for i in range(done, last)]
    s += [("b", i) for i in range(7, 10)] + [("a", last)]
    return s + [("b", i) for i in range(10, npair)]


def _kernel(
    x_hbm, x4_hbm, mem_hbm, wq_hbm, wk_hbm, wv_hbm, wo_hbm, bw_hbm, wphi_hbm, bwo_hbm,
    out_hbm,
    xb_ref, xres_ref, xna_ref, xnb_ref, memf_ref,
    stage_ref, wqkv_ref, wo_ref,
    bw_ref, bwo_stage_ref, bwt_ref, bwo_ref,
    kv_ref, z_ref, xsel_ref, xseln_ref, pre_ref, mem_ref, wphi_ref, wrep_ref,
    wsem, sem, osem,
    *, seg, dh, hb,
):
    S, D = xres_ref.shape
    M = mem_ref.shape[0]
    L = M + seg
    nseg = S // seg
    PW = 2 * dh
    npair = wqkv_ref.shape[0]
    fb = D // hb
    GR = 2 * fb
    HR = D // 2
    NG = HR // GR
    NTILE = 2 * HR // LANES
    spans = []
    for i in range(NTILE):
        lo = (i * LANES) // (2 * GR)
        hi = ((i + 1) * LANES - 1) // (2 * GR) + 1
        spans.append((lo * GR, hi * GR))
    offs = [0]
    for lo, hi in spans:
        offs.append(offs[-1] + hi - lo)

    XH = (A_UNROLL[True] + 2) * seg

    def wcopy(j, t):
        rows = pl.ds(pl.multiple_of(j * PW, PW), PW)
        return pltpu.make_async_copy(
            (wq_hbm, wk_hbm, wv_hbm)[t].at[rows, :],
            stage_ref.at[j % NSLOT, t], wsem.at[j % NSLOT, t])

    def start_pair(j):
        for t in range(3):
            wcopy(j, t).start()

    xsel_copy = pltpu.make_async_copy(
        x4_hbm.at[0:NPRE, seg // 8 - 1], xsel_ref, sem.at[0])
    bw_copy = pltpu.make_async_copy(bw_hbm, bw_ref, sem.at[1])
    bwo_copy = pltpu.make_async_copy(bwo_hbm, bwo_stage_ref, sem.at[2])
    xh_copy = pltpu.make_async_copy(
        x_hbm.at[0:XH, :], xb_ref.at[0:XH, :], sem.at[3])
    xt_copy = pltpu.make_async_copy(
        x_hbm.at[XH:S, :], xb_ref.at[XH:S, :], sem.at[3])
    mem_copy = pltpu.make_async_copy(mem_hbm, mem_ref, sem.at[5])
    wphi_copy = pltpu.make_async_copy(wphi_hbm, wphi_ref, sem.at[6])
    wphi_copy.start()
    xsel_copy.start()
    xh_copy.start()
    start_pair(0)

    wphi_copy.wait()
    hh = lax.broadcasted_iota(jnp.int32, (hb, D), 0)
    cc = lax.broadcasted_iota(jnp.int32, (hb, D), 1)

    def spread(i, wcat):
        for d in range(4):
            sel = jnp.where(cc == hh * fb + (4 * i + d), 1.0, 0.0).astype(BF16)
            wcat += jnp.dot(wphi_ref[4 * i + d], sel, preferred_element_type=F32)
        return wcat

    wcat = lax.fori_loop(0, fb // 4, spread, jnp.zeros((fb, D), F32))
    rr = lax.broadcasted_iota(jnp.int32, (GR, fb), 0)
    ff = lax.broadcasted_iota(jnp.int32, (GR, fb), 1)
    twice = jnp.where((rr >> 1) == ff, 1.0, 0.0).astype(BF16)
    wrep_ref[...] = jnp.dot(twice, wcat.astype(BF16), preferred_element_type=F32)

    xsel_copy.wait()
    xsel = xsel_ref[...].astype(F32).reshape(NPRE * 8, D)
    xseln_ref[...] = _pack(_layernorm(xsel).astype(BF16))
    xh_copy.wait()
    xna_ref[0:seg, :] = _layernorm(xb_ref[0:seg, :].astype(F32))

    def load_pair(j, c):
        slot = j % NSLOT
        for t in range(3):
            wcopy(j, t).wait()

        @pl.when(j == 0)
        def _():
            for n in range(1, NSLOT - 1):
                start_pair(n)
            mem_copy.start()

        @pl.when(j + NSLOT - 1 < npair)
        def _():
            start_pair(j + NSLOT - 1)

        part = pl.ds(pl.multiple_of(j * PW, PW), PW)
        pltpu.make_async_copy(
            wo_hbm.at[part, :], wo_ref.at[part, :], sem.at[4]).start()
        for t in range(3):
            cols = slice(t * PW, (t + 1) * PW)
            wqkv_ref[j, :, cols] = _pack(
                stage_ref[slot, t].astype(F32).T.astype(BF16))
            xn = _unpack(xseln_ref[...])
            if t == 0:
                y = lax.dot_general(
                    xn, stage_ref[slot, t], NT, preferred_element_type=F32)
            else:
                y = jnp.dot(xn, _unpack(wqkv_ref[j, :, cols]),
                            preferred_element_type=F32)
            pre_ref[j, :, cols] = y
        return c

    lax.fori_loop(0, npair, load_pair, 0)
    mem_copy.wait()
    pltpu.make_async_copy(wo_hbm, wo_ref, sem.at[4]).wait()
    xt_copy.start()
    bw_copy.start()
    bwo_copy.start()

    def b_weights():
        bw_copy.wait()
        bwo_copy.wait()
        rr = lax.broadcasted_iota(jnp.int32, (GR, LANES), 0)
        cc = lax.broadcasted_iota(jnp.int32, (GR, LANES), 1) - (rr & 1) * fb
        for t in range(2):
            parts = [None] * (D // GR)
            for n in range(D // LANES):
                lo = (n * LANES) // GR
                hi = ((n + 1) * LANES - 1) // GR + 1
                col = cc + n * LANES
                lhs = jnp.concatenate([
                    jnp.where((col >= g * GR) & (col < g * GR + fb),
                              wrep_ref[:, n * LANES:(n + 1) * LANES], 0.0)
                    for g in range(lo, hi)
                ], axis=0)
                y = lax.dot_general(
                    lhs, bw_ref[:, t * D + n * LANES:t * D + (n + 1) * LANES], NT,
                    preferred_element_type=F32)
                for g in range(lo, hi):
                    piece = y[(g - lo) * GR:(g - lo + 1) * GR]
                    parts[g] = piece if parts[g] is None else parts[g] + piece
            w = jnp.concatenate(parts, axis=0) * LOG2E
            bwt_ref[t] = _pack(w.astype(BF16))
        bwt_ref[2] = _pack(bw_ref[:, 2 * D:3 * D].T)
        bwo_ref[...] = _pack(bwo_stage_ref[...])

    def a_step(short, s, mem, chained_in):
        rows = pl.ds(pl.multiple_of(s * seg, seg), seg)
        row = lax.broadcasted_iota(jnp.int32, (L, LANES), 0)
        lane = lax.broadcasted_iota(jnp.int32, (L, LANES), 1)
        is_a = lane < L
        col = jnp.where(is_a, lane, lane - L)
        inside = col < L
        vis = ((row < M) | (row >= col)) & inside
        vis_a = vis & is_a
        vis_b = vis & jnp.logical_not(is_a)
        fill_a = jnp.where(is_a, -1e9 * LOG2E, -jnp.inf)
        fill_b = jnp.where(inside & jnp.logical_not(is_a), -1e9 * LOG2E, -jnp.inf)
        low = lane < dh - LANES
        scale = dh ** -0.5 * LOG2E

        def part(j, t, lo, hi):
            n = seg - 8 if short else seg
            x = xna_ref[pl.ds(pl.multiple_of(s * seg, seg), n), lo:hi]
            h = jnp.concatenate([mem[:, lo:hi], x], axis=0)
            w = _unpack(wqkv_ref[j, lo // 2:hi // 2, t * PW:(t + 1) * PW])
            return jnp.dot(h.astype(BF16) if short else h, w,
                           preferred_element_type=F32)

        def proj(j, t, head=None):
            if head is None:
                y = part(j, t, 0, D)
            else:
                y = part(j, t, PW, D) + head
            if short:
                tail = pl.ds(pl.multiple_of(s * 8, 8), 8)
                y = jnp.concatenate(
                    [y, pre_ref[j, tail, t * PW:(t + 1) * PW]], axis=0)
            return y

        def blockdiag(a):
            zero = jnp.zeros((L, LANES), F32)
            mid = a[:, LANES:2 * LANES]
            top = jnp.concatenate(
                [a[:, :LANES], jnp.where(low, mid, 0.0), zero], axis=1)
            bot = jnp.concatenate(
                [zero, jnp.where(low, 0.0, mid), a[:, 2 * LANES:]], axis=1)
            pad = jnp.zeros((LANES - 2 * L, PW), F32)
            return jnp.concatenate([top, bot, pad], axis=0).astype(BF16)

        def probs(q, k):
            sc = lax.dot_general(q, blockdiag(k), NT, preferred_element_type=F32)
            sc = sc * scale
            sa = jnp.where(vis_a, sc, fill_a)
            sb = jnp.where(vis_b, sc, fill_b)
            ma = jnp.max(sa, axis=1, keepdims=True)
            mb = jnp.max(sb, axis=1, keepdims=True)
            e = jnp.exp2(jnp.where(is_a, sa - ma, sb - mb))
            la = jnp.sum(jnp.where(is_a, e, 0.0), axis=1, keepdims=True)
            lb = jnp.sum(jnp.where(is_a, 0.0, e), axis=1, keepdims=True)
            return e * (1.0 / jnp.where(is_a, la, lb))

        prv = pl.ds(pl.multiple_of(jnp.maximum(s - 1, 0) * seg, seg), seg)
        nxt = pl.ds(pl.multiple_of(jnp.minimum(s + 1, nseg - 1) * seg, seg), seg)
        if short:
            far = jnp.where(s < A_UNROLL[True], s, nseg - 1 + A_UNROLL[True] - s)
            far = jnp.where(far < NPRE, s, far)
            far = pl.ds(pl.multiple_of(far * seg, seg), seg)
            xres_ref[far, :] = xb_ref[far, :].astype(F32)
        xnb_ref[prv, :] = _layernorm(xres_ref[prv, :]).astype(BF16)
        xin_ref = xb_ref if short else xres_ref
        xn_next = _layernorm(xin_ref[nxt, :].astype(F32))

        q, k, v, p, o = {}, {}, {}, {}, {}
        acc = [None, None]
        head_k = head_q = None
        if chained_in:
            head_k, head_q = part(0, 1, 0, PW), part(0, 0, 0, PW)
        for op, j in _a_schedule(npair, short):
            if op == "q":
                q[j] = proj(j, 0, head_q if j == 0 else None)
            elif op == "k":
                k[j] = proj(j, 1, head_k if j == 0 else None)
            elif op == "v":
                v[j] = proj(j, 2)
            elif op == "s":
                p[j] = probs(q.pop(j), k.pop(j))
            elif op == "p":
                o[j] = jnp.dot(
                    p.pop(j), blockdiag(v.pop(j)), preferred_element_type=F32)
                if j == npair - 1:
                    xna_ref[nxt, :] = xn_next
            else:
                n = "ab".index(op)
                cols = (slice(0, PW), slice(PW, D))[n]
                y = jnp.dot(o[j], wo_ref[j * PW:(j + 1) * PW, cols],
                            preferred_element_type=F32)
                acc[n] = y if acc[n] is None else acc[n] + y
        acc = jnp.concatenate(acc, axis=1)
        xres_ref[rows, :] = xin_ref[rows, :].astype(F32) + acc[M:]
        return acc[:M]

    def a_steps(short, i, c):
        if short:
            pl.when(i == 1)(xt_copy.wait)
        mem = memf_ref[...]
        n = A_UNROLL[short]
        for u in range(n):
            mem = a_step(short, i * n + u, mem, u > 0)
        memf_ref[...] = mem
        return c

    def layer_a(n):
        memf_ref[...] = mem_ref[...].astype(F32)
        lax.fori_loop(0, jnp.where(n == 0, NPRE // A_UNROLL[True], 0),
                      functools.partial(a_steps, True), 0)
        lax.fori_loop(jnp.where(n == 0, NPRE // A_UNROLL[False], 0),
                      nseg // A_UNROLL[False],
                      functools.partial(a_steps, False), 0)

    def b_proj(t, half, rows):
        w = _unpack(bwt_ref[t, half * (HR // 2):(half + 1) * (HR // 2), :])
        return lax.dot_general(
            w, xnb_ref[rows, :], NT, preferred_element_type=F32)

    def fold(vals, op):
        r = functools.reduce(op, vals)
        r = op(r, pltpu.roll(r, 4, 0))
        return op(r, pltpu.roll(r, 2, 0))

    def exps(a, g):
        slabs = [a[g * GR + 8 * i:g * GR + 8 * i + 8] for i in range(GR // 8)]
        mx = fold(slabs, jnp.maximum)
        mn = fold(slabs, jnp.minimum)
        ep = [jnp.exp2(u - mx) for u in slabs]
        en = [jnp.exp2(mn - u) for u in slabs]
        return ep, en, fold(ep, jnp.add), fold(en, jnp.add)

    def b_pass1(i, c):
        rows = pl.ds(pl.multiple_of(i * TB, TB), TB)

        def features(half):
            a = b_proj(1, half, rows)
            phi = []
            for g in range(NG):
                ep, en, sp, sn = exps(a, g)
                inv = 1.0 / (sp * sn)
                ip, im = sn * inv, sp * inv
                phi += [e * ip for e in ep] + [e * im for e in en]
            phi = jnp.concatenate(phi, axis=0)
            zsum = phi[:, :LANES]
            for n in range(1, TB // LANES):
                zsum = zsum + phi[:, n * LANES:(n + 1) * LANES]
            z_ref[half] = jnp.where(i > 0, z_ref[half], 0.0) + zsum
            return phi.astype(BF16)

        def outer(half, vt, phi):
            for n, (lo, hi) in enumerate(spans):
                y = lax.dot_general(
                    vt[lo:hi], phi[n * LANES:(n + 1) * LANES], NT,
                    preferred_element_type=F32)
                r = lax.broadcasted_iota(jnp.int32, (hi - lo, LANES), 0) + lo
                f = lax.broadcasted_iota(jnp.int32, (1, LANES), 1) + n * LANES
                first = (f & 1) * fb
                for g in range(lo // GR, hi // GR):
                    first = jnp.where(f >= g * 2 * GR, g * GR + (f & 1) * fb, first)
                keep = (r >= first) & (r < first + fb)
                blk = slice(offs[n], offs[n + 1])
                old = jnp.where(i > 0, kv_ref[half, blk, :], 0.0)
                kv_ref[half, blk, :] = jnp.where(keep, old + y, 0.0)

        phi0 = features(0)
        phi1 = features(1)
        vt0 = b_proj(2, 0, rows)
        vt1 = b_proj(2, 1, rows)
        outer(0, vt0, phi0)
        outer(1, vt1, phi1)
        xnb_ref[S - seg:S, :] = _layernorm(xres_ref[S - seg:S, :]).astype(BF16)
        return c

    def out_copy(i):
        r = pl.ds(pl.multiple_of(i * TB, TB), TB)
        return pltpu.make_async_copy(xb_ref.at[r, :], out_hbm.at[r, :], osem.at[i])

    def b_pass2(layer, i, c):
        tu = TB // 2

        def unit_rows(u):
            return pl.ds(pl.multiple_of(i * TB + u * tu, tu), tu)

        def features(u, half):
            a = b_proj(0, half, unit_rows(u))
            phi = []
            for g in range(NG):
                ep, en, sp, sn = exps(a, g)

                def zdot(es, base):
                    terms = []
                    for n, e in enumerate(es):
                        z = z_ref[half, base + 8 * n:base + 8 * n + 8, :]
                        terms.append(e * jnp.concatenate([z] * (tu // LANES), axis=1))
                    return functools.reduce(jnp.add, terms)

                den = zdot(ep, 2 * GR * g) * sn + zdot(en, 2 * GR * g + GR) * sp
                inv = 1.0 / (fold([den], jnp.add) + 1e-6 * (sp * sn))
                ip, im = sn * inv, sp * inv
                phi += [e * ip for e in ep] + [e * im for e in en]
            return jnp.concatenate(phi, axis=0).astype(BF16)

        def mix(half, phi):
            parts = [None] * NG
            for n, (lo, hi) in enumerate(spans):
                y = jnp.dot(
                    kv_ref[half, offs[n]:offs[n + 1], :],
                    phi[n * LANES:(n + 1) * LANES], preferred_element_type=F32)
                for g in range(lo // GR, hi // GR):
                    piece = y[g * GR - lo:(g + 1) * GR - lo]
                    parts[g] = piece if parts[g] is None else parts[g] + piece
            return jnp.concatenate(parts, axis=0)

        def finish(u, cols, o):
            rows = unit_rows(u)
            y = jnp.dot(o, _unpack(bwo_ref[:, cols]), preferred_element_type=F32)
            y = xres_ref[rows, cols] + y
            xres_ref[rows, cols] = y
            xb_ref[rows, cols] = y.astype(BF16)
            return y[:seg]

        phi, ot, o = {}, {}, {}
        for op in P2.split():
            u = int(op[1])
            if op[0] == "f":
                phi[op[1:]] = features(u, int(op[2]))
            elif op[0] == "m":
                ot[op[1:]] = mix(int(op[2]), phi.pop(op[1:]))
                if op[2] == "1":
                    o[u] = jnp.concatenate(
                        [ot.pop(op[1] + "0"), ot.pop(op[1:])], axis=0).T
            else:
                cols = slice(0, PW) if op[0] == "a" else slice(PW, D)
                ot[op] = finish(u, cols, o[u])
        xna_ref[pl.ds(pl.multiple_of(i * TB, TB), seg), :] = _layernorm(
            jnp.concatenate([ot["a0"], ot["b0"]], axis=1))

        @pl.when(layer == 1)
        def _():
            out_copy(i).start()

        return c

    nblk = S // TB

    def layer(n, c):
        layer_a(n)
        pl.when(n == 0)(b_weights)
        lax.fori_loop(0, nblk, b_pass1, 0)
        z_ref[...] = jnp.broadcast_to(
            jnp.sum(z_ref[...], axis=2, keepdims=True), z_ref.shape)
        lax.fori_loop(0, nblk, functools.partial(b_pass2, n), 0)
        return c

    lax.fori_loop(0, 2, layer, 0)
    for i in range(nblk):
        out_copy(i).wait()


@functools.partial(jax.jit, static_argnames=("A_seg_len",))
def pallas_interleave_layers__memory_aug_recurrent_mem_tr__linear_kernel_hedgehog__prompt_kernel(
    A_x: jax.Array,
    A_mem0: jax.Array,
    A_Wq: jax.Array,
    A_Wk: jax.Array,
    A_Wv: jax.Array,
    A_Wo: jax.Array,
    A_seg_len: int,
    B_x: jax.Array,
    B_wqkv: jax.Array,
    B_w_phi: jax.Array,
    B_wo: jax.Array,
):
    del B_x
    _, S, D = A_x.shape
    M = A_mem0.shape[1]
    _, H, dh = A_Wq.shape
    hb = B_w_phi.shape[0]
    seg = int(A_seg_len)
    npair, PW = H // 2, 2 * dh
    assert A_x.shape[0] == 1 and PW == 3 * LANES and 2 * (M + seg) <= LANES
    assert (2 * NPRE - A_UNROLL[True]) * seg >= S and D == 5 * LANES and hb == 32 and S % TB == 0

    def rows_first(w):
        return jnp.transpose(w, (1, 2, 0)).reshape(H * dh, D)

    hbm = pl.BlockSpec(memory_space=pl.ANY)
    out = pl.pallas_call(
        functools.partial(_kernel, seg=seg, dh=dh, hb=hb),
        out_shape=jax.ShapeDtypeStruct((S, D), BF16),
        in_specs=[hbm] * 10,
        out_specs=hbm,
        scratch_shapes=[
            pltpu.VMEM((S, D), BF16),
            pltpu.VMEM((S, D), F32),
            pltpu.VMEM((S, D), F32),
            pltpu.VMEM((S, D), BF16),
            pltpu.VMEM((M, D), F32),
            pltpu.VMEM((NSLOT, 3, PW, D), BF16),
            pltpu.VMEM((npair, D // 2, 3 * PW), U32),
            pltpu.VMEM((H * dh, D), BF16),
            pltpu.VMEM((D, 3 * D), BF16),
            pltpu.VMEM((D, D), BF16),
            pltpu.VMEM((3, D // 2, D), U32),
            pltpu.VMEM((D // 2, D), U32),
            pltpu.VMEM((2, 480, LANES), F32),
            pltpu.VMEM((2, D, LANES), F32),
            pltpu.VMEM((NPRE, 8, D), BF16),
            pltpu.VMEM((NPRE * 4, D), U32),
            pltpu.VMEM((npair, NPRE * 8, 3 * PW), F32),
            pltpu.VMEM((M, D), BF16),
            pltpu.VMEM((D // hb, D // hb, hb), BF16),
            pltpu.VMEM((2 * D // hb, D), F32),
            pltpu.SemaphoreType.DMA((NSLOT, 3)),
            pltpu.SemaphoreType.DMA((7,)),
            pltpu.SemaphoreType.DMA((S // TB,)),
        ],
        compiler_params=pltpu.CompilerParams(
            vmem_limit_bytes=112 * 1024 * 1024, disable_bounds_checks=NOBC),
    )(
        A_x.reshape(S, D),
        A_x.reshape(S // seg, seg // 8, 8, D),
        A_mem0.reshape(M, D),
        rows_first(A_Wq),
        rows_first(A_Wk),
        rows_first(A_Wv),
        A_Wo.reshape(H * dh, D),
        B_wqkv,
        jnp.transpose(B_w_phi, (1, 2, 0)),
        B_wo,
    )
    return out.reshape(1, S, D)
```

```python
import functools

import jax
import jax.numpy as jnp
from jax import lax
import jax.experimental.pallas as pl
import jax.experimental.pallas.tpu as pltpu

F32 = jnp.float32
BF16 = jnp.bfloat16
U32 = jnp.uint32
LOG2E = 1.4426950408889634
NT = (((1,), (1,)), ((), ()))
TN = (((0,), (0,)), ((), ()))
LANES = 128

TB = 512
P2 = "f00 f01 f10 f11 m00 m01 m10 a0 m11 b0 a1 b1"
A_UNROLL = {False: 2, True: 2}
NOBC = True
NSLOT = 3
NPRE = 40


def _layernorm(x):
    m = jnp.mean(x, axis=-1, keepdims=True)
    xc = x - m
    v = jnp.mean(xc * xc, axis=-1, keepdims=True)
    return xc * lax.rsqrt(v + 1e-5)


def _pack(w):
    return pltpu.bitcast(w, U32)


def _unpack(w):
    return pltpu.bitcast(w, BF16)


def _a_schedule(npair, short):
    last = npair - 1

    def kqv(j):
        return [("k", j), ("q", j), ("v", j)]

    def outs(op, lo, hi):
        return [(op, j) for j in range(lo, hi)]

    if short:
        s = kqv(0) + [("s", 0)] + kqv(1)
        s += [("k", 2), ("p", 0), ("q", 2), ("v", 2), ("a", 0), ("b", 0)]
        s += [("s", 1)] + kqv(3) + [("p", 1)]
        for j in range(2, last - 1):
            s += [("s", j), ("k", j + 2), ("a", j - 1), ("q", j + 2), ("v", j + 2)]
            s += [("p", j)]
        s += [("s", last - 1)] + outs("b", 1, 6) + [("a", last - 2), ("p", last - 1)]
        s += [("s", last)] + outs("b", 6, 11) + [("a", last - 1), ("p", last)]
        return s + outs("b", 11, 13) + [("a", last)] + outs("b", 13, npair)
    s = kqv(0)
    for j in range(last):
        s += [("s", j)] + kqv(j + 1) + [("p", j)]
    s += [("s", last)] + outs("b", 0, 7) + [("p", last)] + outs("a", 0, last)
    return s + outs("b", 7, 10) + [("a", last)] + outs("b", 10, npair)


def _kernel(
    x_hbm, x4_hbm, mem_hbm, wq_hbm, wk_hbm, wv_hbm, wo_hbm, bw_hbm, wphi_hbm, bwo_hbm,
    out_hbm,
    xb_ref, xres_ref, xna_ref, xnb_ref, memf_ref,
    stage_ref, wqkv_ref, wo_ref,
    bw_ref, bwo_stage_ref, bwt_ref, bwo_ref,
    kv_ref, z_ref, xsel_ref, xseln_ref, pre_ref, mem_ref, wphi_ref, wrep_ref,
    wsem, sem, osem,
    *, seg, dh, hb,
):
    S, D = xres_ref.shape
    M = mem_ref.shape[0]
    L = M + seg
    nseg = S // seg
    PW = 2 * dh
    npair = wqkv_ref.shape[0]
    fb = D // hb
    GR = 2 * fb
    HR = D // 2
    NG = HR // GR
    NTILE = 2 * HR // LANES
    spans = []
    for i in range(NTILE):
        lo = (i * LANES) // (2 * GR)
        hi = ((i + 1) * LANES - 1) // (2 * GR) + 1
        spans.append((lo * GR, hi * GR))
    offs = [0]
    for lo, hi in spans:
        offs.append(offs[-1] + hi - lo)

    XH = (A_UNROLL[True] + 2) * seg

    def wcopy(j, t):
        rows = pl.ds(pl.multiple_of(j * PW, PW), PW)
        return pltpu.make_async_copy(
            (wq_hbm, wk_hbm, wv_hbm)[t].at[rows, :],
            stage_ref.at[j % NSLOT, t], wsem.at[j % NSLOT, t])

    def start_pair(j):
        for t in range(3):
            wcopy(j, t).start()

    xsel_copy = pltpu.make_async_copy(
        x4_hbm.at[0:NPRE, seg // 8 - 1], xsel_ref, sem.at[0])
    bw_copy = pltpu.make_async_copy(bw_hbm, bw_ref, sem.at[1])
    bwo_copy = pltpu.make_async_copy(bwo_hbm, bwo_stage_ref, sem.at[2])
    xh_copy = pltpu.make_async_copy(
        x_hbm.at[0:XH, :], xb_ref.at[0:XH, :], sem.at[3])
    xt_copy = pltpu.make_async_copy(
        x_hbm.at[XH:S, :], xb_ref.at[XH:S, :], sem.at[3])
    mem_copy = pltpu.make_async_copy(mem_hbm, mem_ref, sem.at[5])
    wphi_copy = pltpu.make_async_copy(wphi_hbm, wphi_ref, sem.at[6])
    wphi_copy.start()
    xsel_copy.start()
    xh_copy.start()
    start_pair(0)

    wphi_copy.wait()
    hh = lax.broadcasted_iota(jnp.int32, (hb, D), 0)
    cc = lax.broadcasted_iota(jnp.int32, (hb, D), 1)

    def spread(i, wcat):
        for d in range(4):
            sel = jnp.where(cc == hh * fb + (4 * i + d), 1.0, 0.0).astype(BF16)
            wcat += jnp.dot(wphi_ref[4 * i + d], sel, preferred_element_type=F32)
        return wcat

    wcat = lax.fori_loop(0, fb // 4, spread, jnp.zeros((fb, D), F32))
    rr = lax.broadcasted_iota(jnp.int32, (GR, fb), 0)
    ff = lax.broadcasted_iota(jnp.int32, (GR, fb), 1)
    twice = jnp.where((rr >> 1) == ff, 1.0, 0.0).astype(BF16)
    wrep_ref[...] = jnp.dot(twice, wcat.astype(BF16), preferred_element_type=F32)

    xsel_copy.wait()
    xsel = xsel_ref[...].astype(F32).reshape(NPRE * 8, D)
    xseln_ref[...] = _pack(_layernorm(xsel).astype(BF16))
    xh_copy.wait()
    xna_ref[0:seg, :] = _layernorm(xb_ref[0:seg, :].astype(F32))

    def load_pair(j, c):
        slot = j % NSLOT
        for t in range(3):
            wcopy(j, t).wait()

        @pl.when(j == 0)
        def _():
            for n in range(1, NSLOT - 1):
                start_pair(n)
            mem_copy.start()

        @pl.when(j + NSLOT - 1 < npair)
        def _():
            start_pair(j + NSLOT - 1)

        part = pl.ds(pl.multiple_of(j * PW, PW), PW)
        pltpu.make_async_copy(
            wo_hbm.at[part, :], wo_ref.at[part, :], sem.at[4]).start()
        for t in range(3):
            cols = slice(t * PW, (t + 1) * PW)
            wqkv_ref[j, :, cols] = _pack(
                stage_ref[slot, t].astype(F32).T.astype(BF16))
            xn = _unpack(xseln_ref[...])
            if t == 0:
                y = lax.dot_general(
                    xn, stage_ref[slot, t], NT, preferred_element_type=F32)
            else:
                y = jnp.dot(xn, _unpack(wqkv_ref[j, :, cols]),
                            preferred_element_type=F32)
            pre_ref[j, :, cols] = y
        return c

    lax.fori_loop(0, npair, load_pair, 0)
    mem_copy.wait()
    pltpu.make_async_copy(wo_hbm, wo_ref, sem.at[4]).wait()
    xt_copy.start()
    bw_copy.start()
    bwo_copy.start()

    def b_weights():
        bw_copy.wait()
        bwo_copy.wait()
        rr = lax.broadcasted_iota(jnp.int32, (GR, LANES), 0)
        cc = lax.broadcasted_iota(jnp.int32, (GR, LANES), 1) - (rr & 1) * fb
        for t in range(2):
            parts = [None] * (D // GR)
            for n in range(D // LANES):
                lo = (n * LANES) // GR
                hi = ((n + 1) * LANES - 1) // GR + 1
                col = cc + n * LANES
                lhs = jnp.concatenate([
                    jnp.where((col >= g * GR) & (col < g * GR + fb),
                              wrep_ref[:, n * LANES:(n + 1) * LANES], 0.0)
                    for g in range(lo, hi)
                ], axis=0)
                y = lax.dot_general(
                    lhs, bw_ref[:, t * D + n * LANES:t * D + (n + 1) * LANES], NT,
                    preferred_element_type=F32)
                for g in range(lo, hi):
                    piece = y[(g - lo) * GR:(g - lo + 1) * GR]
                    parts[g] = piece if parts[g] is None else parts[g] + piece
            w = jnp.concatenate(parts, axis=0) * LOG2E
            bwt_ref[t] = _pack(w.astype(BF16))
        bwt_ref[2] = _pack(bw_ref[:, 2 * D:3 * D].T)
        bwo_ref[...] = _pack(bwo_stage_ref[...])

    def a_step(short, s, mem, chained_in):
        rows = pl.ds(pl.multiple_of(s * seg, seg), seg)
        row = lax.broadcasted_iota(jnp.int32, (L, LANES), 0)
        lane = lax.broadcasted_iota(jnp.int32, (L, LANES), 1)
        is_a = lane < L
        col = jnp.where(is_a, lane, lane - L)
        inside = col < L
        vis = ((row < M) | (row >= col)) & inside
        vis_a = vis & is_a
        vis_b = vis & jnp.logical_not(is_a)
        fill_a = jnp.where(is_a, -1e9 * LOG2E, -jnp.inf)
        fill_b = jnp.where(inside & jnp.logical_not(is_a), -1e9 * LOG2E, -jnp.inf)
        low = lane < dh - LANES
        scale = dh ** -0.5 * LOG2E

        def part(j, t, lo, hi):
            n = seg - 8 if short else seg
            x = xna_ref[pl.ds(pl.multiple_of(s * seg, seg), n), lo:hi]
            h = jnp.concatenate([mem[:, lo:hi], x], axis=0)
            w = _unpack(wqkv_ref[j, lo // 2:hi // 2, t * PW:(t + 1) * PW])
            return jnp.dot(h.astype(BF16) if short else h, w,
                           preferred_element_type=F32)

        def proj(j, t, head=None):
            if head is None:
                y = part(j, t, 0, D)
            else:
                y = part(j, t, PW, D) + head
            if short:
                tail = pl.ds(pl.multiple_of(s * 8, 8), 8)
                y = jnp.concatenate(
                    [y, pre_ref[j, tail, t * PW:(t + 1) * PW]], axis=0)
            return y

        def blockdiag(a):
            zero = jnp.zeros((L, LANES), F32)
            mid = a[:, LANES:2 * LANES]
            top = jnp.concatenate(
                [a[:, :LANES], jnp.where(low, mid, 0.0), zero], axis=1)
            bot = jnp.concatenate(
                [zero, jnp.where(low, 0.0, mid), a[:, 2 * LANES:]], axis=1)
            pad = jnp.zeros((LANES - 2 * L, PW), F32)
            return jnp.concatenate([top, bot, pad], axis=0).astype(BF16)

        def probs(q, k):
            sc = lax.dot_general(q, blockdiag(k), NT, preferred_element_type=F32)
            sc = sc * scale
            sa = jnp.where(vis_a, sc, fill_a)
            sb = jnp.where(vis_b, sc, fill_b)
            ma = jnp.max(sa, axis=1, keepdims=True)
            mb = jnp.max(sb, axis=1, keepdims=True)
            e = jnp.exp2(jnp.where(is_a, sa - ma, sb - mb))
            la = jnp.sum(jnp.where(is_a, e, 0.0), axis=1, keepdims=True)
            lb = jnp.sum(jnp.where(is_a, 0.0, e), axis=1, keepdims=True)
            return e * (1.0 / jnp.where(is_a, la, lb))

        prv = pl.ds(pl.multiple_of(jnp.maximum(s - 1, 0) * seg, seg), seg)
        nxt = pl.ds(pl.multiple_of(jnp.minimum(s + 1, nseg - 1) * seg, seg), seg)
        if short:
            far = jnp.where(s < A_UNROLL[True], s, nseg - 1 + A_UNROLL[True] - s)
            far = jnp.where(far < NPRE, s, far)
            far = pl.ds(pl.multiple_of(far * seg, seg), seg)
            xres_ref[far, :] = xb_ref[far, :].astype(F32)
        xnb_ref[prv, :] = _layernorm(xres_ref[prv, :]).astype(BF16)
        xin_ref = xb_ref if short else xres_ref
        xn_next = _layernorm(xin_ref[nxt, :].astype(F32))

        q, k, v, p, o = {}, {}, {}, {}, {}
        acc = [None, None]
        head_k = head_q = None
        if chained_in:
            head_k, head_q = part(0, 1, 0, PW), part(0, 0, 0, PW)
        for op, j in _a_schedule(npair, short):
            if op == "q":
                q[j] = proj(j, 0, head_q if j == 0 else None)
            elif op == "k":
                k[j] = proj(j, 1, head_k if j == 0 else None)
            elif op == "v":
                v[j] = proj(j, 2)
            elif op == "s":
                p[j] = probs(q.pop(j), k.pop(j))
            elif op == "p":
                o[j] = jnp.dot(
                    p.pop(j), blockdiag(v.pop(j)), preferred_element_type=F32)
                if j == npair - 1:
                    xna_ref[nxt, :] = xn_next
            else:
                n = "ab".index(op)
                cols = (slice(0, PW), slice(PW, D))[n]
                y = jnp.dot(o[j], wo_ref[j * PW:(j + 1) * PW, cols],
                            preferred_element_type=F32)
                acc[n] = y if acc[n] is None else acc[n] + y
        acc = jnp.concatenate(acc, axis=1)
        xres_ref[rows, :] = xin_ref[rows, :].astype(F32) + acc[M:]
        return acc[:M]

    def a_steps(short, i, c):
        if short:
            pl.when(i == 1)(xt_copy.wait)
        mem = memf_ref[...]
        n = A_UNROLL[short]
        for u in range(n):
            mem = a_step(short, i * n + u, mem, u > 0)
        memf_ref[...] = mem
        return c

    def layer_a(n):
        memf_ref[...] = mem_ref[...].astype(F32)
        lax.fori_loop(0, jnp.where(n == 0, NPRE // A_UNROLL[True], 0),
                      functools.partial(a_steps, True), 0)
        lax.fori_loop(jnp.where(n == 0, NPRE // A_UNROLL[False], 0),
                      nseg // A_UNROLL[False],
                      functools.partial(a_steps, False), 0)

    def b_proj(t, half, rows):
        w = _unpack(bwt_ref[t, half * (HR // 2):(half + 1) * (HR // 2), :])
        return lax.dot_general(
            w, xnb_ref[rows, :], NT, preferred_element_type=F32)

    def fold(vals, op):
        r = functools.reduce(op, vals)
        r = op(r, pltpu.roll(r, 4, 0))
        return op(r, pltpu.roll(r, 2, 0))

    def exps(a, g):
        slabs = [a[g * GR + 8 * i:g * GR + 8 * i + 8] for i in range(GR // 8)]
        mx = fold(slabs, jnp.maximum)
        mn = fold(slabs, jnp.minimum)
        ep = [jnp.exp2(u - mx) for u in slabs]
        en = [jnp.exp2(mn - u) for u in slabs]
        return ep, en, fold(ep, jnp.add), fold(en, jnp.add)

    def b_pass1(i, c):
        rows = pl.ds(pl.multiple_of(i * TB, TB), TB)

        def features(half):
            a = b_proj(1, half, rows)
            phi = []
            for g in range(NG):
                ep, en, sp, sn = exps(a, g)
                inv = 1.0 / (sp * sn)
                ip, im = sn * inv, sp * inv
                phi += [e * ip for e in ep] + [e * im for e in en]
            phi = jnp.concatenate(phi, axis=0)
            zsum = phi[:, :LANES]
            for n in range(1, TB // LANES):
                zsum = zsum + phi[:, n * LANES:(n + 1) * LANES]
            return phi.astype(BF16), zsum

        def outer(half, vt, phi):
            for n, (lo, hi) in enumerate(spans):
                y = lax.dot_general(
                    vt[lo:hi], phi[n * LANES:(n + 1) * LANES], NT,
                    preferred_element_type=F32)
                r = lax.broadcasted_iota(jnp.int32, (hi - lo, LANES), 0) + lo
                f = lax.broadcasted_iota(jnp.int32, (1, LANES), 1) + n * LANES
                first = (f & 1) * fb
                for g in range(lo // GR, hi // GR):
                    first = jnp.where(f >= g * 2 * GR, g * GR + (f & 1) * fb, first)
                keep = (r >= first) & (r < first + fb)
                blk = slice(offs[n], offs[n + 1])
                old = jnp.where(i > 0, kv_ref[half, blk, :], 0.0)
                kv_ref[half, blk, :] = jnp.where(keep, old + y, 0.0)

        phi0, z0 = features(0)
        phi1, z1 = features(1)
        for half, z in enumerate((z0, z1)):
            z_ref[half] = jnp.where(i > 0, z_ref[half], 0.0) + z
        vt0 = b_proj(2, 0, rows)
        vt1 = b_proj(2, 1, rows)
        outer(0, vt0, phi0)
        outer(1, vt1, phi1)
        xnb_ref[S - seg:S, :] = _layernorm(xres_ref[S - seg:S, :]).astype(BF16)
        return c

    def b_pass2(i, c):
        tu = TB // 2

        def unit_rows(u):
            return pl.ds(pl.multiple_of(i * TB + u * tu, tu), tu)

        def features(u, half):
            a = b_proj(0, half, unit_rows(u))
            phi = []
            for g in range(NG):
                ep, en, sp, sn = exps(a, g)

                def zdot(es, base):
                    terms = []
                    for n, e in enumerate(es):
                        z = z_ref[half, base + 8 * n:base + 8 * n + 8, :]
                        terms.append(e * jnp.concatenate([z] * (tu // LANES), axis=1))
                    return functools.reduce(jnp.add, terms)

                den = zdot(ep, 2 * GR * g) * sn + zdot(en, 2 * GR * g + GR) * sp
                inv = 1.0 / (fold([den], jnp.add) + 1e-6 * (sp * sn))
                ip, im = sn * inv, sp * inv
                phi += [e * ip for e in ep] + [e * im for e in en]
            return jnp.concatenate(phi, axis=0).astype(BF16)

        def mix(half, phi):
            parts = [None] * NG
            for n, (lo, hi) in enumerate(spans):
                y = jnp.dot(
                    kv_ref[half, offs[n]:offs[n + 1], :],
                    phi[n * LANES:(n + 1) * LANES], preferred_element_type=F32)
                for g in range(lo // GR, hi // GR):
                    piece = y[g * GR - lo:(g + 1) * GR - lo]
                    parts[g] = piece if parts[g] is None else parts[g] + piece
            return jnp.concatenate(parts, axis=0)

        def finish(u, cols, o):
            rows = unit_rows(u)
            y = jnp.dot(o, _unpack(bwo_ref[:, cols]), preferred_element_type=F32)
            y = xres_ref[rows, cols] + y
            xres_ref[rows, cols] = y
            xb_ref[rows, cols] = y.astype(BF16)
            return y[:seg]

        phi, ot, o = {}, {}, {}
        for op in P2.split():
            u = int(op[1])
            if op[0] == "f":
                phi[op[1:]] = features(u, int(op[2]))
            elif op[0] == "m":
                ot[op[1:]] = mix(int(op[2]), phi.pop(op[1:]))
                if op[2] == "1":
                    o[u] = jnp.concatenate(
                        [ot.pop(op[1] + "0"), ot.pop(op[1:])], axis=0).T
            else:
                cols = slice(0, PW) if op[0] == "a" else slice(PW, D)
                ot[op] = finish(u, cols, o[u])
                if op[0] == "b":
                    pltpu.make_async_copy(
                        xb_ref.at[unit_rows(u), :], out_hbm.at[unit_rows(u), :],
                        osem).start()
        xna_ref[pl.ds(pl.multiple_of(i * TB, TB), seg), :] = _layernorm(
            jnp.concatenate([ot["a0"], ot["b0"]], axis=1))
        return c

    nblk = S // TB
    out_copy = pltpu.make_async_copy(xb_ref, out_hbm, osem)

    def layer(n, c):
        layer_a(n)
        pl.when(n == 0)(b_weights)
        lax.fori_loop(0, nblk, b_pass1, 0)
        z_ref[...] = jnp.broadcast_to(
            jnp.sum(z_ref[...], axis=2, keepdims=True), z_ref.shape)
        pl.when(n == 1)(out_copy.wait)
        lax.fori_loop(0, nblk, b_pass2, 0)
        return c

    lax.fori_loop(0, 2, layer, 0)
    out_copy.wait()


@functools.partial(jax.jit, static_argnames=("A_seg_len",))
def pallas_interleave_layers__memory_aug_recurrent_mem_tr__linear_kernel_hedgehog__prompt_kernel(
    A_x: jax.Array,
    A_mem0: jax.Array,
    A_Wq: jax.Array,
    A_Wk: jax.Array,
    A_Wv: jax.Array,
    A_Wo: jax.Array,
    A_seg_len: int,
    B_x: jax.Array,
    B_wqkv: jax.Array,
    B_w_phi: jax.Array,
    B_wo: jax.Array,
):
    del B_x
    _, S, D = A_x.shape
    M = A_mem0.shape[1]
    _, H, dh = A_Wq.shape
    hb = B_w_phi.shape[0]
    seg = int(A_seg_len)
    npair, PW = H // 2, 2 * dh
    assert A_x.shape[0] == 1 and PW == 3 * LANES and 2 * (M + seg) <= LANES
    assert (2 * NPRE - A_UNROLL[True]) * seg >= S and D == 5 * LANES and hb == 32 and S % TB == 0

    def rows_first(w):
        return jnp.transpose(w, (1, 2, 0)).reshape(H * dh, D)

    hbm = pl.BlockSpec(memory_space=pl.ANY)
    out = pl.pallas_call(
        functools.partial(_kernel, seg=seg, dh=dh, hb=hb),
        out_shape=jax.ShapeDtypeStruct((S, D), BF16),
        in_specs=[hbm] * 10,
        out_specs=hbm,
        scratch_shapes=[
            pltpu.VMEM((S, D), BF16),
            pltpu.VMEM((S, D), F32),
            pltpu.VMEM((S, D), F32),
            pltpu.VMEM((S, D), BF16),
            pltpu.VMEM((M, D), F32),
            pltpu.VMEM((NSLOT, 3, PW, D), BF16),
            pltpu.VMEM((npair, D // 2, 3 * PW), U32),
            pltpu.VMEM((H * dh, D), BF16),
            pltpu.VMEM((D, 3 * D), BF16),
            pltpu.VMEM((D, D), BF16),
            pltpu.VMEM((3, D // 2, D), U32),
            pltpu.VMEM((D // 2, D), U32),
            pltpu.VMEM((2, 480, LANES), F32),
            pltpu.VMEM((2, D, LANES), F32),
            pltpu.VMEM((NPRE, 8, D), BF16),
            pltpu.VMEM((NPRE * 4, D), U32),
            pltpu.VMEM((npair, NPRE * 8, 3 * PW), F32),
            pltpu.VMEM((M, D), BF16),
            pltpu.VMEM((D // hb, D // hb, hb), BF16),
            pltpu.VMEM((2 * D // hb, D), F32),
            pltpu.SemaphoreType.DMA((NSLOT, 3)),
            pltpu.SemaphoreType.DMA((7,)),
            pltpu.SemaphoreType.DMA,
        ],
        compiler_params=pltpu.CompilerParams(
            vmem_limit_bytes=112 * 1024 * 1024, disable_bounds_checks=NOBC),
    )(
        A_x.reshape(S, D),
        A_x.reshape(S // seg, seg // 8, 8, D),
        A_mem0.reshape(M, D),
        rows_first(A_Wq),
        rows_first(A_Wk),
        rows_first(A_Wv),
        A_Wo.reshape(H * dh, D),
        B_wqkv,
        jnp.transpose(B_w_phi, (1, 2, 0)),
        B_wo,
    )
    return out.reshape(1, S, D)
```

```python
import functools

import jax
import jax.numpy as jnp
from jax import lax
import jax.experimental.pallas as pl
import jax.experimental.pallas.tpu as pltpu

F32 = jnp.float32
BF16 = jnp.bfloat16
U32 = jnp.uint32
LOG2E = 1.4426950408889634
NT = (((1,), (1,)), ((), ()))
TN = (((0,), (0,)), ((), ()))
LANES = 128

TB = 512
P2 = "f00 f01 f10 f11 m00 m01 m10 a0 m11 b0 a1 b1"
A_UNROLL = {False: 2, True: 2}
NOBC = True
SCHED = {True: ['k0 q0 v0 s0 k1 q1 v1 k2 p0 v2 b0 s1 q2 k3 v3 q3 p1 a0 s2 k4 a1 q4 v4 p2 s3 k5 a2 q5 v5 p3 s4 k6 v6 a3 q6 p4 s5 k7 a4 q7 v7 p5 s6 k8 a5 q8 v8 p6 s7 v9 k9 a6 q9 p7 s8 q10 k10 a7 v10 p8 s9 k11 a8 q11 v11 p9 s10 k12 a9 q12 v12 p10 s11 k13 q13 a10 v13 p11 s12 k14 a11 q14 v14 p12 s13 k15 a12 v15 q15 p13 s14 b2 s15 b8 b4 b1 b5 b3 p14 a13 b6 b7 b10 b9 a14 p15 b11 b12 a15 b15 b13 b14', 'k0 q0 v0 s0 k1 q1 v1 k2 p0 v2 s1 q2 k3 b0 v3 q3 p1 a0 s2 k4 a1 q4 v4 p2 s3 k5 a2 q5 v5 p3 s4 v6 k6 a3 q6 p4 s5 k7 a4 q7 v7 p5 s6 k8 a5 q8 v8 p6 s7 v9 k9 a6 q9 p7 s8 q10 k10 a7 v10 p8 s9 k11 q11 a8 v11 p9 s10 v12 k12 a9 q12 p10 s11 k13 q13 a10 v13 p11 s12 k14 a11 q14 v14 p12 s13 k15 a12 v15 q15 p13 s14 b2 s15 b4 b1 b8 b5 b3 p14 b6 b10 b7 a13 b9 a14 p15 b12 b11 b13 a15 b14 b15'], False: ['k0 q0 v0 s0 k1 q1 v1 p0 s1 k2 q2 v2 p1 s2 k3 q3 v3 p2 s3 k4 q4 v4 p3 s4 k5 q5 v5 p4 s5 o0 k6 q6 v6 p5 s6 k7 q7 v7 p6 s7 k8 q8 o1 v8 p7 s8 k9 q9 o2 v9 p8 s9 k10 q10 o3 v10 p9 s10 k11 q11 o4 v11 p10 s11 k12 q12 o5 v12 p11 s12 k13 q13 o6 v13 p12 s13 k14 q14 o7 v14 p13 v15 s14 k15 q15 o8 p14 s15 o9 o10 o11 p15 o12 a13 a14 a15 b13 b14 b15', 'k0 q0 v0 s0 k1 q1 v1 p0 s1 k2 q2 v2 p1 s2 k3 q3 v3 p2 s3 k4 q4 v4 p3 s4 k5 q5 o0 v5 p4 s5 k6 q6 o1 v6 p5 s6 k7 q7 o2 v7 p6 s7 k8 q8 o3 v8 p7 s8 q9 k9 o4 v9 p8 s9 v10 k10 q10 o5 p9 s10 k11 q11 o6 v11 p10 s11 k12 q12 o7 v12 p11 s12 k13 v13 q13 o8 q14 p12 s13 k14 o9 v14 p13 s14 k15 q15 o10 v15 p14 s15 o11 o13 o12 p15 o14 o15']}
NSCORE = {False: ['1111111111111000', '1211111111111100'], True: ['0111111111111000', '0111101111111011']}
MASKED = -1e9 * LOG2E
NSLOT = 3
NPRE = 40


def _layernorm(x):
    m = jnp.mean(x, axis=-1, keepdims=True)
    xc = x - m
    v = jnp.mean(xc * xc, axis=-1, keepdims=True)
    return xc * lax.rsqrt(v + 1e-5)


def _pack(w):
    return pltpu.bitcast(w, U32)


def _unpack(w):
    return pltpu.bitcast(w, BF16)


def _kernel(
    x_hbm, x4_hbm, mem_hbm, wq_hbm, wk_hbm, wv_hbm, wo_hbm, bw_hbm, wphi_hbm, bwo_hbm,
    out_hbm,
    xb_ref, xres_ref, xna_ref, xnb_ref, memf_ref,
    stage_ref, wqkv_ref, wop_ref,
    bw_ref, bwo_stage_ref, bwt_ref, bwo_ref,
    kv_ref, z_ref, xsel_ref, xseln_ref, pre_ref, mem_ref, wphi_ref, wrep_ref, row_ref,
    wsem, sem, osem,
    *, seg, dh, hb,
):
    S, D = xres_ref.shape
    M = mem_ref.shape[0]
    L = M + seg
    nseg = S // seg
    PW = 2 * dh
    npair = wqkv_ref.shape[0]
    HL = LANES // 2
    mixed = [h * dh + r for r in range(0, dh, HL) for h in range(2)]
    fb = D // hb
    GR = 2 * fb
    HR = D // 2
    NG = HR // GR
    NTILE = 2 * HR // LANES
    spans = []
    for i in range(NTILE):
        lo = (i * LANES) // (2 * GR)
        hi = ((i + 1) * LANES - 1) // (2 * GR) + 1
        spans.append((lo * GR, hi * GR))
    offs = [0]
    for lo, hi in spans:
        offs.append(offs[-1] + hi - lo)

    XH = (A_UNROLL[True] + 2) * seg

    def wcopy(j, t):
        rows = pl.ds(pl.multiple_of(j * PW, PW), PW)
        return pltpu.make_async_copy(
            (wq_hbm, wk_hbm, wv_hbm)[t].at[rows, :],
            stage_ref.at[j % NSLOT, t], wsem.at[j % NSLOT, t])

    def start_pair(j):
        for t in range(3):
            wcopy(j, t).start()

    xsel_copy = pltpu.make_async_copy(
        x4_hbm.at[0:NPRE, seg // 8 - 1], xsel_ref, sem.at[0])
    bw_copy = pltpu.make_async_copy(bw_hbm, bw_ref, sem.at[1])
    bwo_copy = pltpu.make_async_copy(bwo_hbm, bwo_stage_ref, sem.at[2])
    xh_copy = pltpu.make_async_copy(
        x_hbm.at[0:XH, :], xb_ref.at[0:XH, :], sem.at[3])
    xt_copy = pltpu.make_async_copy(
        x_hbm.at[XH:S, :], xb_ref.at[XH:S, :], sem.at[3])
    mem_copy = pltpu.make_async_copy(mem_hbm, mem_ref, sem.at[5])
    wphi_copy = pltpu.make_async_copy(wphi_hbm, wphi_ref, sem.at[6])
    wphi_copy.start()
    xsel_copy.start()
    xh_copy.start()
    start_pair(0)

    wphi_copy.wait()
    hh = lax.broadcasted_iota(jnp.int32, (hb, D), 0)
    cc = lax.broadcasted_iota(jnp.int32, (hb, D), 1)

    def spread(i, wcat):
        for d in range(4):
            sel = jnp.where(cc == hh * fb + (4 * i + d), 1.0, 0.0).astype(BF16)
            wcat += jnp.dot(wphi_ref[4 * i + d], sel, preferred_element_type=F32)
        return wcat

    wcat = lax.fori_loop(0, fb // 4, spread, jnp.zeros((fb, D), F32))
    rr = lax.broadcasted_iota(jnp.int32, (GR, fb), 0)
    ff = lax.broadcasted_iota(jnp.int32, (GR, fb), 1)
    twice = jnp.where((rr >> 1) == ff, 1.0, 0.0).astype(BF16)
    wrep_ref[...] = jnp.dot(twice, wcat.astype(BF16), preferred_element_type=F32)

    xsel_copy.wait()
    xsel = xsel_ref[...].astype(F32).reshape(NPRE * 8, D)
    xseln_ref[...] = _pack(_layernorm(xsel).astype(BF16))
    xh_copy.wait()
    xna_ref[0:seg, :] = _layernorm(xb_ref[0:seg, :].astype(F32))

    def load_pair(j, c):
        slot = j % NSLOT
        for t in range(3):
            wcopy(j, t).wait()

        @pl.when(j == 0)
        def _():
            for n in range(1, NSLOT - 1):
                start_pair(n)
            mem_copy.start()

        @pl.when(j + NSLOT - 1 < npair)
        def _():
            start_pair(j + NSLOT - 1)

        part = pl.ds(pl.multiple_of(j * dh, dh), dh)
        pltpu.make_async_copy(
            wo_hbm.bitcast(U32).at[part, :], wop_ref.at[part, :], sem.at[4]).start()
        for t in range(3):
            cols = slice(t * PW, (t + 1) * PW)
            w = jnp.concatenate(
                [stage_ref[slot, t, r:r + HL, :]
                 for r in (mixed if t == 2 else range(0, PW, HL))], axis=0)
            wqkv_ref[j, :, cols] = _pack(w.astype(F32).T.astype(BF16))
            xn = _unpack(xseln_ref[...])
            if t == 0:
                y = lax.dot_general(
                    xn, stage_ref[slot, t], NT, preferred_element_type=F32)
            else:
                y = jnp.dot(xn, _unpack(wqkv_ref[j, :, cols]),
                            preferred_element_type=F32)
            pre_ref[j, :, cols] = y
        return c

    lax.fori_loop(0, npair, load_pair, 0)
    mem_copy.wait()
    pltpu.make_async_copy(wop_ref, wop_ref, sem.at[4]).wait()
    xt_copy.start()
    bw_copy.start()
    bwo_copy.start()

    def b_weights():
        bw_copy.wait()
        bwo_copy.wait()
        rr = lax.broadcasted_iota(jnp.int32, (GR, LANES), 0)
        cc = lax.broadcasted_iota(jnp.int32, (GR, LANES), 1) - (rr & 1) * fb
        for t in range(2):
            parts = [None] * (D // GR)
            for n in range(D // LANES):
                lo = (n * LANES) // GR
                hi = ((n + 1) * LANES - 1) // GR + 1
                col = cc + n * LANES
                lhs = jnp.concatenate([
                    jnp.where((col >= g * GR) & (col < g * GR + fb),
                              wrep_ref[:, n * LANES:(n + 1) * LANES], 0.0)
                    for g in range(lo, hi)
                ], axis=0)
                y = lax.dot_general(
                    lhs, bw_ref[:, t * D + n * LANES:t * D + (n + 1) * LANES], NT,
                    preferred_element_type=F32)
                for g in range(lo, hi):
                    piece = y[(g - lo) * GR:(g - lo + 1) * GR]
                    parts[g] = piece if parts[g] is None else parts[g] + piece
            w = jnp.concatenate(parts, axis=0) * LOG2E
            bwt_ref[t] = _pack(w.astype(BF16))
        bwt_ref[2] = _pack(bw_ref[:, 2 * D:3 * D].T)
        bwo_ref[...] = _pack(bwo_stage_ref[...])

    def a_step(short, s, mem, u):
        rows = pl.ds(pl.multiple_of(s * seg, seg), seg)
        sub = lax.broadcasted_iota(jnp.int32, (8, LANES), 0)
        lane = lax.broadcasted_iota(jnp.int32, (8, LANES), 1)
        is_a = lane < L
        col = jnp.where(is_a, lane, lane - L)
        low = lane < HL
        lows = lax.broadcasted_iota(jnp.int32, (L, LANES), 1) < HL
        scale = jnp.where(
            lax.broadcasted_iota(jnp.int32, (L, PW), 1) + s >= 0,
            dh ** -0.5 * LOG2E, 0.0)
        nscore = [min(int(n), 2) for n in NSCORE[short][u]]
        nmix = [(int(n) + 1) // 2 for n in NSCORE[short][u]]

        def part(j, t, lo, hi):
            n = seg - 8 if short else seg
            x = xna_ref[pl.ds(pl.multiple_of(s * seg, seg), n), lo:hi]
            h = jnp.concatenate([mem[:, lo:hi], x], axis=0)
            w = _unpack(wqkv_ref[j, lo // 2:hi // 2, t * PW:(t + 1) * PW])
            return jnp.dot(h.astype(BF16) if short else h, w,
                           preferred_element_type=F32)

        def proj(j, t, head=None):
            if head is None:
                y = part(j, t, 0, D)
            else:
                y = part(j, t, PW, D) + head
            if short:
                tail = pl.ds(pl.multiple_of(s * 8, 8), 8)
                y = jnp.concatenate(
                    [y, pre_ref[j, tail, t * PW:(t + 1) * PW]], axis=0)
            if t == 0:
                return y * scale
            for b in range(nscore[j] if t == 1 else nmix[j]):
                n = M + 8 * b + 8
                row_ref[j, 2 * b + t - 1, 0:n, :] = y[:n]
            return y

        def spread_row(j, t, r, c):
            return jnp.broadcast_to(
                row_ref[j, t - 1, r:r + 1, c * LANES:(c + 1) * LANES], (8, LANES))

        def stack(top, bot):
            pad = jnp.zeros((LANES - 2 * L, PW), F32)
            return jnp.concatenate([top, bot, pad], axis=0).astype(BF16)

        def keys(k):
            zero = jnp.zeros((L, LANES), F32)
            mid = k[:, LANES:2 * LANES]
            return stack(
                jnp.concatenate(
                    [k[:, :LANES], jnp.where(lows, mid, 0.0), zero], axis=1),
                jnp.concatenate(
                    [zero, jnp.where(lows, 0.0, mid), k[:, 2 * LANES:]], axis=1))

        def values(v):
            first = jnp.concatenate([lows] * 3, axis=1)
            return stack(jnp.where(first, v, 0.0), jnp.where(first, 0.0, v))

        def softmax(sc, row):
            inside = col < L
            vis = inside if row < M else col <= sub + row
            sc = jnp.where(vis, sc, jnp.where(inside, MASKED, -jnp.inf))
            ma = jnp.max(jnp.where(is_a, sc, -jnp.inf), axis=1, keepdims=True)
            mb = jnp.max(jnp.where(is_a, -jnp.inf, sc), axis=1, keepdims=True)
            e = jnp.exp2(sc - jnp.where(is_a, ma, mb))
            la = jnp.sum(jnp.where(is_a, e, 0.0), axis=1, keepdims=True)
            lb = jnp.sum(jnp.where(is_a, 0.0, e), axis=1, keepdims=True)
            return e * (1.0 / jnp.where(is_a, la, lb))

        def vpu_scores(j, q, row):
            q = q[row:row + 8]
            mid = q[:, LANES:2 * LANES]
            qa, qb = jnp.where(low, mid, 0.0), jnp.where(low, 0.0, mid)
            out = []
            for r in range(row + 8):
                k0, k1, k2 = (spread_row(j, (row - M) // 4 + 1, r, c) for c in range(3))
                out.append((
                    jnp.sum(q[:, :LANES] * k0 + qa * k1, axis=1, keepdims=True),
                    jnp.sum(q[:, 2 * LANES:] * k2 + qb * k1, axis=1, keepdims=True)))
            return out

        def to_lanes(scores):
            out = None
            for h in range(2):
                vals = [jnp.broadcast_to(x[h], (8, LANES)) for x in scores]
                for bit in (1, 2, 4):
                    vals = [jnp.where((lane & bit) == 0, vals[i], vals[i + 1])
                            for i in range(0, len(vals), 2)]
                for g, x in enumerate(vals):
                    out = x if out is None else jnp.where(
                        lane < h * L + 8 * g, out, x)
            return out

        def vpu_attend(j, scores):
            row = len(scores) - 8
            sc = [jnp.where(low, a, b) for a, b in scores]
            sc = [x if r <= row else jnp.where(sub >= r - row, x, MASKED)
                  for r, x in enumerate(sc)]
            top = functools.reduce(jnp.maximum, sc)
            acc = None
            for r, x in enumerate(sc):
                e = jnp.exp2(x - top)
                t = [e * spread_row(j, (row - M) // 4 + 2, r, c) for c in range(3)] + [e]
                acc = t if acc is None else [u + w for u, w in zip(acc, t)]
            inv = 1.0 / acc[3]
            return jnp.concatenate([x * inv for x in acc[:3]], axis=1)

        def probs(j, q, k):
            far = M + 8 * nscore[j]
            sc = lax.dot_general(
                jnp.concatenate([q[:M], q[far:]], axis=0), keys(k), NT,
                preferred_element_type=F32)
            p = {0: softmax(sc[:M], 0)}
            for row in range(far, L, 8):
                p[row] = softmax(sc[row - far + M:row - far + M + 8], row)
            first = [vpu_scores(j, q, M + 8 * b) for b in range(nmix[j])]
            for row in range(M + 8 * nmix[j], far, 8):
                p[row] = softmax(to_lanes(vpu_scores(j, q, row)), row)
            return jnp.concatenate([p[row] for row in sorted(p)], axis=0), first

        prv = pl.ds(pl.multiple_of(jnp.maximum(s - 1, 0) * seg, seg), seg)
        nxt = pl.ds(pl.multiple_of(jnp.minimum(s + 1, nseg - 1) * seg, seg), seg)
        if short:
            far = jnp.where(s < A_UNROLL[True], s, nseg - 1 + A_UNROLL[True] - s)
            far = jnp.where(far < NPRE, s, far)
            far = pl.ds(pl.multiple_of(far * seg, seg), seg)
            xres_ref[far, :] = xb_ref[far, :].astype(F32)
        xnb_ref[prv, :] = _layernorm(xres_ref[prv, :]).astype(BF16)
        xin_ref = xb_ref if short else xres_ref
        xn_next = _layernorm(xin_ref[nxt, :].astype(F32))

        q, k, v, p, o = {}, {}, {}, {}, {}
        acc, whole = [None, None], None
        head_k = head_q = None
        if u > 0:
            head_k, head_q = part(0, 1, 0, PW), part(0, 0, 0, PW)
        for op, j in ((t[0], int(t[1:])) for t in SCHED[short][u].split()):
            if op == "q":
                q[j] = proj(j, 0, head_q if j == 0 else None)
            elif op == "k":
                k[j] = proj(j, 1, head_k if j == 0 else None)
            elif op == "v":
                v[j] = proj(j, 2)
            elif op == "s":
                p[j] = probs(j, q.pop(j), k.pop(j))
            elif op == "p":
                y = jnp.dot(
                    p[j][0], values(v.pop(j)), preferred_element_type=F32)
                o[j] = jnp.concatenate(
                    [y[:M]] + [vpu_attend(j, x) for x in p[j][1]] + [y[M:]], axis=0)
                if j == npair - 1:
                    xna_ref[nxt, :] = xn_next
            else:
                lo, hi = {"a": (0, PW), "b": (PW, D), "o": (0, D)}[op]
                w = _unpack(jnp.concatenate(
                    [wop_ref[(j * PW + r) // 2:(j * PW + r + HL) // 2, lo:hi]
                     for r in mixed], axis=0))
                y = jnp.dot(o[j], w, preferred_element_type=F32)
                if op == "o":
                    whole = y if whole is None else whole + y
                else:
                    n = "ab".index(op)
                    if acc[n] is None and whole is not None:
                        acc[n] = whole[:, lo:hi]
                    acc[n] = y if acc[n] is None else acc[n] + y
        acc = whole if acc[0] is None else jnp.concatenate(acc, axis=1)
        xres_ref[rows, :] = xin_ref[rows, :].astype(F32) + acc[M:]
        return acc[:M]

    def a_steps(short, i, c):
        if short:
            pl.when(i == 1)(xt_copy.wait)
        mem = memf_ref[...]
        n = A_UNROLL[short]
        for u in range(n):
            mem = a_step(short, i * n + u, mem, u)
        memf_ref[...] = mem
        return c

    def layer_a(n):
        memf_ref[...] = mem_ref[...].astype(F32)
        lax.fori_loop(0, jnp.where(n == 0, NPRE // A_UNROLL[True], 0),
                      functools.partial(a_steps, True), 0)
        lax.fori_loop(jnp.where(n == 0, NPRE // A_UNROLL[False], 0),
                      nseg // A_UNROLL[False],
                      functools.partial(a_steps, False), 0)

    def b_proj(t, half, rows):
        w = _unpack(bwt_ref[t, half * (HR // 2):(half + 1) * (HR // 2), :])
        return lax.dot_general(
            w, xnb_ref[rows, :], NT, preferred_element_type=F32)

    def fold(vals, op):
        r = functools.reduce(op, vals)
        r = op(r, pltpu.roll(r, 4, 0))
        return op(r, pltpu.roll(r, 2, 0))

    def exps(a, g):
        slabs = [a[g * GR + 8 * i:g * GR + 8 * i + 8] for i in range(GR // 8)]
        mx = fold(slabs, jnp.maximum)
        mn = fold(slabs, jnp.minimum)
        ep = [jnp.exp2(u - mx) for u in slabs]
        en = [jnp.exp2(mn - u) for u in slabs]
        return ep, en, fold(ep, jnp.add), fold(en, jnp.add)

    def b_pass1(i, c):
        rows = pl.ds(pl.multiple_of(i * TB, TB), TB)

        def features(half):
            a = b_proj(1, half, rows)
            phi = []
            for g in range(NG):
                ep, en, sp, sn = exps(a, g)
                inv = 1.0 / (sp * sn)
                ip, im = sn * inv, sp * inv
                phi += [e * ip for e in ep] + [e * im for e in en]
            phi = jnp.concatenate(phi, axis=0)
            zsum = phi[:, :LANES]
            for n in range(1, TB // LANES):
                zsum = zsum + phi[:, n * LANES:(n + 1) * LANES]
            return phi.astype(BF16), zsum

        def outer(half, vt, phi):
            for n, (lo, hi) in enumerate(spans):
                y = lax.dot_general(
                    vt[lo:hi], phi[n * LANES:(n + 1) * LANES], NT,
                    preferred_element_type=F32)
                r = lax.broadcasted_iota(jnp.int32, (hi - lo, LANES), 0) + lo
                f = lax.broadcasted_iota(jnp.int32, (1, LANES), 1) + n * LANES
                first = (f & 1) * fb
                for g in range(lo // GR, hi // GR):
                    first = jnp.where(f >= g * 2 * GR, g * GR + (f & 1) * fb, first)
                keep = (r >= first) & (r < first + fb)
                blk = slice(offs[n], offs[n + 1])
                old = jnp.where(i > 0, kv_ref[half, blk, :], 0.0)
                kv_ref[half, blk, :] = jnp.where(keep, old + y, 0.0)

        phi0, z0 = features(0)
        phi1, z1 = features(1)
        for half, z in enumerate((z0, z1)):
            z_ref[half] = jnp.where(i > 0, z_ref[half], 0.0) + z
        vt0 = b_proj(2, 0, rows)
        vt1 = b_proj(2, 1, rows)
        outer(0, vt0, phi0)
        outer(1, vt1, phi1)
        xnb_ref[S - seg:S, :] = _layernorm(xres_ref[S - seg:S, :]).astype(BF16)
        return c

    def b_pass2(i, c):
        tu = TB // 2

        def unit_rows(u):
            return pl.ds(pl.multiple_of(i * TB + u * tu, tu), tu)

        def features(u, half):
            a = b_proj(0, half, unit_rows(u))
            phi = []
            for g in range(NG):
                ep, en, sp, sn = exps(a, g)

                def zdot(es, base):
                    terms = []
                    for n, e in enumerate(es):
                        z = z_ref[half, base + 8 * n:base + 8 * n + 8, :]
                        terms.append(e * jnp.concatenate([z] * (tu // LANES), axis=1))
                    return functools.reduce(jnp.add, terms)

                den = zdot(ep, 2 * GR * g) * sn + zdot(en, 2 * GR * g + GR) * sp
                inv = 1.0 / (fold([den], jnp.add) + 1e-6 * (sp * sn))
                ip, im = sn * inv, sp * inv
                phi += [e * ip for e in ep] + [e * im for e in en]
            return jnp.concatenate(phi, axis=0).astype(BF16)

        def mix(half, phi):
            parts = [None] * NG
            for n, (lo, hi) in enumerate(spans):
                y = jnp.dot(
                    kv_ref[half, offs[n]:offs[n + 1], :],
                    phi[n * LANES:(n + 1) * LANES], preferred_element_type=F32)
                for g in range(lo // GR, hi // GR):
                    piece = y[g * GR - lo:(g + 1) * GR - lo]
                    parts[g] = piece if parts[g] is None else parts[g] + piece
            return jnp.concatenate(parts, axis=0)

        def finish(u, cols, o):
            rows = unit_rows(u)
            y = jnp.dot(o, _unpack(bwo_ref[:, cols]), preferred_element_type=F32)
            y = xres_ref[rows, cols] + y
            xres_ref[rows, cols] = y
            xb_ref[rows, cols] = y.astype(BF16)
            return y[:seg]

        phi, ot, o = {}, {}, {}
        for op in P2.split():
            u = int(op[1])
            if op[0] == "f":
                phi[op[1:]] = features(u, int(op[2]))
            elif op[0] == "m":
                ot[op[1:]] = mix(int(op[2]), phi.pop(op[1:]))
                if op[2] == "1":
                    o[u] = jnp.concatenate(
                        [ot.pop(op[1] + "0"), ot.pop(op[1:])], axis=0).T
            else:
                cols = slice(0, PW) if op[0] == "a" else slice(PW, D)
                ot[op] = finish(u, cols, o[u])
                if op[0] == "b":
                    pltpu.make_async_copy(
                        xb_ref.at[unit_rows(u), :], out_hbm.at[unit_rows(u), :],
                        osem).start()
        xna_ref[pl.ds(pl.multiple_of(i * TB, TB), seg), :] = _layernorm(
            jnp.concatenate([ot["a0"], ot["b0"]], axis=1))
        return c

    nblk = S // TB
    out_copy = pltpu.make_async_copy(xb_ref, out_hbm, osem)

    def layer(n, c):
        layer_a(n)
        pl.when(n == 0)(b_weights)
        lax.fori_loop(0, nblk, b_pass1, 0)
        z_ref[...] = jnp.broadcast_to(
            jnp.sum(z_ref[...], axis=2, keepdims=True), z_ref.shape)
        pl.when(n == 1)(out_copy.wait)
        lax.fori_loop(0, nblk, b_pass2, 0)
        return c

    lax.fori_loop(0, 2, layer, 0)
    out_copy.wait()


@functools.partial(jax.jit, static_argnames=("A_seg_len",))
def pallas_interleave_layers__memory_aug_recurrent_mem_tr__linear_kernel_hedgehog__prompt_kernel(
    A_x: jax.Array,
    A_mem0: jax.Array,
    A_Wq: jax.Array,
    A_Wk: jax.Array,
    A_Wv: jax.Array,
    A_Wo: jax.Array,
    A_seg_len: int,
    B_x: jax.Array,
    B_wqkv: jax.Array,
    B_w_phi: jax.Array,
    B_wo: jax.Array,
):
    del B_x
    _, S, D = A_x.shape
    M = A_mem0.shape[1]
    _, H, dh = A_Wq.shape
    hb = B_w_phi.shape[0]
    seg = int(A_seg_len)
    npair, PW = H // 2, 2 * dh
    assert A_x.shape[0] == 1 and PW == 3 * LANES and 2 * (M + seg) <= LANES
    assert (2 * NPRE - A_UNROLL[True]) * seg >= S and D == 5 * LANES and hb == 32 and S % TB == 0

    def rows_first(w):
        return jnp.transpose(w, (1, 2, 0)).reshape(H * dh, D)

    hbm = pl.BlockSpec(memory_space=pl.ANY)
    out = pl.pallas_call(
        functools.partial(_kernel, seg=seg, dh=dh, hb=hb),
        out_shape=jax.ShapeDtypeStruct((S, D), BF16),
        in_specs=[hbm] * 10,
        out_specs=hbm,
        scratch_shapes=[
            pltpu.VMEM((S, D), BF16),
            pltpu.VMEM((S, D), F32),
            pltpu.VMEM((S, D), F32),
            pltpu.VMEM((S, D), BF16),
            pltpu.VMEM((M, D), F32),
            pltpu.VMEM((NSLOT, 3, PW, D), BF16),
            pltpu.VMEM((npair, D // 2, 3 * PW), U32),
            pltpu.VMEM((H * dh // 2, D), U32),
            pltpu.VMEM((D, 3 * D), BF16),
            pltpu.VMEM((D, D), BF16),
            pltpu.VMEM((3, D // 2, D), U32),
            pltpu.VMEM((D // 2, D), U32),
            pltpu.VMEM((2, 480, LANES), F32),
            pltpu.VMEM((2, D, LANES), F32),
            pltpu.VMEM((NPRE, 8, D), BF16),
            pltpu.VMEM((NPRE * 4, D), U32),
            pltpu.VMEM((npair, NPRE * 8, 3 * PW), F32),
            pltpu.VMEM((M, D), BF16),
            pltpu.VMEM((D // hb, D // hb, hb), BF16),
            pltpu.VMEM((2 * D // hb, D), F32),
            pltpu.VMEM((npair, 4, M + 16, PW), F32),
            pltpu.SemaphoreType.DMA((NSLOT, 3)),
            pltpu.SemaphoreType.DMA((7,)),
            pltpu.SemaphoreType.DMA,
        ],
        compiler_params=pltpu.CompilerParams(
            vmem_limit_bytes=112 * 1024 * 1024, disable_bounds_checks=NOBC),
    )(
        A_x.reshape(S, D),
        A_x.reshape(S // seg, seg // 8, 8, D),
        A_mem0.reshape(M, D),
        rows_first(A_Wq),
        rows_first(A_Wk),
        rows_first(A_Wv),
        A_Wo.reshape(H * dh, D),
        B_wqkv,
        jnp.transpose(B_w_phi, (1, 2, 0)),
        B_wo,
    )
    return out.reshape(1, S, D)
```

```python
import functools

import jax
import jax.numpy as jnp
from jax import lax
import jax.experimental.pallas as pl
import jax.experimental.pallas.tpu as pltpu

F32 = jnp.float32
BF16 = jnp.bfloat16
U32 = jnp.uint32
LOG2E = 1.4426950408889634
NT = (((1,), (1,)), ((), ()))
TN = (((0,), (0,)), ((), ()))
LANES = 128

TB = 512
P2 = "f00 f01 f10 f11 m00 m01 m10 a0 m11 b0 a1 b1"
A_UNROLL = {False: 2, True: 2}
NOBC = True
OLAG = 1
SCHED = {True: ['k0 q0 v0 s0 k1 q1 v1 k2 p0 v2 b0 s1 q2 k3 v3 q3 p1 a0 s2 k4 a1 q4 v4 p2 s3 k5 a2 q5 v5 p3 s4 k6 v6 a3 q6 p4 s5 k7 a4 q7 v7 p5 s6 k8 a5 q8 v8 p6 s7 v9 k9 a6 q9 p7 s8 q10 k10 a7 v10 p8 s9 k11 a8 q11 v11 p9 s10 k12 a9 q12 v12 p10 s11 k13 q13 a10 v13 p11 s12 k14 a11 q14 v14 p12 s13 k15 a12 v15 q15 p13 s14 b2 s15 b8 b4 b1 b5 b3 p14 a13 b6 b7 b10 b9 a14 p15 b11 b12 a15 b15 b13 b14', 'k0 q0 v0 s0 k1 q1 v1 k2 p0 v2 s1 q2 k3 b0 v3 q3 p1 a0 s2 k4 a1 q4 v4 p2 s3 k5 a2 q5 v5 p3 s4 v6 k6 a3 q6 p4 s5 k7 a4 q7 v7 p5 s6 k8 a5 q8 v8 p6 s7 v9 k9 a6 q9 p7 s8 q10 k10 a7 v10 p8 s9 k11 q11 a8 v11 p9 s10 v12 k12 a9 q12 p10 s11 k13 q13 a10 v13 p11 s12 k14 a11 q14 v14 p12 s13 k15 a12 v15 q15 p13 s14 b2 s15 b4 b1 b8 b5 b3 p14 b6 b10 b7 a13 b9 a14 p15 b12 b11 b13 a15 b14 b15'], False: ['k0 q0 v0 s0 k1 q1 v1 p0 s1 k2 q2 v2 p1 s2 k3 q3 v3 p2 s3 k4 q4 v4 p3 s4 k5 q5 v5 p4 s5 o0 k6 q6 v6 p5 s6 k7 q7 v7 p6 s7 k8 q8 o1 v8 p7 s8 k9 q9 o2 v9 p8 s9 k10 q10 o3 v10 p9 s10 k11 q11 o4 v11 p10 s11 k12 q12 o5 v12 p11 s12 k13 q13 o6 v13 p12 s13 k14 q14 o7 v14 p13 v15 s14 k15 q15 o8 p14 s15 o9 o10 o11 p15 o12 a13 a14 a15 b13 b14 b15', 'k0 q0 v0 s0 k1 q1 v1 p0 s1 k2 q2 v2 p1 s2 k3 q3 v3 p2 s3 k4 q4 v4 p3 s4 k5 q5 o0 v5 p4 s5 k6 q6 o1 v6 p5 s6 k7 q7 o2 v7 p6 s7 k8 q8 o3 v8 p7 s8 q9 k9 o4 v9 p8 s9 v10 k10 q10 o5 p9 s10 k11 q11 o6 v11 p10 s11 k12 q12 o7 v12 p11 s12 k13 v13 q13 o8 q14 p12 s13 k14 o9 v14 p13 s14 k15 q15 o10 v15 p14 s15 o11 o13 o12 p15 o14 o15']}
NSCORE = {False: ['1111111111111000', '1211111111111100'], True: ['0111111111111000', '0111101111111011']}
MASKED = -1e9 * LOG2E
NSLOT = 3
NPRE = 40


def _layernorm(x):
    m = jnp.mean(x, axis=-1, keepdims=True)
    xc = x - m
    v = jnp.mean(xc * xc, axis=-1, keepdims=True)
    return xc * lax.rsqrt(v + 1e-5)


def _pack(w):
    return pltpu.bitcast(w, U32)


def _unpack(w):
    return pltpu.bitcast(w, BF16)


def _kernel(
    x_hbm, x4_hbm, mem_hbm, wq_hbm, wk_hbm, wv_hbm, wo_hbm, bw_hbm, wphi_hbm, bwo_hbm,
    out_hbm,
    xb_ref, xres_ref, xna_ref, xnb_ref, memf_ref,
    stage_ref, wo_ref, w_ref,
    bw_ref, bwo_stage_ref, bwt_ref, bwo_ref,
    kv_ref, z_ref, xsel_ref, xseln_ref, pre_ref, mem_ref, wphi_ref, wrep_ref, row_ref,
    wsem, wosem, sem, osem,
    *, seg, dh, hb,
):
    S, D = xres_ref.shape
    M = mem_ref.shape[0]
    L = M + seg
    nseg = S // seg
    PW = 2 * dh
    npair = w_ref.shape[0]
    HL = LANES // 2
    mixed = [h * dh + r for r in range(0, dh, HL) for h in range(2)]
    fb = D // hb
    GR = 2 * fb
    HR = D // 2
    NG = HR // GR
    NTILE = 2 * HR // LANES
    spans = []
    for i in range(NTILE):
        lo = (i * LANES) // (2 * GR)
        hi = ((i + 1) * LANES - 1) // (2 * GR) + 1
        spans.append((lo * GR, hi * GR))
    offs = [0]
    for lo, hi in spans:
        offs.append(offs[-1] + hi - lo)

    XH = (A_UNROLL[True] + 2) * seg

    def wcopy(j, t):
        rows = pl.ds(pl.multiple_of(j * PW, PW), PW)
        return pltpu.make_async_copy(
            (wq_hbm, wk_hbm, wv_hbm)[t].at[rows, :],
            stage_ref.at[j % NSLOT, t], wsem.at[j % NSLOT, t])

    def ocopy(j):
        rows = pl.ds(pl.multiple_of(j * PW, PW), PW)
        return pltpu.make_async_copy(
            wo_hbm.at[rows, :], wo_ref.at[rows, :], wosem.at[j % 8])

    def keep_wo(j):
        w = jnp.concatenate(
            [wo_ref[pl.ds(pl.multiple_of(j * PW + r, HL), HL), :] for r in mixed],
            axis=0)
        w_ref[j, D // 2:D // 2 + dh, 0:D] = _pack(w)

    def start_pair(j):
        for t in range(3):
            wcopy(j, t).start()

    xsel_copy = pltpu.make_async_copy(
        x4_hbm.at[0:NPRE, seg // 8 - 1], xsel_ref, sem.at[0])
    bw_copy = pltpu.make_async_copy(bw_hbm, bw_ref, sem.at[1])
    bwo_copy = pltpu.make_async_copy(bwo_hbm, bwo_stage_ref, sem.at[2])
    xh_copy = pltpu.make_async_copy(
        x_hbm.at[0:XH, :], xb_ref.at[0:XH, :], sem.at[3])
    xt_copy = pltpu.make_async_copy(
        x_hbm.at[XH:S, :], xb_ref.at[XH:S, :], sem.at[3])
    mem_copy = pltpu.make_async_copy(mem_hbm, mem_ref, sem.at[5])
    wphi_copy = pltpu.make_async_copy(wphi_hbm, wphi_ref, sem.at[4])
    wphi_copy.start()
    xsel_copy.start()
    xh_copy.start()
    start_pair(0)

    wphi_copy.wait()
    hh = lax.broadcasted_iota(jnp.int32, (hb, D), 0)
    cc = lax.broadcasted_iota(jnp.int32, (hb, D), 1)

    def spread(i, wcat):
        for d in range(4):
            sel = jnp.where(cc == hh * fb + (4 * i + d), 1.0, 0.0).astype(BF16)
            wcat += jnp.dot(wphi_ref[4 * i + d], sel, preferred_element_type=F32)
        return wcat

    wcat = lax.fori_loop(0, fb // 4, spread, jnp.zeros((fb, D), F32))
    rr = lax.broadcasted_iota(jnp.int32, (GR, fb), 0)
    ff = lax.broadcasted_iota(jnp.int32, (GR, fb), 1)
    twice = jnp.where((rr >> 1) == ff, 1.0, 0.0).astype(BF16)
    wrep_ref[...] = jnp.dot(twice, wcat.astype(BF16), preferred_element_type=F32)

    xsel_copy.wait()
    xsel = xsel_ref[...].astype(F32).reshape(NPRE * 8, D)
    xseln_ref[...] = _pack(_layernorm(xsel).astype(BF16))
    xh_copy.wait()
    xna_ref[0:seg, :] = _layernorm(xb_ref[0:seg, :].astype(F32))

    def load_pair(j, c):
        slot = j % NSLOT
        for t in range(3):
            wcopy(j, t).wait()

        @pl.when(j == 0)
        def _():
            start_pair(1)
            mem_copy.start()

        @pl.when(j + 2 < npair)
        def _():
            start_pair(j + 2)

        @pl.when(j >= OLAG)
        def _():
            ocopy(j - OLAG).start()

        @pl.when(j >= npair - OLAG)
        def _():
            ocopy(j).start()

        @pl.when(j >= OLAG + 2)
        def _():
            ocopy(j - OLAG - 2).wait()

        keep_wo(jnp.where(j >= OLAG + 2, j - OLAG - 2, npair - 1))
        for t in range(3):
            cols = slice(t * PW, (t + 1) * PW)
            w = jnp.concatenate(
                [stage_ref[slot, t, r:r + HL, :]
                 for r in (mixed if t == 2 else range(0, PW, HL))], axis=0)
            w_ref[j, 0:D // 2, cols] = _pack(w.astype(F32).T.astype(BF16))
            xn = _unpack(xseln_ref[...])
            if t == 0:
                y = lax.dot_general(
                    xn, stage_ref[slot, t], NT, preferred_element_type=F32)
            else:
                y = jnp.dot(xn, _unpack(w_ref[j, 0:D // 2, cols]),
                            preferred_element_type=F32)
            pre_ref[j, :, cols] = y
        return c

    lax.fori_loop(0, npair, load_pair, 0)
    mem_copy.wait()

    @pl.loop(npair - OLAG - 2, npair)
    def _(j):
        ocopy(j).wait()
        keep_wo(j)

    xt_copy.start()
    bw_copy.start()
    bwo_copy.start()

    def b_weights():
        bw_copy.wait()
        bwo_copy.wait()
        rr = lax.broadcasted_iota(jnp.int32, (GR, LANES), 0)
        cc = lax.broadcasted_iota(jnp.int32, (GR, LANES), 1) - (rr & 1) * fb
        for t in range(2):
            parts = [None] * (D // GR)
            for n in range(D // LANES):
                lo = (n * LANES) // GR
                hi = ((n + 1) * LANES - 1) // GR + 1
                col = cc + n * LANES
                lhs = jnp.concatenate([
                    jnp.where((col >= g * GR) & (col < g * GR + fb),
                              wrep_ref[:, n * LANES:(n + 1) * LANES], 0.0)
                    for g in range(lo, hi)
                ], axis=0)
                y = lax.dot_general(
                    lhs, bw_ref[:, t * D + n * LANES:t * D + (n + 1) * LANES], NT,
                    preferred_element_type=F32)
                for g in range(lo, hi):
                    piece = y[(g - lo) * GR:(g - lo + 1) * GR]
                    parts[g] = piece if parts[g] is None else parts[g] + piece
            w = jnp.concatenate(parts, axis=0) * LOG2E
            bwt_ref[t] = _pack(w.astype(BF16))
        bwt_ref[2] = _pack(bw_ref[:, 2 * D:3 * D].T)
        bwo_ref[...] = _pack(bwo_stage_ref[...])

    def a_step(short, s, mem, u):
        rows = pl.ds(pl.multiple_of(s * seg, seg), seg)
        sub = lax.broadcasted_iota(jnp.int32, (8, LANES), 0)
        lane = lax.broadcasted_iota(jnp.int32, (8, LANES), 1)
        is_a = lane < L
        col = jnp.where(is_a, lane, lane - L)
        low = lane < HL
        lows = lax.broadcasted_iota(jnp.int32, (L, LANES), 1) < HL
        scale = jnp.where(
            lax.broadcasted_iota(jnp.int32, (L, PW), 1) + s >= 0,
            dh ** -0.5 * LOG2E, 0.0)
        nscore = [min(int(n), 2) for n in NSCORE[short][u]]
        nmix = [(int(n) + 1) // 2 for n in NSCORE[short][u]]

        def part(j, t, lo, hi):
            n = seg - 8 if short else seg
            x = xna_ref[pl.ds(pl.multiple_of(s * seg, seg), n), lo:hi]
            h = jnp.concatenate([mem[:, lo:hi], x], axis=0)
            w = _unpack(w_ref[j, lo // 2:hi // 2, t * PW:(t + 1) * PW])
            return jnp.dot(h.astype(BF16) if short else h, w,
                           preferred_element_type=F32)

        def proj(j, t, head=None):
            if head is None:
                y = part(j, t, 0, D)
            else:
                y = part(j, t, PW, D) + head
            if short:
                tail = pl.ds(pl.multiple_of(s * 8, 8), 8)
                y = jnp.concatenate(
                    [y, pre_ref[j, tail, t * PW:(t + 1) * PW]], axis=0)
            if t == 0:
                return y * scale
            for b in range(nscore[j] if t == 1 else nmix[j]):
                n = M + 8 * b + 8
                row_ref[j, 2 * b + t - 1, 0:n, :] = y[:n]
            return y

        def spread_row(j, t, r, c):
            return jnp.broadcast_to(
                row_ref[j, t - 1, r:r + 1, c * LANES:(c + 1) * LANES], (8, LANES))

        def stack(top, bot):
            pad = jnp.zeros((LANES - 2 * L, PW), F32)
            return jnp.concatenate([top, bot, pad], axis=0).astype(BF16)

        def keys(k):
            zero = jnp.zeros((L, LANES), F32)
            mid = k[:, LANES:2 * LANES]
            return stack(
                jnp.concatenate(
                    [k[:, :LANES], jnp.where(lows, mid, 0.0), zero], axis=1),
                jnp.concatenate(
                    [zero, jnp.where(lows, 0.0, mid), k[:, 2 * LANES:]], axis=1))

        def values(v):
            first = jnp.concatenate([lows] * 3, axis=1)
            return stack(jnp.where(first, v, 0.0), jnp.where(first, 0.0, v))

        def softmax(sc, row):
            inside = col < L
            vis = inside if row < M else col <= sub + row
            sc = jnp.where(vis, sc, jnp.where(inside, MASKED, -jnp.inf))
            ma = jnp.max(jnp.where(is_a, sc, -jnp.inf), axis=1, keepdims=True)
            mb = jnp.max(jnp.where(is_a, -jnp.inf, sc), axis=1, keepdims=True)
            e = jnp.exp2(sc - jnp.where(is_a, ma, mb))
            la = jnp.sum(jnp.where(is_a, e, 0.0), axis=1, keepdims=True)
            lb = jnp.sum(jnp.where(is_a, 0.0, e), axis=1, keepdims=True)
            return e * (1.0 / jnp.where(is_a, la, lb))

        def vpu_scores(j, q, row):
            q = q[row:row + 8]
            mid = q[:, LANES:2 * LANES]
            qa, qb = jnp.where(low, mid, 0.0), jnp.where(low, 0.0, mid)
            out = []
            for r in range(row + 8):
                k0, k1, k2 = (spread_row(j, (row - M) // 4 + 1, r, c) for c in range(3))
                out.append((
                    jnp.sum(q[:, :LANES] * k0 + qa * k1, axis=1, keepdims=True),
                    jnp.sum(q[:, 2 * LANES:] * k2 + qb * k1, axis=1, keepdims=True)))
            return out

        def to_lanes(scores):
            out = None
            for h in range(2):
                vals = [jnp.broadcast_to(x[h], (8, LANES)) for x in scores]
                for bit in (1, 2, 4):
                    vals = [jnp.where((lane & bit) == 0, vals[i], vals[i + 1])
                            for i in range(0, len(vals), 2)]
                for g, x in enumerate(vals):
                    out = x if out is None else jnp.where(
                        lane < h * L + 8 * g, out, x)
            return out

        def vpu_attend(j, scores):
            row = len(scores) - 8
            sc = [jnp.where(low, a, b) for a, b in scores]
            sc = [x if r <= row else jnp.where(sub >= r - row, x, MASKED)
                  for r, x in enumerate(sc)]
            top = functools.reduce(jnp.maximum, sc)
            acc = None
            for r, x in enumerate(sc):
                e = jnp.exp2(x - top)
                t = [e * spread_row(j, (row - M) // 4 + 2, r, c) for c in range(3)] + [e]
                acc = t if acc is None else [u + w for u, w in zip(acc, t)]
            inv = 1.0 / acc[3]
            return jnp.concatenate([x * inv for x in acc[:3]], axis=1)

        def probs(j, q, k):
            far = M + 8 * nscore[j]
            sc = lax.dot_general(
                jnp.concatenate([q[:M], q[far:]], axis=0), keys(k), NT,
                preferred_element_type=F32)
            p = {0: softmax(sc[:M], 0)}
            for row in range(far, L, 8):
                p[row] = softmax(sc[row - far + M:row - far + M + 8], row)
            first = [vpu_scores(j, q, M + 8 * b) for b in range(nmix[j])]
            for row in range(M + 8 * nmix[j], far, 8):
                p[row] = softmax(to_lanes(vpu_scores(j, q, row)), row)
            return jnp.concatenate([p[row] for row in sorted(p)], axis=0), first

        prv = pl.ds(pl.multiple_of(jnp.maximum(s - 1, 0) * seg, seg), seg)
        nxt = pl.ds(pl.multiple_of(jnp.minimum(s + 1, nseg - 1) * seg, seg), seg)
        if short:
            far = jnp.where(s < A_UNROLL[True], s, nseg - 1 + A_UNROLL[True] - s)
            far = jnp.where(far < NPRE, s, far)
            far = pl.ds(pl.multiple_of(far * seg, seg), seg)
            xres_ref[far, :] = xb_ref[far, :].astype(F32)
        xnb_ref[prv, :] = _layernorm(xres_ref[prv, :]).astype(BF16)
        xin_ref = xb_ref if short else xres_ref
        xn_next = _layernorm(xin_ref[nxt, :].astype(F32))

        q, k, v, p, o = {}, {}, {}, {}, {}
        acc, whole = [None, None], None
        head_k = head_q = None
        if u > 0:
            head_k, head_q = part(0, 1, 0, PW), part(0, 0, 0, PW)
        for op, j in ((t[0], int(t[1:])) for t in SCHED[short][u].split()):
            if op == "q":
                q[j] = proj(j, 0, head_q if j == 0 else None)
            elif op == "k":
                k[j] = proj(j, 1, head_k if j == 0 else None)
            elif op == "v":
                v[j] = proj(j, 2)
            elif op == "s":
                p[j] = probs(j, q.pop(j), k.pop(j))
            elif op == "p":
                y = jnp.dot(
                    p[j][0], values(v.pop(j)), preferred_element_type=F32)
                o[j] = jnp.concatenate(
                    [y[:M]] + [vpu_attend(j, x) for x in p[j][1]] + [y[M:]], axis=0)
                if j == npair - 1:
                    xna_ref[nxt, :] = xn_next
            else:
                lo, hi = {"a": (0, PW), "b": (PW, D), "o": (0, D)}[op]
                w = _unpack(w_ref[j, D // 2:D // 2 + dh, lo:hi])
                y = jnp.dot(o[j], w, preferred_element_type=F32)
                if op == "o":
                    whole = y if whole is None else whole + y
                else:
                    n = "ab".index(op)
                    if acc[n] is None and whole is not None:
                        acc[n] = whole[:, lo:hi]
                    acc[n] = y if acc[n] is None else acc[n] + y
        acc = whole if acc[0] is None else jnp.concatenate(acc, axis=1)
        xres_ref[rows, :] = xin_ref[rows, :].astype(F32) + acc[M:]
        return acc[:M]

    def a_steps(short, i, c):
        if short:
            pl.when(i == 1)(xt_copy.wait)
        mem = memf_ref[...]
        n = A_UNROLL[short]
        for u in range(n):
            mem = a_step(short, i * n + u, mem, u)
        memf_ref[...] = mem
        return c

    def layer_a(n):
        memf_ref[...] = mem_ref[...].astype(F32)
        lax.fori_loop(0, jnp.where(n == 0, NPRE // A_UNROLL[True], 0),
                      functools.partial(a_steps, True), 0)
        lax.fori_loop(jnp.where(n == 0, NPRE // A_UNROLL[False], 0),
                      nseg // A_UNROLL[False],
                      functools.partial(a_steps, False), 0)

    def b_proj(t, half, rows):
        w = _unpack(bwt_ref[t, half * (HR // 2):(half + 1) * (HR // 2), :])
        return lax.dot_general(
            w, xnb_ref[rows, :], NT, preferred_element_type=F32)

    def fold(vals, op):
        r = functools.reduce(op, vals)
        r = op(r, pltpu.roll(r, 4, 0))
        return op(r, pltpu.roll(r, 2, 0))

    def exps(a, g):
        slabs = [a[g * GR + 8 * i:g * GR + 8 * i + 8] for i in range(GR // 8)]
        mx = fold(slabs, jnp.maximum)
        mn = fold(slabs, jnp.minimum)
        ep = [jnp.exp2(u - mx) for u in slabs]
        en = [jnp.exp2(mn - u) for u in slabs]
        return ep, en, fold(ep, jnp.add), fold(en, jnp.add)

    def b_pass1(i, c):
        rows = pl.ds(pl.multiple_of(i * TB, TB), TB)

        def features(half):
            a = b_proj(1, half, rows)
            phi = []
            for g in range(NG):
                ep, en, sp, sn = exps(a, g)
                inv = 1.0 / (sp * sn)
                ip, im = sn * inv, sp * inv
                phi += [e * ip for e in ep] + [e * im for e in en]
            phi = jnp.concatenate(phi, axis=0)
            zsum = phi[:, :LANES]
            for n in range(1, TB // LANES):
                zsum = zsum + phi[:, n * LANES:(n + 1) * LANES]
            return phi.astype(BF16), zsum

        def outer(half, vt, phi):
            for n, (lo, hi) in enumerate(spans):
                y = lax.dot_general(
                    vt[lo:hi], phi[n * LANES:(n + 1) * LANES], NT,
                    preferred_element_type=F32)
                r = lax.broadcasted_iota(jnp.int32, (hi - lo, LANES), 0) + lo
                f = lax.broadcasted_iota(jnp.int32, (1, LANES), 1) + n * LANES
                first = (f & 1) * fb
                for g in range(lo // GR, hi // GR):
                    first = jnp.where(f >= g * 2 * GR, g * GR + (f & 1) * fb, first)
                keep = (r >= first) & (r < first + fb)
                blk = slice(offs[n], offs[n + 1])
                old = jnp.where(i > 0, kv_ref[half, blk, :], 0.0)
                kv_ref[half, blk, :] = jnp.where(keep, old + y, 0.0)

        phi0, z0 = features(0)
        phi1, z1 = features(1)
        for half, z in enumerate((z0, z1)):
            z_ref[half] = jnp.where(i > 0, z_ref[half], 0.0) + z
        vt0 = b_proj(2, 0, rows)
        vt1 = b_proj(2, 1, rows)
        outer(0, vt0, phi0)
        outer(1, vt1, phi1)
        xnb_ref[S - seg:S, :] = _layernorm(xres_ref[S - seg:S, :]).astype(BF16)
        return c

    def b_pass2(i, c):
        tu = TB // 2

        def unit_rows(u):
            return pl.ds(pl.multiple_of(i * TB + u * tu, tu), tu)

        def features(u, half):
            a = b_proj(0, half, unit_rows(u))
            phi = []
            for g in range(NG):
                ep, en, sp, sn = exps(a, g)

                def zdot(es, base):
                    terms = []
                    for n, e in enumerate(es):
                        z = z_ref[half, base + 8 * n:base + 8 * n + 8, :]
                        terms.append(e * jnp.concatenate([z] * (tu // LANES), axis=1))
                    return functools.reduce(jnp.add, terms)

                den = zdot(ep, 2 * GR * g) * sn + zdot(en, 2 * GR * g + GR) * sp
                inv = 1.0 / (fold([den], jnp.add) + 1e-6 * (sp * sn))
                ip, im = sn * inv, sp * inv
                phi += [e * ip for e in ep] + [e * im for e in en]
            return jnp.concatenate(phi, axis=0).astype(BF16)

        def mix(half, phi):
            parts = [None] * NG
            for n, (lo, hi) in enumerate(spans):
                y = jnp.dot(
                    kv_ref[half, offs[n]:offs[n + 1], :],
                    phi[n * LANES:(n + 1) * LANES], preferred_element_type=F32)
                for g in range(lo // GR, hi // GR):
                    piece = y[g * GR - lo:(g + 1) * GR - lo]
                    parts[g] = piece if parts[g] is None else parts[g] + piece
            return jnp.concatenate(parts, axis=0)

        def finish(u, cols, o):
            rows = unit_rows(u)
            y = jnp.dot(o, _unpack(bwo_ref[:, cols]), preferred_element_type=F32)
            y = xres_ref[rows, cols] + y
            xres_ref[rows, cols] = y
            xb_ref[rows, cols] = y.astype(BF16)
            return y[:seg]

        phi, ot, o = {}, {}, {}
        for op in P2.split():
            u = int(op[1])
            if op[0] == "f":
                phi[op[1:]] = features(u, int(op[2]))
            elif op[0] == "m":
                ot[op[1:]] = mix(int(op[2]), phi.pop(op[1:]))
                if op[2] == "1":
                    o[u] = jnp.concatenate(
                        [ot.pop(op[1] + "0"), ot.pop(op[1:])], axis=0).T
            else:
                cols = slice(0, PW) if op[0] == "a" else slice(PW, D)
                ot[op] = finish(u, cols, o[u])
                if op[0] == "b":
                    pltpu.make_async_copy(
                        xb_ref.at[unit_rows(u), :], out_hbm.at[unit_rows(u), :],
                        osem).start()
        xna_ref[pl.ds(pl.multiple_of(i * TB, TB), seg), :] = _layernorm(
            jnp.concatenate([ot["a0"], ot["b0"]], axis=1))
        return c

    nblk = S // TB
    out_copy = pltpu.make_async_copy(xb_ref, out_hbm, osem)

    def layer(n, c):
        layer_a(n)
        pl.when(n == 0)(b_weights)
        lax.fori_loop(0, nblk, b_pass1, 0)
        z_ref[...] = jnp.broadcast_to(
            jnp.sum(z_ref[...], axis=2, keepdims=True), z_ref.shape)
        pl.when(n == 1)(out_copy.wait)
        lax.fori_loop(0, nblk, b_pass2, 0)
        return c

    lax.fori_loop(0, 2, layer, 0)
    out_copy.wait()


@functools.partial(jax.jit, static_argnames=("A_seg_len",))
def pallas_interleave_layers__memory_aug_recurrent_mem_tr__linear_kernel_hedgehog__prompt_kernel(
    A_x: jax.Array,
    A_mem0: jax.Array,
    A_Wq: jax.Array,
    A_Wk: jax.Array,
    A_Wv: jax.Array,
    A_Wo: jax.Array,
    A_seg_len: int,
    B_x: jax.Array,
    B_wqkv: jax.Array,
    B_w_phi: jax.Array,
    B_wo: jax.Array,
):
    del B_x
    _, S, D = A_x.shape
    M = A_mem0.shape[1]
    _, H, dh = A_Wq.shape
    hb = B_w_phi.shape[0]
    seg = int(A_seg_len)
    npair, PW = H // 2, 2 * dh
    assert A_x.shape[0] == 1 and PW == 3 * LANES and 2 * (M + seg) <= LANES
    assert (2 * NPRE - A_UNROLL[True]) * seg >= S and D == 5 * LANES and hb == 32 and S % TB == 0

    def rows_first(w):
        return jnp.transpose(w, (1, 2, 0)).reshape(H * dh, D)

    hbm = pl.BlockSpec(memory_space=pl.ANY)
    out = pl.pallas_call(
        functools.partial(_kernel, seg=seg, dh=dh, hb=hb),
        out_shape=jax.ShapeDtypeStruct((S, D), BF16),
        in_specs=[hbm] * 10,
        out_specs=hbm,
        scratch_shapes=[
            pltpu.VMEM((S, D), BF16),
            pltpu.VMEM((S, D), F32),
            pltpu.VMEM((S, D), F32),
            pltpu.VMEM((S, D), BF16),
            pltpu.VMEM((M, D), F32),
            pltpu.VMEM((NSLOT, 3, PW, D), BF16),
            pltpu.VMEM((H * dh, D), BF16),
            pltpu.VMEM((npair, D // 2 + dh, 3 * PW), U32),
            pltpu.VMEM((D, 3 * D), BF16),
            pltpu.VMEM((D, D), BF16),
            pltpu.VMEM((3, D // 2, D), U32),
            pltpu.VMEM((D // 2, D), U32),
            pltpu.VMEM((2, 480, LANES), F32),
            pltpu.VMEM((2, D, LANES), F32),
            pltpu.VMEM((NPRE, 8, D), BF16),
            pltpu.VMEM((NPRE * 4, D), U32),
            pltpu.VMEM((npair, NPRE * 8, 3 * PW), F32),
            pltpu.VMEM((M, D), BF16),
            pltpu.VMEM((D // hb, D // hb, hb), BF16),
            pltpu.VMEM((2 * D // hb, D), F32),
            pltpu.VMEM((npair, 4, M + 16, PW), F32),
            pltpu.SemaphoreType.DMA((NSLOT, 3)),
            pltpu.SemaphoreType.DMA((8,)),
            pltpu.SemaphoreType.DMA((6,)),
            pltpu.SemaphoreType.DMA,
        ],
        compiler_params=pltpu.CompilerParams(
            vmem_limit_bytes=112 * 1024 * 1024, disable_bounds_checks=NOBC),
    )(
        A_x.reshape(S, D),
        A_x.reshape(S // seg, seg // 8, 8, D),
        A_mem0.reshape(M, D),
        rows_first(A_Wq),
        rows_first(A_Wk),
        rows_first(A_Wv),
        A_Wo.reshape(H * dh, D),
        B_wqkv,
        jnp.transpose(B_w_phi, (1, 2, 0)),
        B_wo,
    )
    return out.reshape(1, S, D)
```

```python
import functools

import jax
import jax.numpy as jnp
from jax import lax
import jax.experimental.pallas as pl
import jax.experimental.pallas.tpu as pltpu

F32 = jnp.float32
BF16 = jnp.bfloat16
U32 = jnp.uint32
LOG2E = 1.4426950408889634
NT = (((1,), (1,)), ((), ()))
TN = (((0,), (0,)), ((), ()))
LANES = 128

TB = 512
P2 = "f00 f01 f10 f11 m00 m01 m10 a0 m11 b0 a1 b1"
A_UNROLL = {False: 2, True: 2}
NOBC = True
OLAG = 1
SCHED = {True: ['k0 q0 v0 s0 k1 q1 v1 k2 p0 v2 b0 s1 q2 k3 v3 q3 p1 a0 s2 k4 a1 q4 v4 p2 s3 k5 a2 q5 v5 p3 s4 k6 v6 a3 q6 s5 p4 k7 a4 q7 v7 p5 s6 k8 a5 q8 v8 p6 s7 v9 k9 a6 q9 p7 s8 q10 k10 a7 v10 p8 s9 k11 a8 q11 v11 p9 s10 k12 a9 q12 v12 p10 s11 k13 q13 a10 v13 p11 s12 k14 a11 v14 q14 p12 s13 k15 a12 v15 q15 p13 s14 b2 s15 b8 b4 b5 b3 b1 p14 a13 b6 b7 b10 b9 a14 p15 b11 b12 a15 b13 b14 b15', 'k0 q0 v0 s0 k1 q1 v1 k2 p0 v2 s1 q2 k3 b0 v3 q3 p1 a0 s2 k4 a1 q4 v4 p2 s3 k5 a2 q5 v5 p3 s4 v6 k6 a3 q6 p4 s5 k7 a4 q7 v7 p5 s6 k8 a5 q8 v8 p6 s7 v9 k9 a6 q9 p7 s8 q10 k10 a7 v10 p8 s9 k11 q11 a8 v11 p9 s10 v12 k12 a9 q12 p10 s11 k13 q13 a10 v13 p11 s12 k14 a11 q14 v14 p12 s13 k15 a12 v15 q15 p13 s14 b2 s15 b8 b4 b1 b5 b3 p14 b6 b12 b10 b7 a13 b9 a14 p15 b11 b13 a15 b14 b15'], False: ['k0 q0 v0 s0 K1 K1 K1 Q1 Q1 w0 Q1 w0 V1 w0 V1 w0 V1 w0 p0 s1 w1 K2 m0 m0 K2 K2 w1 Q2 m0 w1 Q2 w1 Q2 m0 V2 m0 V2 V2 p1 w1 s2 K3 K3 w2 K3 m1 m1 Q3 w2 O0 Q3 m1 O0 Q3 w2 V3 m1 O0 w2 m1 V3 V3 O0 p2 w2 s3 K4 K4 w3 K4 m2 m2 Q4 w3 O0 Q4 m2 O1 Q4 w3 V4 m2 O1 w3 m2 V4 V4 O1 p3 w3 s4 K5 K5 w4 K5 m3 m3 Q5 w4 O1 Q5 m3 O1 Q5 w4 V5 m3 O2 w4 m3 V5 V5 O2 p4 w4 s5 K6 K6 w5 K6 m4 m4 Q6 w5 O2 Q6 m4 O2 Q6 w5 V6 m4 O2 w5 m4 V6 V6 O3 p5 w5 s6 K7 K7 w6 K7 m5 m5 Q7 w6 O3 Q7 m5 O3 Q7 w6 V7 m5 O3 w6 m5 V7 V7 O3 p6 w6 s7 K8 K8 w7 K8 m6 m6 Q8 w7 O4 Q8 m6 O4 Q8 w7 V8 m6 O4 w7 m6 V8 V8 O4 p7 w7 s8 K9 K9 w8 K9 m7 m7 Q9 w8 O4 Q9 m7 O5 Q9 w8 V9 m7 O5 w8 m7 V9 V9 O5 p8 w8 s9 K10 K10 w9 K10 m8 m8 Q10 w9 O5 Q10 m8 O5 Q10 w9 V10 m8 O6 w9 m8 V10 V10 O6 p9 w9 s10 K11 K11 w10 K11 m9 m9 Q11 w10 O6 Q11 m9 O6 Q11 w10 V11 m9 O6 w10 m9 V11 V11 O7 p10 w10 s11 K12 K12 w11 K12 m10 m10 Q12 w11 O7 Q12 m10 O7 Q12 w11 V12 m10 O7 w11 m10 V12 V12 O7 p11 w11 s12 K13 K13 w12 K13 m11 m11 Q13 w12 O8 Q13 m11 O8 Q13 w12 V13 m11 O8 w12 m11 V13 V13 O8 p12 w12 s13 K14 K14 w13 K14 m12 m12 Q14 w13 O8 Q14 m12 O9 Q14 w13 V14 m12 O9 w13 m12 V14 V14 O9 p13 w13 s14 K15 K15 w14 K15 m13 m13 Q15 w14 O9 Q15 m13 O9 Q15 w14 V15 m13 O10 w14 m13 V15 V15 O10 p14 w14 s15 m14 O10 O10 O10 m14 O11 O11 O11 m14 O11 O11 O12 m14 O12 O12 O12 m14 O12 O13 p15 O13 O13 O13 O13 a14 a15 b14 b15', 'k0 q0 v0 s0 K1 K1 K1 Q1 Q1 w0 Q1 w0 V1 w0 V1 w0 V1 w0 p0 s1 w1 K2 m0 m0 K2 K2 w1 Q2 m0 w1 Q2 w1 Q2 m0 V2 m0 V2 V2 p1 w1 s2 K3 K3 w2 K3 m1 m1 Q3 w2 O0 Q3 m1 O0 Q3 w2 V3 m1 O0 w2 m1 V3 V3 O0 p2 w2 s3 K4 K4 w3 K4 m2 m2 Q4 w3 O0 Q4 m2 O1 Q4 w3 V4 m2 O1 w3 m2 V4 V4 O1 p3 w3 s4 K5 K5 w4 K5 m3 m3 Q5 w4 O1 Q5 m3 O1 Q5 w4 V5 m3 O2 w4 m3 V5 V5 O2 p4 w4 s5 K6 K6 w5 K6 m4 m4 Q6 w5 O2 Q6 m4 O2 Q6 w5 V6 m4 O2 w5 m4 V6 V6 O3 p5 w5 s6 K7 K7 w6 K7 m5 m5 Q7 w6 O3 Q7 m5 O3 Q7 w6 V7 m5 O3 w6 m5 V7 V7 O3 p6 w6 s7 K8 K8 w7 K8 m6 m6 Q8 w7 O4 Q8 m6 O4 Q8 w7 V8 m6 O4 w7 m6 V8 V8 O4 p7 w7 s8 K9 K9 w8 K9 m7 m7 Q9 w8 O4 Q9 m7 O5 Q9 w8 V9 m7 O5 w8 m7 V9 V9 O5 p8 w8 s9 K10 K10 w9 K10 m8 m8 Q10 w9 O5 Q10 m8 O5 Q10 w9 V10 m8 O6 w9 m8 V10 V10 O6 p9 w9 s10 K11 K11 w10 K11 m9 m9 Q11 w10 O6 Q11 m9 O6 Q11 w10 V11 m9 O6 w10 m9 V11 V11 O7 p10 w10 s11 K12 K12 w11 K12 m10 m10 Q12 w11 O7 Q12 m10 O7 Q12 w11 V12 m10 O7 w11 m10 V12 V12 O7 p11 w11 s12 K13 K13 w12 K13 m11 m11 Q13 w12 O8 Q13 m11 O8 Q13 w12 V13 m11 O8 w12 m11 V13 V13 O8 p12 w12 s13 K14 K14 w13 K14 m12 m12 Q14 w13 O8 Q14 m12 O9 Q14 w13 V14 m12 O9 w13 m12 V14 V14 O9 p13 w13 s14 K15 K15 w14 K15 m13 m13 Q15 w14 O9 Q15 m13 O9 Q15 w14 V15 m13 O10 w14 m13 V15 V15 O10 p14 w14 s15 m14 O10 O10 O10 m14 O11 O11 O11 m14 O11 O11 O12 m14 O12 O12 O12 m14 O12 O13 p15 O13 O13 O13 O13 o14 o15']}
NSCORE = {False: ['2222222212222200', '2222222222222210'], True: ['0111101111110000', '0101101101110111']}
MASKED = -1e9 * LOG2E
NSLOT = 3
NPRE = 38


def _layernorm(x):
    m = jnp.mean(x, axis=-1, keepdims=True)
    xc = x - m
    v = jnp.mean(xc * xc, axis=-1, keepdims=True)
    return xc * lax.rsqrt(v + 1e-5)


def _pack(w):
    return pltpu.bitcast(w, U32)


def _unpack(w):
    return pltpu.bitcast(w, BF16)


def _kernel(
    x_hbm, x4_hbm, mem_hbm, wq_hbm, wk_hbm, wv_hbm, wo_hbm, bw_hbm, wphi_hbm, bwo_hbm,
    out_hbm,
    xb_ref, xres_ref, xna_ref, xnb_ref, memf_ref,
    stage_ref, wo_ref, w_ref,
    bw_ref, bwo_stage_ref, bwt_ref, bwo_ref,
    kv_ref, z_ref, xsel_ref, xseln_ref, pre_ref, mem_ref, wphi_ref, wrep_ref, row_ref,
    wsem, wosem, sem, osem,
    *, seg, dh, hb,
):
    S, D = xres_ref.shape
    M = mem_ref.shape[0]
    L = M + seg
    nseg = S // seg
    PW = 2 * dh
    npair = w_ref.shape[0]
    HL = LANES // 2
    mixed = [h * dh + r for r in range(0, dh, HL) for h in range(2)]
    fb = D // hb
    GR = 2 * fb
    HR = D // 2
    NG = HR // GR
    NTILE = 2 * HR // LANES
    spans = []
    for i in range(NTILE):
        lo = (i * LANES) // (2 * GR)
        hi = ((i + 1) * LANES - 1) // (2 * GR) + 1
        spans.append((lo * GR, hi * GR))
    offs = [0]
    for lo, hi in spans:
        offs.append(offs[-1] + hi - lo)

    XH = (A_UNROLL[True] + 2) * seg

    def wcopy(j, t):
        rows = pl.ds(pl.multiple_of(j * PW, PW), PW)
        return pltpu.make_async_copy(
            (wq_hbm, wk_hbm, wv_hbm)[t].at[rows, :],
            stage_ref.at[j % NSLOT, t], wsem.at[j % NSLOT, t])

    def ocopy(j):
        rows = pl.ds(pl.multiple_of(j * PW, PW), PW)
        return pltpu.make_async_copy(
            wo_hbm.at[rows, :], wo_ref.at[rows, :], wosem.at[j % 8])

    def keep_wo(j):
        w = jnp.concatenate(
            [wo_ref[pl.ds(pl.multiple_of(j * PW + r, HL), HL), :] for r in mixed],
            axis=0)
        w_ref[j, D // 2:D // 2 + dh, 0:D] = _pack(w)

    def start_pair(j):
        for t in range(3):
            wcopy(j, t).start()

    xsel_copy = pltpu.make_async_copy(
        x4_hbm.at[0:NPRE, seg // 8 - 1], xsel_ref, sem.at[0])
    bw_copy = pltpu.make_async_copy(bw_hbm, bw_ref, sem.at[1])
    bwo_copy = pltpu.make_async_copy(bwo_hbm, bwo_stage_ref, sem.at[2])
    xh_copy = pltpu.make_async_copy(
        x_hbm.at[0:XH, :], xb_ref.at[0:XH, :], sem.at[3])
    xt_copy = pltpu.make_async_copy(
        x_hbm.at[XH:S, :], xb_ref.at[XH:S, :], sem.at[3])
    mem_copy = pltpu.make_async_copy(mem_hbm, mem_ref, sem.at[5])
    wphi_copy = pltpu.make_async_copy(wphi_hbm, wphi_ref, sem.at[4])
    wphi_copy.start()
    xsel_copy.start()
    xh_copy.start()
    start_pair(0)

    wphi_copy.wait()
    hh = lax.broadcasted_iota(jnp.int32, (hb, D), 0)
    cc = lax.broadcasted_iota(jnp.int32, (hb, D), 1)

    def spread(i, wcat):
        for d in range(4):
            sel = jnp.where(cc == hh * fb + (4 * i + d), 1.0, 0.0).astype(BF16)
            wcat += jnp.dot(wphi_ref[4 * i + d], sel, preferred_element_type=F32)
        return wcat

    wcat = lax.fori_loop(0, fb // 4, spread, jnp.zeros((fb, D), F32))
    rr = lax.broadcasted_iota(jnp.int32, (GR, fb), 0)
    ff = lax.broadcasted_iota(jnp.int32, (GR, fb), 1)
    twice = jnp.where((rr >> 1) == ff, 1.0, 0.0).astype(BF16)
    wrep_ref[...] = jnp.dot(twice, wcat.astype(BF16), preferred_element_type=F32)

    xsel_copy.wait()
    xsel = xsel_ref[...].astype(F32).reshape(NPRE * 8, D)
    xseln_ref[...] = _pack(_layernorm(xsel).astype(BF16))
    xh_copy.wait()
    xna_ref[0:seg, :] = _layernorm(xb_ref[0:seg, :].astype(F32))

    def load_pair(j, c):
        slot = j % NSLOT
        for t in range(3):
            wcopy(j, t).wait()

        @pl.when(j == 0)
        def _():
            start_pair(1)
            mem_copy.start()

        @pl.when(j + 2 < npair)
        def _():
            start_pair(j + 2)

        @pl.when(j >= OLAG)
        def _():
            ocopy(j - OLAG).start()

        @pl.when(j >= npair - OLAG)
        def _():
            ocopy(j).start()

        @pl.when(j >= OLAG + 2)
        def _():
            ocopy(j - OLAG - 2).wait()

        keep_wo(jnp.where(j >= OLAG + 2, j - OLAG - 2, npair - 1))
        for t in range(3):
            cols = slice(t * PW, (t + 1) * PW)
            w = jnp.concatenate(
                [stage_ref[slot, t, r:r + HL, :]
                 for r in (mixed if t == 2 else range(0, PW, HL))], axis=0)
            w_ref[j, 0:D // 2, cols] = _pack(w.astype(F32).T.astype(BF16))
            xn = _unpack(xseln_ref[...])
            if t == 0:
                y = lax.dot_general(
                    xn, stage_ref[slot, t], NT, preferred_element_type=F32)
            else:
                y = jnp.dot(xn, _unpack(w_ref[j, 0:D // 2, cols]),
                            preferred_element_type=F32)
            pre_ref[j, :, cols] = y
        return c

    lax.fori_loop(0, npair, load_pair, 0)
    mem_copy.wait()

    @pl.loop(npair - OLAG - 2, npair)
    def _(j):
        ocopy(j).wait()
        keep_wo(j)

    xt_copy.start()
    bw_copy.start()
    bwo_copy.start()

    def b_weights():
        bw_copy.wait()
        bwo_copy.wait()
        rr = lax.broadcasted_iota(jnp.int32, (GR, LANES), 0)
        cc = lax.broadcasted_iota(jnp.int32, (GR, LANES), 1) - (rr & 1) * fb
        for t in range(2):
            parts = [None] * (D // GR)
            for n in range(D // LANES):
                lo = (n * LANES) // GR
                hi = ((n + 1) * LANES - 1) // GR + 1
                col = cc + n * LANES
                lhs = jnp.concatenate([
                    jnp.where((col >= g * GR) & (col < g * GR + fb),
                              wrep_ref[:, n * LANES:(n + 1) * LANES], 0.0)
                    for g in range(lo, hi)
                ], axis=0)
                y = lax.dot_general(
                    lhs, bw_ref[:, t * D + n * LANES:t * D + (n + 1) * LANES], NT,
                    preferred_element_type=F32)
                for g in range(lo, hi):
                    piece = y[(g - lo) * GR:(g - lo + 1) * GR]
                    parts[g] = piece if parts[g] is None else parts[g] + piece
            w = jnp.concatenate(parts, axis=0) * LOG2E
            bwt_ref[t] = _pack(w.astype(BF16))
        bwt_ref[2] = _pack(bw_ref[:, 2 * D:3 * D].T)
        bwo_ref[...] = _pack(bwo_stage_ref[...])

    def a_step(short, s, mem, u):
        rows = pl.ds(pl.multiple_of(s * seg, seg), seg)
        sub = lax.broadcasted_iota(jnp.int32, (8, LANES), 0)
        lane = lax.broadcasted_iota(jnp.int32, (8, LANES), 1)
        is_a = lane < L
        col = jnp.where(is_a, lane, lane - L)
        low = lane < HL
        lows = lax.broadcasted_iota(jnp.int32, (L, LANES), 1) < HL
        scale = jnp.where(
            lax.broadcasted_iota(jnp.int32, (L, PW), 1) + s >= 0,
            dh ** -0.5 * LOG2E, 0.0)
        never = lane + s < 0
        early = [int(n) for n in NSCORE[short][u]]
        due = []

        def pin(lhs):
            if not due:
                return lhs
            top = lhs[:8, :LANES]
            while due:
                top = jnp.where(never, due.pop(), top)
            top = jnp.concatenate([top, lhs[:8, LANES:]], axis=1)
            return jnp.concatenate([top, lhs[8:]], axis=0)

        def part(j, t, lo, hi, c0=0, c1=PW):
            n = seg - 8 if short else seg
            x = xna_ref[pl.ds(pl.multiple_of(s * seg, seg), n), lo:hi]
            h = pin(jnp.concatenate([mem[:, lo:hi], x], axis=0))
            w = _unpack(w_ref[j, lo // 2:hi // 2, t * PW + c0:t * PW + c1])
            return jnp.dot(h.astype(BF16) if short else h, w,
                           preferred_element_type=F32)

        def proj(j, t, y):
            if short:
                tail = pl.ds(pl.multiple_of(s * 8, 8), 8)
                y = jnp.concatenate(
                    [y, pre_ref[j, tail, t * PW:(t + 1) * PW]], axis=0)
            if t == 0:
                return y * scale
            for b in range(early[j]):
                n = M + 8 * b + 8
                row_ref[j, 2 * b + t - 1, 0:n, :] = y[:n]
            return y

        def spread_row(j, n, r, c):
            return jnp.broadcast_to(
                row_ref[j, n, r:r + 1, c * LANES:(c + 1) * LANES], (8, LANES))

        def stack(top, bot):
            pad = jnp.zeros((LANES - 2 * L, PW), F32)
            return jnp.concatenate([top, bot, pad], axis=0).astype(BF16)

        def keys(k):
            zero = jnp.zeros((L, LANES), F32)
            mid = k[:, LANES:2 * LANES]
            return stack(
                jnp.concatenate(
                    [k[:, :LANES], jnp.where(lows, mid, 0.0), zero], axis=1),
                jnp.concatenate(
                    [zero, jnp.where(lows, 0.0, mid), k[:, 2 * LANES:]], axis=1))

        def values(v):
            first = jnp.concatenate([lows] * 3, axis=1)
            return stack(jnp.where(first, v, 0.0), jnp.where(first, 0.0, v))

        def softmax(sc, row):
            inside = col < L
            vis = inside if row < M else col <= sub + row
            sc = jnp.where(vis, sc, jnp.where(inside, MASKED, -jnp.inf))
            ma = jnp.max(jnp.where(is_a, sc, -jnp.inf), axis=1, keepdims=True)
            mb = jnp.max(jnp.where(is_a, -jnp.inf, sc), axis=1, keepdims=True)
            e = jnp.exp2(sc - jnp.where(is_a, ma, mb))
            la = jnp.sum(jnp.where(is_a, e, 0.0), axis=1, keepdims=True)
            lb = jnp.sum(jnp.where(is_a, 0.0, e), axis=1, keepdims=True)
            return e * (1.0 / jnp.where(is_a, la, lb))

        def vpu_scores(j, q, out):
            for b in range(early[j]):
                row = M + 8 * b
                mid = q[row:row + 8, LANES:2 * LANES]
                qa, qb = jnp.where(low, mid, 0.0), jnp.where(low, 0.0, mid)
                scores, top = [], None
                for r in range(row + 8):
                    k0, k1, k2 = (spread_row(j, 2 * b, r, c) for c in range(3))
                    x = jnp.where(
                        low,
                        jnp.sum(q[row:row + 8, :LANES] * k0 + qa * k1,
                                axis=1, keepdims=True),
                        jnp.sum(q[row:row + 8, 2 * LANES:] * k2 + qb * k1,
                                axis=1, keepdims=True))
                    if r > row:
                        x = jnp.where(sub >= r - row, x, MASKED)
                    top = x if top is None else jnp.maximum(top, x)
                    scores.append(x)
                    if r == row + 7:
                        out.append((scores, top))
                    if r % 8 == 7:
                        yield [top]

        def vpu_mix(j, scores, out):
            for b in range(early[j]):
                acc = None
                for r, x in enumerate(scores[b][0]):
                    e = jnp.exp2(x - scores[b][1])
                    t = [e * spread_row(j, 2 * b + 1, r, c) for c in range(3)] + [e]
                    acc = t if acc is None else [x + y for x, y in zip(acc, t)]
                    if r == M + 8 * b + 7:
                        inv = 1.0 / acc[3]
                        out.append(
                            jnp.concatenate([x * inv for x in acc[:3]], axis=1))
                    if r % 8 == 7:
                        yield acc[:3]

        def probs(j, q, k):
            far = M + 8 * early[j]
            sc = lax.dot_general(
                jnp.concatenate([q[:M], q[far:]], axis=0), keys(k), NT,
                preferred_element_type=F32)
            return jnp.concatenate([
                softmax(sc[8 * n:8 * n + 8], row)
                for n, row in enumerate([0] + list(range(far, L, 8)))
            ], axis=0)

        prv = pl.ds(pl.multiple_of(jnp.maximum(s - 1, 0) * seg, seg), seg)
        nxt = pl.ds(pl.multiple_of(jnp.minimum(s + 1, nseg - 1) * seg, seg), seg)
        if short:
            far = jnp.where(s < A_UNROLL[True], s, nseg - 1 + A_UNROLL[True] - s)
            far = jnp.where(far < NPRE, s, far)
            far = pl.ds(pl.multiple_of(far * seg, seg), seg)
            xres_ref[far, :] = xb_ref[far, :].astype(F32)
        xnb_ref[prv, :] = _layernorm(xres_ref[prv, :]).astype(BF16)
        xin_ref = xb_ref if short else xres_ref
        xn_next = _layernorm(xin_ref[nxt, :].astype(F32))

        qkv, p, o, tiles = ({}, {}, {}), {}, {}, {}
        scored = [[] for _ in range(npair)]
        mixed_rows = [[] for _ in range(npair)]
        work = {}
        acc = [None] * (D // LANES)
        heads = [part(0, t, 0, PW) for t in (1, 0)] if u > 0 else []

        def piece(op, j):
            if (op, j) not in work:
                work[op, j] = (
                    vpu_scores(j, qkv[0][j], scored[j]) if op == "w"
                    else vpu_mix(j, scored[j], mixed_rows[j]))
            return next(work[op, j], None)

        for op, j in ((t[0], int(t[1:])) for t in SCHED[short][u].split()):
            if op in "qkv":
                t = "qkv".index(op)
                if heads:
                    y = part(j, t, PW, D) + heads.pop(0)
                else:
                    y = part(j, t, 0, D)
                qkv[t][j] = proj(j, t, y)
            elif op in "QKV":
                t = "QKV".index(op)
                done = tiles.setdefault((op, j), [])
                c = len(done) * LANES
                done.append(part(j, t, 0, D, c, c + LANES))
                if len(done) == 3:
                    qkv[t][j] = proj(j, t, jnp.concatenate(done, axis=1))
            elif op in "wm":
                due.extend(piece(op, j) or [])
            elif op == "s":
                p[j] = probs(j, qkv[0][j], qkv[1][j])
            elif op == "p":
                o[j] = jnp.dot(
                    p[j], values(qkv[2][j]), preferred_element_type=F32)
                if j == npair - 1:
                    xna_ref[nxt, :] = xn_next
            else:
                for rest in "wm":
                    while piece(rest, j):
                        pass
                if op == "O":
                    lo = tiles.get((op, j), 0)
                    hi = tiles[op, j] = lo + 1
                else:
                    lo, hi = {"a": (0, 3), "b": (3, 5), "o": (0, 5)}[op]
                lhs = jnp.concatenate(
                    [o[j][:M]] + mixed_rows[j] + [o[j][M:]], axis=0)
                w = _unpack(w_ref[j, D // 2:D // 2 + dh, lo * LANES:hi * LANES])
                y = jnp.dot(pin(lhs), w, preferred_element_type=F32)
                for n in range(lo, hi):
                    t = y[:, (n - lo) * LANES:(n - lo + 1) * LANES]
                    acc[n] = t if acc[n] is None else acc[n] + t
        acc = jnp.concatenate(acc, axis=1)
        xres_ref[rows, :] = xin_ref[rows, :].astype(F32) + acc[M:]
        return acc[:M]

    def a_steps(short, i, c):
        if short:
            pl.when(i == 1)(xt_copy.wait)
        mem = memf_ref[...]
        n = A_UNROLL[short]
        for u in range(n):
            mem = a_step(short, i * n + u, mem, u)
        memf_ref[...] = mem
        return c

    def layer_a(n):
        memf_ref[...] = mem_ref[...].astype(F32)
        lax.fori_loop(0, jnp.where(n == 0, NPRE // A_UNROLL[True], 0),
                      functools.partial(a_steps, True), 0)
        lax.fori_loop(jnp.where(n == 0, NPRE // A_UNROLL[False], 0),
                      nseg // A_UNROLL[False],
                      functools.partial(a_steps, False), 0)

    def b_proj(t, half, rows):
        w = _unpack(bwt_ref[t, half * (HR // 2):(half + 1) * (HR // 2), :])
        return lax.dot_general(
            w, xnb_ref[rows, :], NT, preferred_element_type=F32)

    def fold(vals, op):
        r = functools.reduce(op, vals)
        r = op(r, pltpu.roll(r, 4, 0))
        return op(r, pltpu.roll(r, 2, 0))

    def exps(a, g):
        slabs = [a[g * GR + 8 * i:g * GR + 8 * i + 8] for i in range(GR // 8)]
        mx = fold(slabs, jnp.maximum)
        mn = fold(slabs, jnp.minimum)
        ep = [jnp.exp2(u - mx) for u in slabs]
        en = [jnp.exp2(mn - u) for u in slabs]
        return ep, en, fold(ep, jnp.add), fold(en, jnp.add)

    def b_pass1(i, c):
        rows = pl.ds(pl.multiple_of(i * TB, TB), TB)

        def features(half):
            a = b_proj(1, half, rows)
            phi = []
            for g in range(NG):
                ep, en, sp, sn = exps(a, g)
                inv = 1.0 / (sp * sn)
                ip, im = sn * inv, sp * inv
                phi += [e * ip for e in ep] + [e * im for e in en]
            phi = jnp.concatenate(phi, axis=0)
            zsum = phi[:, :LANES]
            for n in range(1, TB // LANES):
                zsum = zsum + phi[:, n * LANES:(n + 1) * LANES]
            return phi.astype(BF16), zsum

        def outer(half, vt, phi):
            for n, (lo, hi) in enumerate(spans):
                y = lax.dot_general(
                    vt[lo:hi], phi[n * LANES:(n + 1) * LANES], NT,
                    preferred_element_type=F32)
                r = lax.broadcasted_iota(jnp.int32, (hi - lo, LANES), 0) + lo
                f = lax.broadcasted_iota(jnp.int32, (1, LANES), 1) + n * LANES
                first = (f & 1) * fb
                for g in range(lo // GR, hi // GR):
                    first = jnp.where(f >= g * 2 * GR, g * GR + (f & 1) * fb, first)
                keep = (r >= first) & (r < first + fb)
                blk = slice(offs[n], offs[n + 1])
                old = jnp.where(i > 0, kv_ref[half, blk, :], 0.0)
                kv_ref[half, blk, :] = jnp.where(keep, old + y, 0.0)

        phi0, z0 = features(0)
        phi1, z1 = features(1)
        for half, z in enumerate((z0, z1)):
            z_ref[half] = jnp.where(i > 0, z_ref[half], 0.0) + z
        vt0 = b_proj(2, 0, rows)
        vt1 = b_proj(2, 1, rows)
        outer(0, vt0, phi0)
        outer(1, vt1, phi1)
        xnb_ref[S - seg:S, :] = _layernorm(xres_ref[S - seg:S, :]).astype(BF16)
        return c

    def b_pass2(i, c):
        tu = TB // 2

        def unit_rows(u):
            return pl.ds(pl.multiple_of(i * TB + u * tu, tu), tu)

        def features(u, half):
            a = b_proj(0, half, unit_rows(u))
            phi = []
            for g in range(NG):
                ep, en, sp, sn = exps(a, g)

                def zdot(es, base):
                    terms = []
                    for n, e in enumerate(es):
                        z = z_ref[half, base + 8 * n:base + 8 * n + 8, :]
                        terms.append(e * jnp.concatenate([z] * (tu // LANES), axis=1))
                    return functools.reduce(jnp.add, terms)

                den = zdot(ep, 2 * GR * g) * sn + zdot(en, 2 * GR * g + GR) * sp
                inv = 1.0 / (fold([den], jnp.add) + 1e-6 * (sp * sn))
                ip, im = sn * inv, sp * inv
                phi += [e * ip for e in ep] + [e * im for e in en]
            return jnp.concatenate(phi, axis=0).astype(BF16)

        def mix(half, phi):
            parts = [None] * NG
            for n, (lo, hi) in enumerate(spans):
                y = jnp.dot(
                    kv_ref[half, offs[n]:offs[n + 1], :],
                    phi[n * LANES:(n + 1) * LANES], preferred_element_type=F32)
                for g in range(lo // GR, hi // GR):
                    piece = y[g * GR - lo:(g + 1) * GR - lo]
                    parts[g] = piece if parts[g] is None else parts[g] + piece
            return jnp.concatenate(parts, axis=0)

        def finish(u, cols, o):
            rows = unit_rows(u)
            y = jnp.dot(o, _unpack(bwo_ref[:, cols]), preferred_element_type=F32)
            y = xres_ref[rows, cols] + y
            xres_ref[rows, cols] = y
            xb_ref[rows, cols] = y.astype(BF16)
            return y[:seg]

        phi, ot, o = {}, {}, {}
        for op in P2.split():
            u = int(op[1])
            if op[0] == "f":
                phi[op[1:]] = features(u, int(op[2]))
            elif op[0] == "m":
                ot[op[1:]] = mix(int(op[2]), phi.pop(op[1:]))
                if op[2] == "1":
                    o[u] = jnp.concatenate(
                        [ot.pop(op[1] + "0"), ot.pop(op[1:])], axis=0).T
            else:
                cols = slice(0, PW) if op[0] == "a" else slice(PW, D)
                ot[op] = finish(u, cols, o[u])
                if op[0] == "b":
                    pltpu.make_async_copy(
                        xb_ref.at[unit_rows(u), :], out_hbm.at[unit_rows(u), :],
                        osem).start()
        xna_ref[pl.ds(pl.multiple_of(i * TB, TB), seg), :] = _layernorm(
            jnp.concatenate([ot["a0"], ot["b0"]], axis=1))
        return c

    nblk = S // TB
    out_copy = pltpu.make_async_copy(xb_ref, out_hbm, osem)

    def layer(n, c):
        layer_a(n)
        pl.when(n == 0)(b_weights)
        lax.fori_loop(0, nblk, b_pass1, 0)
        z_ref[...] = jnp.broadcast_to(
            jnp.sum(z_ref[...], axis=2, keepdims=True), z_ref.shape)
        pl.when(n == 1)(out_copy.wait)
        lax.fori_loop(0, nblk, b_pass2, 0)
        return c

    lax.fori_loop(0, 2, layer, 0)
    out_copy.wait()


@functools.partial(jax.jit, static_argnames=("A_seg_len",))
def pallas_interleave_layers__memory_aug_recurrent_mem_tr__linear_kernel_hedgehog__prompt_kernel(
    A_x: jax.Array,
    A_mem0: jax.Array,
    A_Wq: jax.Array,
    A_Wk: jax.Array,
    A_Wv: jax.Array,
    A_Wo: jax.Array,
    A_seg_len: int,
    B_x: jax.Array,
    B_wqkv: jax.Array,
    B_w_phi: jax.Array,
    B_wo: jax.Array,
):
    del B_x
    _, S, D = A_x.shape
    M = A_mem0.shape[1]
    _, H, dh = A_Wq.shape
    hb = B_w_phi.shape[0]
    seg = int(A_seg_len)
    npair, PW = H // 2, 2 * dh
    assert A_x.shape[0] == 1 and PW == 3 * LANES and 2 * (M + seg) <= LANES
    assert (2 * NPRE - A_UNROLL[True]) * seg >= S and D == 5 * LANES and hb == 32 and S % TB == 0

    def rows_first(w):
        return jnp.transpose(w, (1, 2, 0)).reshape(H * dh, D)

    hbm = pl.BlockSpec(memory_space=pl.ANY)
    out = pl.pallas_call(
        functools.partial(_kernel, seg=seg, dh=dh, hb=hb),
        out_shape=jax.ShapeDtypeStruct((S, D), BF16),
        in_specs=[hbm] * 10,
        out_specs=hbm,
        scratch_shapes=[
            pltpu.VMEM((S, D), BF16),
            pltpu.VMEM((S, D), F32),
            pltpu.VMEM((S, D), F32),
            pltpu.VMEM((S, D), BF16),
            pltpu.VMEM((M, D), F32),
            pltpu.VMEM((NSLOT, 3, PW, D), BF16),
            pltpu.VMEM((H * dh, D), BF16),
            pltpu.VMEM((npair, D // 2 + dh, 3 * PW), U32),
            pltpu.VMEM((D, 3 * D), BF16),
            pltpu.VMEM((D, D), BF16),
            pltpu.VMEM((3, D // 2, D), U32),
            pltpu.VMEM((D // 2, D), U32),
            pltpu.VMEM((2, 480, LANES), F32),
            pltpu.VMEM((2, D, LANES), F32),
            pltpu.VMEM((NPRE, 8, D), BF16),
            pltpu.VMEM((NPRE * 4, D), U32),
            pltpu.VMEM((npair, NPRE * 8, 3 * PW), F32),
            pltpu.VMEM((M, D), BF16),
            pltpu.VMEM((D // hb, D // hb, hb), BF16),
            pltpu.VMEM((2 * D // hb, D), F32),
            pltpu.VMEM((npair, 4, M + 16, PW), F32),
            pltpu.SemaphoreType.DMA((NSLOT, 3)),
            pltpu.SemaphoreType.DMA((8,)),
            pltpu.SemaphoreType.DMA((6,)),
            pltpu.SemaphoreType.DMA,
        ],
        compiler_params=pltpu.CompilerParams(
            vmem_limit_bytes=112 * 1024 * 1024, disable_bounds_checks=NOBC),
    )(
        A_x.reshape(S, D),
        A_x.reshape(S // seg, seg // 8, 8, D),
        A_mem0.reshape(M, D),
        rows_first(A_Wq),
        rows_first(A_Wk),
        rows_first(A_Wv),
        A_Wo.reshape(H * dh, D),
        B_wqkv,
        jnp.transpose(B_w_phi, (1, 2, 0)),
        B_wo,
    )
    return out.reshape(1, S, D)
```

```python
import functools

import jax
import jax.numpy as jnp
from jax import lax
import jax.experimental.pallas as pl
import jax.experimental.pallas.tpu as pltpu

F32 = jnp.float32
BF16 = jnp.bfloat16
U32 = jnp.uint32
LOG2E = 1.4426950408889634
NT = (((1,), (1,)), ((), ()))
LANES = 128
MASKED = -1e9 * LOG2E

NPRE = 38
NSLOT = 3
OLAG = 2
UNROLL = 2
TB = 512


def _full_order(ranges):
    first, second, rest = (
        "sKKKQQwQwVwVwVwp", "swKmmKKwQmwQwQmVmVVpw", "sKKwKmmQwOQmOQwVmOwmVVOpw")
    order, n = ["k0", "q0", "v0"], 0
    for j in range(15):
        for c in first if j == 0 else second if j == 1 else rest:
            pair = {"s": j, "p": j, "w": j, "m": j - 1, "O": n // 5}.get(c, j + 1)
            order.append(f"{c}{pair}")
            n += c == "O"
    order.append("s15")
    for i in range(14):
        order += ["m14"] * (i % 3 == 0) + [f"O{(n + i) // 5}"]
    return " ".join(order + ["p15 O13 O13 O13 O13", ranges])


FULL_ORDER = (_full_order("a14 a15 b14 b15"), _full_order("o14 o15"))
SHORT_ORDER = (
    "k0 q0 v0 s0 k1 q1 v1 k2 p0 v2 b0 s1 q2 k3 v3 q3 p1 a0 s2 k4 a1 q4 v4 p2 s3 "
    "k5 a2 q5 v5 p3 s4 k6 v6 a3 q6 s5 p4 k7 a4 q7 v7 p5 s6 k8 a5 q8 v8 p6 s7 v9 "
    "k9 a6 q9 p7 s8 q10 k10 a7 v10 p8 s9 k11 a8 q11 v11 p9 s10 k12 a9 q12 v12 "
    "p10 s11 k13 q13 a10 v13 p11 s12 k14 a11 v14 q14 p12 s13 k15 a12 v15 q15 "
    "p13 s14 b2 s15 b8 b4 b5 b3 b1 p14 a13 b6 b7 b10 b9 a14 p15 b11 b12 a15 b13 "
    "b14 b15",
    "k0 q0 v0 s0 k1 q1 v1 k2 p0 v2 s1 q2 k3 b0 v3 q3 p1 a0 s2 k4 a1 q4 v4 p2 s3 "
    "k5 a2 q5 v5 p3 s4 v6 k6 a3 q6 p4 s5 k7 a4 q7 v7 p5 s6 k8 a5 q8 v8 p6 s7 v9 "
    "k9 a6 q9 p7 s8 q10 k10 a7 v10 p8 s9 k11 q11 a8 v11 p9 s10 v12 k12 a9 q12 "
    "p10 s11 k13 q13 a10 v13 p11 s12 k14 a11 q14 v14 p12 s13 k15 a12 v15 q15 "
    "p13 s14 b2 s15 b8 b4 b1 b5 b3 p14 b6 b12 b10 b7 a13 b9 a14 p15 b11 b13 a15 "
    "b14 b15",
)
FULL_EARLY = ('2222222212222200', '2222222222222210')
SHORT_EARLY = ('0111101111110000', '0101101101110111')
B_ORDER = "f00 f01 f10 f11 m00 m01 m10 a0 m11 b0 a1 b1"


def _layernorm(x):
    m = jnp.mean(x, axis=-1, keepdims=True)
    xc = x - m
    v = jnp.mean(xc * xc, axis=-1, keepdims=True)
    return xc * lax.rsqrt(v + 1e-5)


def _pack(w):
    return pltpu.bitcast(w, U32)


def _unpack(w):
    return pltpu.bitcast(w, BF16)


def _kernel(
    x_hbm, x4_hbm, mem_hbm, wq_hbm, wk_hbm, wv_hbm, wo_hbm,
    bw_hbm, wphi_hbm, bwo_hbm,
    out_hbm,
    xb_ref, xres_ref, xna_ref, xnb_ref, memf_ref,
    stage_ref, wo_ref, w_ref,
    bw_ref, bwo_stage_ref, bwt_ref, bwo_ref,
    kv_ref, z_ref, xsel_ref, xseln_ref, pre_ref,
    mem_ref, wphi_ref, wrep_ref, row_ref,
    wsem, wosem, sem, osem,
    *, seg, dh, hb,
):
    S, D = xres_ref.shape
    M = mem_ref.shape[0]
    L = M + seg
    nseg = S // seg
    PW = 2 * dh
    npair = w_ref.shape[0]
    HL = LANES // 2
    mixed = [h * dh + r for r in range(0, dh, HL) for h in range(2)]
    fb = D // hb
    GR = 2 * fb
    HR = D // 2
    NG = HR // GR
    NTILE = 2 * HR // LANES
    spans = []
    for i in range(NTILE):
        lo = (i * LANES) // (2 * GR)
        hi = ((i + 1) * LANES - 1) // (2 * GR) + 1
        spans.append((lo * GR, hi * GR))
    offs = [0]
    for lo, hi in spans:
        offs.append(offs[-1] + hi - lo)

    XH = (UNROLL + 2) * seg

    def wcopy(j, t):
        rows = pl.ds(pl.multiple_of(j * PW, PW), PW)
        return pltpu.make_async_copy(
            (wq_hbm, wk_hbm, wv_hbm)[t].at[rows, :],
            stage_ref.at[j % NSLOT, t], wsem.at[j % NSLOT, t])

    def ocopy(j):
        rows = pl.ds(pl.multiple_of(j * PW, PW), PW)
        return pltpu.make_async_copy(
            wo_hbm.at[rows, :], wo_ref.at[rows, :], wosem.at[j % 8])

    def keep_wo(j):
        w = jnp.concatenate(
            [wo_ref[pl.ds(pl.multiple_of(j * PW + r, HL), HL), :] for r in mixed],
            axis=0)
        w_ref[j, D // 2:D // 2 + dh, 0:D] = _pack(w)

    def start_pair(j):
        for t in range(3):
            wcopy(j, t).start()

    xsel_copy = pltpu.make_async_copy(
        x4_hbm.at[0:NPRE, seg // 8 - 1], xsel_ref, sem.at[0])
    bw_copy = pltpu.make_async_copy(bw_hbm, bw_ref, sem.at[1])
    bwo_copy = pltpu.make_async_copy(bwo_hbm, bwo_stage_ref, sem.at[2])
    xh_copy = pltpu.make_async_copy(
        x_hbm.at[0:XH, :], xb_ref.at[0:XH, :], sem.at[3])
    xt_copy = pltpu.make_async_copy(
        x_hbm.at[XH:S, :], xb_ref.at[XH:S, :], sem.at[3])
    mem_copy = pltpu.make_async_copy(mem_hbm, mem_ref, sem.at[5])
    wphi_copy = pltpu.make_async_copy(wphi_hbm, wphi_ref, sem.at[4])
    wphi_copy.start()
    xsel_copy.start()
    xh_copy.start()
    start_pair(0)

    wphi_copy.wait()
    hh = lax.broadcasted_iota(jnp.int32, (hb, D), 0)
    cc = lax.broadcasted_iota(jnp.int32, (hb, D), 1)

    def spread(i, wcat):
        for d in range(4):
            sel = jnp.where(cc == hh * fb + (4 * i + d), 1.0, 0.0).astype(BF16)
            wcat += jnp.dot(wphi_ref[4 * i + d], sel, preferred_element_type=F32)
        return wcat

    wcat = lax.fori_loop(0, fb // 4, spread, jnp.zeros((fb, D), F32))
    rr = lax.broadcasted_iota(jnp.int32, (GR, fb), 0)
    ff = lax.broadcasted_iota(jnp.int32, (GR, fb), 1)
    twice = jnp.where((rr >> 1) == ff, 1.0, 0.0).astype(BF16)
    wrep_ref[...] = jnp.dot(twice, wcat.astype(BF16), preferred_element_type=F32)

    xsel_copy.wait()
    xsel = xsel_ref[...].astype(F32).reshape(NPRE * 8, D)
    xseln_ref[...] = _pack(_layernorm(xsel).astype(BF16))
    xh_copy.wait()
    xna_ref[0:seg, :] = _layernorm(xb_ref[0:seg, :].astype(F32))

    def load_pair(j, c):
        slot = j % NSLOT
        for t in range(3):
            wcopy(j, t).wait()

        @pl.when(j == 0)
        def _():
            start_pair(1)
            mem_copy.start()

        @pl.when(j + NSLOT - 1 < npair)
        def _():
            start_pair(j + NSLOT - 1)

        @pl.when(j >= OLAG)
        def _():
            ocopy(j - OLAG).start()

        @pl.when(j >= npair - OLAG)
        def _():
            ocopy(j).start()

        @pl.when(j >= OLAG + 2)
        def _():
            ocopy(j - OLAG - 2).wait()

        keep_wo(jnp.where(j >= OLAG + 2, j - OLAG - 2, npair - 1))
        for t in range(3):
            cols = slice(t * PW, (t + 1) * PW)
            w = jnp.concatenate(
                [stage_ref[slot, t, r:r + HL, :]
                 for r in (mixed if t == 2 else range(0, PW, HL))], axis=0)
            w_ref[j, 0:D // 2, cols] = _pack(w.astype(F32).T.astype(BF16))
            xn = _unpack(xseln_ref[...])
            if t == 0:
                y = lax.dot_general(
                    xn, stage_ref[slot, t], NT, preferred_element_type=F32)
            else:
                y = jnp.dot(xn, _unpack(w_ref[j, 0:D // 2, cols]),
                            preferred_element_type=F32)
            pre_ref[j, :, cols] = y
        return c

    lax.fori_loop(0, npair, load_pair, 0)
    mem_copy.wait()

    @pl.loop(npair - OLAG - 2, npair)
    def _(j):
        ocopy(j).wait()
        keep_wo(j)

    xt_copy.start()
    bw_copy.start()
    bwo_copy.start()

    def b_weights():
        bw_copy.wait()
        bwo_copy.wait()
        rr = lax.broadcasted_iota(jnp.int32, (GR, LANES), 0)
        cc = lax.broadcasted_iota(jnp.int32, (GR, LANES), 1) - (rr & 1) * fb
        for t in range(2):
            parts = [None] * (D // GR)
            for n in range(D // LANES):
                lo = (n * LANES) // GR
                hi = ((n + 1) * LANES - 1) // GR + 1
                col = cc + n * LANES
                lhs = jnp.concatenate([
                    jnp.where((col >= g * GR) & (col < g * GR + fb),
                              wrep_ref[:, n * LANES:(n + 1) * LANES], 0.0)
                    for g in range(lo, hi)
                ], axis=0)
                y = lax.dot_general(
                    lhs, bw_ref[:, t * D + n * LANES:t * D + (n + 1) * LANES], NT,
                    preferred_element_type=F32)
                for g in range(lo, hi):
                    piece = y[(g - lo) * GR:(g - lo + 1) * GR]
                    parts[g] = piece if parts[g] is None else parts[g] + piece
            w = jnp.concatenate(parts, axis=0) * LOG2E
            bwt_ref[t] = _pack(w.astype(BF16))
        bwt_ref[2] = _pack(bw_ref[:, 2 * D:3 * D].T)
        bwo_ref[...] = _pack(bwo_stage_ref[...])

    def a_step(short, s, mem, u):
        rows = pl.ds(pl.multiple_of(s * seg, seg), seg)
        sub = lax.broadcasted_iota(jnp.int32, (8, LANES), 0)
        lane = lax.broadcasted_iota(jnp.int32, (8, LANES), 1)
        is_a = lane < L
        col = jnp.where(is_a, lane, lane - L)
        low = lane < HL
        lows = lax.broadcasted_iota(jnp.int32, (L, LANES), 1) < HL
        scale = jnp.where(
            lax.broadcasted_iota(jnp.int32, (L, PW), 1) + s >= 0,
            dh ** -0.5 * LOG2E, 0.0)
        never = lane + s < 0
        early = [int(n) for n in (SHORT_EARLY if short else FULL_EARLY)[u]]
        due = []

        def pin(lhs):
            if not due:
                return lhs
            top = lhs[:8, :LANES]
            while due:
                top = jnp.where(never, due.pop(), top)
            top = jnp.concatenate([top, lhs[:8, LANES:]], axis=1)
            return jnp.concatenate([top, lhs[8:]], axis=0)

        def part(j, t, lo, hi, c0=0, c1=PW):
            n = seg - 8 if short else seg
            x = xna_ref[pl.ds(pl.multiple_of(s * seg, seg), n), lo:hi]
            h = pin(jnp.concatenate([mem[:, lo:hi], x], axis=0))
            w = _unpack(w_ref[j, lo // 2:hi // 2, t * PW + c0:t * PW + c1])
            return jnp.dot(h.astype(BF16) if short else h, w,
                           preferred_element_type=F32)

        def proj(j, t, y):
            if short:
                tail = pl.ds(pl.multiple_of(s * 8, 8), 8)
                y = jnp.concatenate(
                    [y, pre_ref[j, tail, t * PW:(t + 1) * PW]], axis=0)
            if t == 0:
                return y * scale
            for b in range(early[j]):
                n = M + 8 * b + 8
                row_ref[j, 2 * b + t - 1, 0:n, :] = y[:n]
            return y

        def spread_row(j, n, r, c):
            return jnp.broadcast_to(
                row_ref[j, n, r:r + 1, c * LANES:(c + 1) * LANES], (8, LANES))

        def stack(top, bot):
            pad = jnp.zeros((LANES - 2 * L, PW), F32)
            return jnp.concatenate([top, bot, pad], axis=0).astype(BF16)

        def keys(k):
            zero = jnp.zeros((L, LANES), F32)
            mid = k[:, LANES:2 * LANES]
            return stack(
                jnp.concatenate(
                    [k[:, :LANES], jnp.where(lows, mid, 0.0), zero], axis=1),
                jnp.concatenate(
                    [zero, jnp.where(lows, 0.0, mid), k[:, 2 * LANES:]], axis=1))

        def values(v):
            first = jnp.concatenate([lows] * 3, axis=1)
            return stack(jnp.where(first, v, 0.0), jnp.where(first, 0.0, v))

        def softmax(sc, row):
            inside = col < L
            vis = inside if row < M else col <= sub + row
            sc = jnp.where(vis, sc, jnp.where(inside, MASKED, -jnp.inf))
            ma = jnp.max(jnp.where(is_a, sc, -jnp.inf), axis=1, keepdims=True)
            mb = jnp.max(jnp.where(is_a, -jnp.inf, sc), axis=1, keepdims=True)
            e = jnp.exp2(sc - jnp.where(is_a, ma, mb))
            la = jnp.sum(jnp.where(is_a, e, 0.0), axis=1, keepdims=True)
            lb = jnp.sum(jnp.where(is_a, 0.0, e), axis=1, keepdims=True)
            return e * (1.0 / jnp.where(is_a, la, lb))

        def vpu_scores(j, q, out):
            for b in range(early[j]):
                row = M + 8 * b
                mid = q[row:row + 8, LANES:2 * LANES]
                qa, qb = jnp.where(low, mid, 0.0), jnp.where(low, 0.0, mid)
                scores, top = [], None
                for r in range(row + 8):
                    k0, k1, k2 = (spread_row(j, 2 * b, r, c) for c in range(3))
                    x = jnp.where(
                        low,
                        jnp.sum(q[row:row + 8, :LANES] * k0 + qa * k1,
                                axis=1, keepdims=True),
                        jnp.sum(q[row:row + 8, 2 * LANES:] * k2 + qb * k1,
                                axis=1, keepdims=True))
                    if r > row:
                        x = jnp.where(sub >= r - row, x, MASKED)
                    top = x if top is None else jnp.maximum(top, x)
                    scores.append(x)
                    if r == row + 7:
                        out.append((scores, top))
                    if r % 8 == 7:
                        yield [top]

        def vpu_mix(j, scores, out):
            for b in range(early[j]):
                acc = None
                for r, x in enumerate(scores[b][0]):
                    e = jnp.exp2(x - scores[b][1])
                    t = [e * spread_row(j, 2 * b + 1, r, c) for c in range(3)] + [e]
                    acc = t if acc is None else [x + y for x, y in zip(acc, t)]
                    if r == M + 8 * b + 7:
                        inv = 1.0 / acc[3]
                        out.append(
                            jnp.concatenate([x * inv for x in acc[:3]], axis=1))
                    if r % 8 == 7:
                        yield acc[:3]

        def probs(j, q, k):
            far = M + 8 * early[j]
            sc = lax.dot_general(
                jnp.concatenate([q[:M], q[far:]], axis=0), keys(k), NT,
                preferred_element_type=F32)
            return jnp.concatenate([
                softmax(sc[8 * n:8 * n + 8], row)
                for n, row in enumerate([0] + list(range(far, L, 8)))
            ], axis=0)

        prv = pl.ds(pl.multiple_of(jnp.maximum(s - 1, 0) * seg, seg), seg)
        nxt = pl.ds(pl.multiple_of(jnp.minimum(s + 1, nseg - 1) * seg, seg), seg)
        if short:
            far = jnp.where(s < UNROLL, s, nseg - 1 + UNROLL - s)
            far = jnp.where(far < NPRE, s, far)
            far = pl.ds(pl.multiple_of(far * seg, seg), seg)
            xres_ref[far, :] = xb_ref[far, :].astype(F32)
        xnb_ref[prv, :] = _layernorm(xres_ref[prv, :]).astype(BF16)
        xin_ref = xb_ref if short else xres_ref
        xn_next = _layernorm(xin_ref[nxt, :].astype(F32))

        qkv, p, o, tiles = ({}, {}, {}), {}, {}, {}
        scored = [[] for _ in range(npair)]
        mixed_rows = [[] for _ in range(npair)]
        work = {}
        acc = [None] * (D // LANES)
        heads = [part(0, t, 0, PW) for t in (1, 0)] if u > 0 else []

        def piece(op, j):
            if (op, j) not in work:
                work[op, j] = (
                    vpu_scores(j, qkv[0][j], scored[j]) if op == "w"
                    else vpu_mix(j, scored[j], mixed_rows[j]))
            return next(work[op, j], None)

        order = (SHORT_ORDER if short else FULL_ORDER)[u]
        for op, j in ((t[0], int(t[1:])) for t in order.split()):
            if op in "qkv":
                t = "qkv".index(op)
                if heads:
                    y = part(j, t, PW, D) + heads.pop(0)
                else:
                    y = part(j, t, 0, D)
                qkv[t][j] = proj(j, t, y)
            elif op in "QKV":
                t = "QKV".index(op)
                done = tiles.setdefault((op, j), [])
                c = len(done) * LANES
                done.append(part(j, t, 0, D, c, c + LANES))
                if len(done) == 3:
                    qkv[t][j] = proj(j, t, jnp.concatenate(done, axis=1))
            elif op in "wm":
                due.extend(piece(op, j) or [])
            elif op == "s":
                p[j] = probs(j, qkv[0][j], qkv[1][j])
            elif op == "p":
                o[j] = jnp.dot(
                    p[j], values(qkv[2][j]), preferred_element_type=F32)
                if j == npair - 1:
                    xna_ref[nxt, :] = xn_next
            else:
                for rest in "wm":
                    while piece(rest, j):
                        pass
                if op == "O":
                    lo = tiles.get((op, j), 0)
                    hi = tiles[op, j] = lo + 1
                else:
                    lo, hi = {"a": (0, 3), "b": (3, 5), "o": (0, 5)}[op]
                lhs = jnp.concatenate(
                    [o[j][:M]] + mixed_rows[j] + [o[j][M:]], axis=0)
                w = _unpack(w_ref[j, D // 2:D // 2 + dh, lo * LANES:hi * LANES])
                y = jnp.dot(pin(lhs), w, preferred_element_type=F32)
                for n in range(lo, hi):
                    t = y[:, (n - lo) * LANES:(n - lo + 1) * LANES]
                    acc[n] = t if acc[n] is None else acc[n] + t
        acc = jnp.concatenate(acc, axis=1)
        xres_ref[rows, :] = xin_ref[rows, :].astype(F32) + acc[M:]
        return acc[:M]

    def a_steps(short, i, c):
        if short:
            pl.when(i == 1)(xt_copy.wait)
        mem = memf_ref[...]
        for u in range(UNROLL):
            mem = a_step(short, i * UNROLL + u, mem, u)
        memf_ref[...] = mem
        return c

    def layer_a(n):
        memf_ref[...] = mem_ref[...].astype(F32)
        nshort = jnp.where(n == 0, NPRE // UNROLL, 0)
        lax.fori_loop(0, nshort, functools.partial(a_steps, True), 0)
        lax.fori_loop(nshort, nseg // UNROLL, functools.partial(a_steps, False), 0)

    def b_proj(t, half, rows):
        w = _unpack(bwt_ref[t, half * (HR // 2):(half + 1) * (HR // 2), :])
        return lax.dot_general(
            w, xnb_ref[rows, :], NT, preferred_element_type=F32)

    def fold(vals, op):
        r = functools.reduce(op, vals)
        r = op(r, pltpu.roll(r, 4, 0))
        return op(r, pltpu.roll(r, 2, 0))

    def exps(a, g):
        slabs = [a[g * GR + 8 * i:g * GR + 8 * i + 8] for i in range(GR // 8)]
        mx = fold(slabs, jnp.maximum)
        mn = fold(slabs, jnp.minimum)
        ep = [jnp.exp2(u - mx) for u in slabs]
        en = [jnp.exp2(mn - u) for u in slabs]
        return ep, en, fold(ep, jnp.add), fold(en, jnp.add)

    def b_pass1(i, c):
        rows = pl.ds(pl.multiple_of(i * TB, TB), TB)

        def features(half):
            a = b_proj(1, half, rows)
            phi = []
            for g in range(NG):
                ep, en, sp, sn = exps(a, g)
                inv = 1.0 / (sp * sn)
                ip, im = sn * inv, sp * inv
                phi += [e * ip for e in ep] + [e * im for e in en]
            phi = jnp.concatenate(phi, axis=0)
            zsum = phi[:, :LANES]
            for n in range(1, TB // LANES):
                zsum = zsum + phi[:, n * LANES:(n + 1) * LANES]
            return phi.astype(BF16), zsum

        def outer(half, vt, phi):
            for n, (lo, hi) in enumerate(spans):
                y = lax.dot_general(
                    vt[lo:hi], phi[n * LANES:(n + 1) * LANES], NT,
                    preferred_element_type=F32)
                r = lax.broadcasted_iota(jnp.int32, (hi - lo, LANES), 0) + lo
                f = lax.broadcasted_iota(jnp.int32, (1, LANES), 1) + n * LANES
                first = (f & 1) * fb
                for g in range(lo // GR, hi // GR):
                    first = jnp.where(f >= g * 2 * GR, g * GR + (f & 1) * fb, first)
                keep = (r >= first) & (r < first + fb)
                blk = slice(offs[n], offs[n + 1])
                old = jnp.where(i > 0, kv_ref[half, blk, :], 0.0)
                kv_ref[half, blk, :] = jnp.where(keep, old + y, 0.0)

        phi0, z0 = features(0)
        phi1, z1 = features(1)
        for half, z in enumerate((z0, z1)):
            z_ref[half] = jnp.where(i > 0, z_ref[half], 0.0) + z
        vt0 = b_proj(2, 0, rows)
        vt1 = b_proj(2, 1, rows)
        outer(0, vt0, phi0)
        outer(1, vt1, phi1)
        xnb_ref[S - seg:S, :] = _layernorm(xres_ref[S - seg:S, :]).astype(BF16)
        return c

    def b_pass2(i, c):
        tu = TB // 2

        def unit_rows(u):
            return pl.ds(pl.multiple_of(i * TB + u * tu, tu), tu)

        def features(u, half):
            a = b_proj(0, half, unit_rows(u))
            phi = []
            for g in range(NG):
                ep, en, sp, sn = exps(a, g)

                def zdot(es, base):
                    terms = []
                    for n, e in enumerate(es):
                        z = z_ref[half, base + 8 * n:base + 8 * n + 8, :]
                        terms.append(e * jnp.concatenate([z] * (tu // LANES), axis=1))
                    return functools.reduce(jnp.add, terms)

                den = zdot(ep, 2 * GR * g) * sn + zdot(en, 2 * GR * g + GR) * sp
                inv = 1.0 / (fold([den], jnp.add) + 1e-6 * (sp * sn))
                ip, im = sn * inv, sp * inv
                phi += [e * ip for e in ep] + [e * im for e in en]
            return jnp.concatenate(phi, axis=0).astype(BF16)

        def mix(half, phi):
            parts = [None] * NG
            for n, (lo, hi) in enumerate(spans):
                y = jnp.dot(
                    kv_ref[half, offs[n]:offs[n + 1], :],
                    phi[n * LANES:(n + 1) * LANES], preferred_element_type=F32)
                for g in range(lo // GR, hi // GR):
                    piece = y[g * GR - lo:(g + 1) * GR - lo]
                    parts[g] = piece if parts[g] is None else parts[g] + piece
            return jnp.concatenate(parts, axis=0)

        def finish(u, cols, o):
            rows = unit_rows(u)
            y = jnp.dot(o, _unpack(bwo_ref[:, cols]), preferred_element_type=F32)
            y = xres_ref[rows, cols] + y
            xres_ref[rows, cols] = y
            xb_ref[rows, cols] = y.astype(BF16)
            return y[:seg]

        phi, ot, o = {}, {}, {}
        for op in B_ORDER.split():
            u = int(op[1])
            if op[0] == "f":
                phi[op[1:]] = features(u, int(op[2]))
            elif op[0] == "m":
                ot[op[1:]] = mix(int(op[2]), phi.pop(op[1:]))
                if op[2] == "1":
                    o[u] = jnp.concatenate(
                        [ot.pop(op[1] + "0"), ot.pop(op[1:])], axis=0).T
            else:
                cols = slice(0, PW) if op[0] == "a" else slice(PW, D)
                ot[op] = finish(u, cols, o[u])
                pltpu.make_async_copy(
                    xb_ref.at[unit_rows(u), cols], out_hbm.at[unit_rows(u), cols],
                    osem).start()
        xna_ref[pl.ds(pl.multiple_of(i * TB, TB), seg), :] = _layernorm(
            jnp.concatenate([ot["a0"], ot["b0"]], axis=1))
        return c

    nblk = S // TB
    out_copy = pltpu.make_async_copy(xb_ref, out_hbm, osem)

    def layer(n, c):
        layer_a(n)
        pl.when(n == 0)(b_weights)
        lax.fori_loop(0, nblk, b_pass1, 0)
        z_ref[...] = jnp.broadcast_to(
            jnp.sum(z_ref[...], axis=2, keepdims=True), z_ref.shape)
        pl.when(n == 1)(out_copy.wait)
        lax.fori_loop(0, nblk, b_pass2, 0)
        return c

    lax.fori_loop(0, 2, layer, 0)
    out_copy.wait()


@functools.partial(jax.jit, static_argnames=("A_seg_len",))
def pallas_interleave_layers__memory_aug_recurrent_mem_tr__linear_kernel_hedgehog__prompt_kernel(
    A_x: jax.Array,
    A_mem0: jax.Array,
    A_Wq: jax.Array,
    A_Wk: jax.Array,
    A_Wv: jax.Array,
    A_Wo: jax.Array,
    A_seg_len: int,
    B_x: jax.Array,
    B_wqkv: jax.Array,
    B_w_phi: jax.Array,
    B_wo: jax.Array,
):
    del B_x
    _, S, D = A_x.shape
    M = A_mem0.shape[1]
    _, H, dh = A_Wq.shape
    hb = B_w_phi.shape[0]
    seg = int(A_seg_len)
    npair, PW = H // 2, 2 * dh
    assert (A_x.shape[0], M, seg, H, dh, D, hb) == (1, 8, 32, 32, 192, 640, 32)
    assert S % TB == 0 and NPRE * seg <= S <= (2 * NPRE - UNROLL) * seg

    def rows_first(w):
        return jnp.transpose(w, (1, 2, 0)).reshape(H * dh, D)

    hbm = pl.BlockSpec(memory_space=pl.ANY)
    out = pl.pallas_call(
        functools.partial(_kernel, seg=seg, dh=dh, hb=hb),
        out_shape=jax.ShapeDtypeStruct((S, D), BF16),
        in_specs=[hbm] * 10,
        out_specs=hbm,
        scratch_shapes=[
            pltpu.VMEM((S, D), BF16),
            pltpu.VMEM((S, D), F32),
            pltpu.VMEM((S, D), F32),
            pltpu.VMEM((S, D), BF16),
            pltpu.VMEM((M, D), F32),
            pltpu.VMEM((NSLOT, 3, PW, D), BF16),
            pltpu.VMEM((H * dh, D), BF16),
            pltpu.VMEM((npair, D // 2 + dh, 3 * PW), U32),
            pltpu.VMEM((D, 3 * D), BF16),
            pltpu.VMEM((D, D), BF16),
            pltpu.VMEM((3, D // 2, D), U32),
            pltpu.VMEM((D // 2, D), U32),
            pltpu.VMEM((2, 480, LANES), F32),
            pltpu.VMEM((2, D, LANES), F32),
            pltpu.VMEM((NPRE, 8, D), BF16),
            pltpu.VMEM((NPRE * 4, D), U32),
            pltpu.VMEM((npair, NPRE * 8, 3 * PW), F32),
            pltpu.VMEM((M, D), BF16),
            pltpu.VMEM((D // hb, D // hb, hb), BF16),
            pltpu.VMEM((2 * D // hb, D), F32),
            pltpu.VMEM((npair, 4, M + 16, PW), F32),
            pltpu.SemaphoreType.DMA((NSLOT, 3)),
            pltpu.SemaphoreType.DMA((8,)),
            pltpu.SemaphoreType.DMA((6,)),
            pltpu.SemaphoreType.DMA,
        ],
        compiler_params=pltpu.CompilerParams(
            vmem_limit_bytes=112 * 1024 * 1024, disable_bounds_checks=True),
    )(
        A_x.reshape(S, D),
        A_x.reshape(S // seg, seg // 8, 8, D),
        A_mem0.reshape(M, D),
        rows_first(A_Wq),
        rows_first(A_Wk),
        rows_first(A_Wv),
        A_Wo.reshape(H * dh, D),
        B_wqkv,
        jnp.transpose(B_w_phi, (1, 2, 0)),
        B_wo,
    )
    return out.reshape(1, S, D)
```

```python
import functools

import jax
import jax.numpy as jnp
from jax import lax
import jax.experimental.pallas as pl
import jax.experimental.pallas.tpu as pltpu

F32 = jnp.float32
BF16 = jnp.bfloat16
U32 = jnp.uint32
LOG2E = 1.4426950408889634
NT = (((1,), (1,)), ((), ()))
LANES = 128
MASKED = -1e9 * LOG2E

NPRE = 38
NSLOT = 3
OLAG = 2
UNROLL = 2
TB = 512


def _full_order(ranges):
    first, second, rest = (
        "sKKKQQwQwVwVwVwp", "swKmmKKwQmwQwQmVmVVpw", "sKKwKmmQwOQmOQwVmOwmVVOpw")
    order, n = ["k0", "q0", "v0"], 0
    for j in range(15):
        for c in first if j == 0 else second if j == 1 else rest:
            pair = {"s": j, "p": j, "w": j, "m": j - 1, "O": n // 5}.get(c, j + 1)
            order.append(f"{c}{pair}")
            n += c == "O"
    order.append("s15")
    for i in range(14):
        order += ["m14"] * (i % 3 == 0) + [f"O{(n + i) // 5}"]
    return " ".join(order + ["p15 O13 O13 O13 O13", ranges])


FULL_ORDER = (_full_order("a14 a15 b14 b15"), _full_order("o14 o15"))
SHORT_ORDER = (
    "k0 q0 v0 s0 k1 k2 q1 v1 p0 v2 b0 s1 q2 k3 v3 q3 p1 a0 s2 k4 a1 q4 v4 p2 s3 "
    "k5 a2 q5 v5 p3 s4 k6 v6 a3 q6 s5 p4 k7 a4 q7 v7 p5 s6 k8 a5 q8 v8 p6 s7 v9 "
    "k9 a6 q9 p7 s8 q10 k10 a7 v10 p8 s9 k11 a8 q11 v11 p9 s10 k12 a9 v12 q12 "
    "p10 s11 q13 k13 a10 v13 p11 s12 k14 a11 v14 q14 p12 s13 k15 a12 v15 q15 "
    "p13 s14 b2 s15 b8 b5 b4 b3 b1 p14 b6 b9 b10 a13 a14 b7 p15 b11 b12 a15 b14 "
    "b13 b15",
    "k0 q0 v0 s0 k1 v1 k2 q1 p0 v2 s1 q2 k3 b0 v3 q3 p1 a0 s2 k4 a1 q4 v4 p2 s3 "
    "k5 a2 q5 v5 p3 s4 v6 k6 a3 q6 p4 s5 k7 a4 q7 v7 p5 s6 k8 a5 q8 v8 p6 s7 v9 "
    "k9 a6 q9 p7 s8 q10 k10 a7 v10 p8 s9 k11 q11 a8 v11 p9 s10 v12 k12 a9 q12 "
    "p10 s11 k13 q13 a10 v13 p11 s12 k14 a11 q14 v14 p12 s13 k15 a12 v15 q15 "
    "p13 s14 b2 s15 b8 b4 b1 b5 b3 p14 b6 b10 b7 b12 a13 b9 a14 p15 b11 b14 b13 "
    "b15 a15",
)
FULL_EARLY = ("2222222212222200", "2222222222222210")
SHORT_EARLY = ("0111101111110000", "0101101101110111")
B_ORDER = "f00 f01 f10 f11 m00 m01 m10 a0 m11 b0 a1 b1"


def _layernorm(x):
    m = jnp.mean(x, axis=-1, keepdims=True)
    xc = x - m
    v = jnp.mean(xc * xc, axis=-1, keepdims=True)
    return xc * lax.rsqrt(v + 1e-5)


def _pack(w):
    return pltpu.bitcast(w, U32)


def _unpack(w):
    return pltpu.bitcast(w, BF16)


def _kernel(
    x_hbm, x4_hbm, mem_hbm, wq_hbm, wk_hbm, wv_hbm, wo_hbm,
    bw_hbm, wphi_hbm, bwo_hbm,
    out_hbm,
    xb_ref, xres_ref, xna_ref, xnb_ref, memf_ref,
    stage_ref, wo_ref, w_ref,
    bw_ref, bwo_stage_ref, bwt_ref, bwo_ref,
    kv_ref, z_ref, xsel_ref, xseln_ref, pre_ref,
    mem_ref, wphi_ref, wrep_ref, row_ref,
    wsem, wosem, sem, osem,
    *, seg, dh, hb,
):
    S, D = xres_ref.shape
    M = mem_ref.shape[0]
    L = M + seg
    nseg = S // seg
    PW = 2 * dh
    npair = w_ref.shape[0]
    HL = LANES // 2
    mixed = [h * dh + r for r in range(0, dh, HL) for h in range(2)]
    fb = D // hb
    GR = 2 * fb
    HR = D // 2
    NG = HR // GR
    NTILE = 2 * HR // LANES
    spans = []
    for i in range(NTILE):
        lo = (i * LANES) // (2 * GR)
        hi = ((i + 1) * LANES - 1) // (2 * GR) + 1
        spans.append((lo * GR, hi * GR))
    offs = [0]
    for lo, hi in spans:
        offs.append(offs[-1] + hi - lo)

    XH = (UNROLL + 2) * seg

    def wcopy(j, t):
        rows = pl.ds(pl.multiple_of(j * PW, PW), PW)
        return pltpu.make_async_copy(
            (wq_hbm, wk_hbm, wv_hbm)[t].at[rows, :],
            stage_ref.at[j % NSLOT, t], wsem.at[j % NSLOT, t])

    def ocopy(j):
        rows = pl.ds(pl.multiple_of(j * PW, PW), PW)
        return pltpu.make_async_copy(
            wo_hbm.at[rows, :], wo_ref.at[rows, :], wosem.at[j % 8])

    def keep_wo(j):
        w = jnp.concatenate(
            [wo_ref[pl.ds(pl.multiple_of(j * PW + r, HL), HL), :] for r in mixed],
            axis=0)
        w_ref[j, D // 2:D // 2 + dh, 0:D] = _pack(w)

    def start_pair(j):
        for t in range(3):
            wcopy(j, t).start()

    xsel_copy = pltpu.make_async_copy(
        x4_hbm.at[0:NPRE, seg // 8 - 1], xsel_ref, sem.at[0])
    bw_copy = pltpu.make_async_copy(bw_hbm, bw_ref, sem.at[1])
    bwo_copy = pltpu.make_async_copy(bwo_hbm, bwo_stage_ref, sem.at[2])
    xh_copy = pltpu.make_async_copy(
        x_hbm.at[0:XH, :], xb_ref.at[0:XH, :], sem.at[3])
    xt_copy = pltpu.make_async_copy(
        x_hbm.at[XH:S, :], xb_ref.at[XH:S, :], sem.at[3])
    mem_copy = pltpu.make_async_copy(mem_hbm, mem_ref, sem.at[5])
    wphi_copy = pltpu.make_async_copy(wphi_hbm, wphi_ref, sem.at[4])
    wphi_copy.start()
    xsel_copy.start()
    xh_copy.start()
    start_pair(0)

    kv_ref[...] = jnp.zeros(kv_ref.shape, F32)
    z_ref[...] = jnp.zeros(z_ref.shape, F32)
    wo_ref[(npair - 1) * PW:, :] = jnp.zeros((PW, D), BF16)

    wphi_copy.wait()
    hh = lax.broadcasted_iota(jnp.int32, (hb, D), 0)
    cc = lax.broadcasted_iota(jnp.int32, (hb, D), 1)

    def spread(i, wcat):
        for d in range(4):
            sel = jnp.where(cc == hh * fb + (4 * i + d), 1.0, 0.0).astype(BF16)
            wcat += jnp.dot(wphi_ref[4 * i + d], sel, preferred_element_type=F32)
        return wcat

    wcat = lax.fori_loop(0, fb // 4, spread, jnp.zeros((fb, D), F32))
    rr = lax.broadcasted_iota(jnp.int32, (GR, fb), 0)
    ff = lax.broadcasted_iota(jnp.int32, (GR, fb), 1)
    twice = jnp.where((rr >> 1) == ff, 1.0, 0.0).astype(BF16)
    wrep_ref[...] = jnp.dot(twice, wcat.astype(BF16), preferred_element_type=F32)

    xsel_copy.wait()
    xsel = xsel_ref[...].astype(F32).reshape(NPRE * 8, D)
    xseln_ref[...] = _pack(_layernorm(xsel).astype(BF16))
    xh_copy.wait()
    xna_ref[0:seg, :] = _layernorm(xb_ref[0:seg, :].astype(F32))

    def load_pair(j, c):
        slot = j % NSLOT
        for t in range(3):
            wcopy(j, t).wait()

        @pl.when(j == 0)
        def _():
            start_pair(1)
            mem_copy.start()

        @pl.when(j + NSLOT - 1 < npair)
        def _():
            start_pair(j + NSLOT - 1)

        @pl.when(j >= OLAG)
        def _():
            ocopy(j - OLAG).start()

        @pl.when(j >= npair - OLAG)
        def _():
            ocopy(j).start()

        @pl.when(j >= OLAG + 2)
        def _():
            ocopy(j - OLAG - 2).wait()

        keep_wo(jnp.where(j >= OLAG + 2, j - OLAG - 2, npair - 1))
        for t in range(3):
            cols = slice(t * PW, (t + 1) * PW)
            w = jnp.concatenate(
                [stage_ref[slot, t, r:r + HL, :]
                 for r in (mixed if t == 2 else range(0, PW, HL))], axis=0)
            w_ref[j, 0:D // 2, cols] = _pack(w.astype(F32).T.astype(BF16))
            xn = _unpack(xseln_ref[...])
            if t == 0:
                y = lax.dot_general(
                    xn, stage_ref[slot, t], NT, preferred_element_type=F32)
            else:
                y = jnp.dot(xn, _unpack(w_ref[j, 0:D // 2, cols]),
                            preferred_element_type=F32)
            pre_ref[j, :, cols] = y
        return c

    lax.fori_loop(0, npair, load_pair, 0)
    mem_copy.wait()

    @pl.loop(npair - OLAG - 2, npair)
    def _(j):
        ocopy(j).wait()
        keep_wo(j)

    xt_copy.start()
    bw_copy.start()
    bwo_copy.start()

    def b_weights():
        bw_copy.wait()
        bwo_copy.wait()
        rr = lax.broadcasted_iota(jnp.int32, (GR, LANES), 0)
        cc = lax.broadcasted_iota(jnp.int32, (GR, LANES), 1) - (rr & 1) * fb
        for t in range(2):
            parts = [None] * (D // GR)
            for n in range(D // LANES):
                lo = (n * LANES) // GR
                hi = ((n + 1) * LANES - 1) // GR + 1
                col = cc + n * LANES
                lhs = jnp.concatenate([
                    jnp.where((col >= g * GR) & (col < g * GR + fb),
                              wrep_ref[:, n * LANES:(n + 1) * LANES], 0.0)
                    for g in range(lo, hi)
                ], axis=0)
                y = lax.dot_general(
                    lhs, bw_ref[:, t * D + n * LANES:t * D + (n + 1) * LANES], NT,
                    preferred_element_type=F32)
                for g in range(lo, hi):
                    piece = y[(g - lo) * GR:(g - lo + 1) * GR]
                    parts[g] = piece if parts[g] is None else parts[g] + piece
            w = jnp.concatenate(parts, axis=0) * LOG2E
            bwt_ref[t] = _pack(w.astype(BF16))
        bwt_ref[2] = _pack(bw_ref[:, 2 * D:3 * D].T)
        bwo_ref[...] = _pack(bwo_stage_ref[...])

    def a_step(short, s, mem, u):
        rows = pl.ds(pl.multiple_of(s * seg, seg), seg)
        sub = lax.broadcasted_iota(jnp.int32, (8, LANES), 0)
        lane = lax.broadcasted_iota(jnp.int32, (8, LANES), 1)
        is_a = lane < L
        col = jnp.where(is_a, lane, lane - L)
        low = lane < HL
        lows = lax.broadcasted_iota(jnp.int32, (L, LANES), 1) < HL
        scale = jnp.where(
            lax.broadcasted_iota(jnp.int32, (L, PW), 1) + s >= 0,
            dh ** -0.5 * LOG2E, 0.0)
        never = lane + s < 0
        early = [int(n) for n in (SHORT_EARLY if short else FULL_EARLY)[u]]
        due = []

        def pin(lhs):
            if not due:
                return lhs
            top = lhs[:8, :LANES]
            while due:
                top = jnp.where(never, due.pop(), top)
            top = jnp.concatenate([top, lhs[:8, LANES:]], axis=1)
            return jnp.concatenate([top, lhs[8:]], axis=0)

        def part(j, t, lo, hi, c0=0, c1=PW):
            n = seg - 8 if short else seg
            x = xna_ref[pl.ds(pl.multiple_of(s * seg, seg), n), lo:hi]
            h = pin(jnp.concatenate([mem[:, lo:hi], x], axis=0))
            w = _unpack(w_ref[j, lo // 2:hi // 2, t * PW + c0:t * PW + c1])
            return jnp.dot(h.astype(BF16) if short else h, w,
                           preferred_element_type=F32)

        def proj(j, t, y):
            if short:
                tail = pl.ds(pl.multiple_of(s * 8, 8), 8)
                y = jnp.concatenate(
                    [y, pre_ref[j, tail, t * PW:(t + 1) * PW]], axis=0)
            if t == 0:
                return y * scale
            for b in range(early[j]):
                n = M + 8 * b + 8
                row_ref[j, 2 * b + t - 1, 0:n, :] = y[:n]
            return y

        def spread_row(j, n, r, c):
            return jnp.broadcast_to(
                row_ref[j, n, r:r + 1, c * LANES:(c + 1) * LANES], (8, LANES))

        def stack(top, bot):
            pad = jnp.zeros((LANES - 2 * L, PW), F32)
            return jnp.concatenate([top, bot, pad], axis=0).astype(BF16)

        def keys(k):
            zero = jnp.zeros((L, LANES), F32)
            mid = k[:, LANES:2 * LANES]
            return stack(
                jnp.concatenate(
                    [k[:, :LANES], jnp.where(lows, mid, 0.0), zero], axis=1),
                jnp.concatenate(
                    [zero, jnp.where(lows, 0.0, mid), k[:, 2 * LANES:]], axis=1))

        def values(v):
            first = jnp.concatenate([lows] * 3, axis=1)
            return stack(jnp.where(first, v, 0.0), jnp.where(first, 0.0, v))

        def softmax(sc, row):
            inside = col < L
            vis = inside if row < M else col <= sub + row
            sc = jnp.where(vis, sc, jnp.where(inside, MASKED, -jnp.inf))
            ma = jnp.max(jnp.where(is_a, sc, -jnp.inf), axis=1, keepdims=True)
            mb = jnp.max(jnp.where(is_a, -jnp.inf, sc), axis=1, keepdims=True)
            e = jnp.exp2(sc - jnp.where(is_a, ma, mb))
            la = jnp.sum(jnp.where(is_a, e, 0.0), axis=1, keepdims=True)
            lb = jnp.sum(jnp.where(is_a, 0.0, e), axis=1, keepdims=True)
            return e * (1.0 / jnp.where(is_a, la, lb))

        def vpu_scores(j, q, out):
            for b in range(early[j]):
                row = M + 8 * b
                mid = q[row:row + 8, LANES:2 * LANES]
                qa, qb = jnp.where(low, mid, 0.0), jnp.where(low, 0.0, mid)
                scores, top = [], None
                for r in range(row + 8):
                    k0, k1, k2 = (spread_row(j, 2 * b, r, c) for c in range(3))
                    x = jnp.where(
                        low,
                        jnp.sum(q[row:row + 8, :LANES] * k0 + qa * k1,
                                axis=1, keepdims=True),
                        jnp.sum(q[row:row + 8, 2 * LANES:] * k2 + qb * k1,
                                axis=1, keepdims=True))
                    if r > row:
                        x = jnp.where(sub >= r - row, x, MASKED)
                    top = x if top is None else jnp.maximum(top, x)
                    scores.append(x)
                    if r == row + 7:
                        out.append((scores, top))
                    if r % 8 == 7:
                        yield [top]

        def vpu_mix(j, scores, out):
            for b in range(early[j]):
                acc = None
                for r, x in enumerate(scores[b][0]):
                    e = jnp.exp2(x - scores[b][1])
                    t = [e * spread_row(j, 2 * b + 1, r, c) for c in range(3)] + [e]
                    acc = t if acc is None else [x + y for x, y in zip(acc, t)]
                    if r == M + 8 * b + 7:
                        inv = 1.0 / acc[3]
                        out.append(
                            jnp.concatenate([x * inv for x in acc[:3]], axis=1))
                    if r % 8 == 7:
                        yield acc[:3]

        def probs(j, q, k):
            far = M + 8 * early[j]
            sc = lax.dot_general(
                jnp.concatenate([q[:M], q[far:]], axis=0), keys(k), NT,
                preferred_element_type=F32)
            return jnp.concatenate([
                softmax(sc[8 * n:8 * n + 8], row)
                for n, row in enumerate([0] + list(range(far, L, 8)))
            ], axis=0)

        prv = pl.ds(pl.multiple_of(jnp.maximum(s - 1, 0) * seg, seg), seg)
        nxt = pl.ds(pl.multiple_of(jnp.minimum(s + 1, nseg - 1) * seg, seg), seg)
        if short:
            far = jnp.where(s < UNROLL, s, nseg - 1 + UNROLL - s)
            far = jnp.where(far < NPRE, s, far)
            far = pl.ds(pl.multiple_of(far * seg, seg), seg)
            xres_ref[far, :] = xb_ref[far, :].astype(F32)
        xnb_ref[prv, :] = _layernorm(xres_ref[prv, :]).astype(BF16)
        xin_ref = xb_ref if short else xres_ref
        xn_next = _layernorm(xin_ref[nxt, :].astype(F32))

        qkv, p, o, tiles = ({}, {}, {}), {}, {}, {}
        scored = [[] for _ in range(npair)]
        mixed_rows = [[] for _ in range(npair)]
        work = {}
        acc = [None] * (D // LANES)
        heads = [part(0, t, 0, PW) for t in (1, 0)] if u > 0 else []

        def piece(op, j):
            if (op, j) not in work:
                work[op, j] = (
                    vpu_scores(j, qkv[0][j], scored[j]) if op == "w"
                    else vpu_mix(j, scored[j], mixed_rows[j]))
            return next(work[op, j], None)

        order = (SHORT_ORDER if short else FULL_ORDER)[u]
        for op, j in ((t[0], int(t[1:])) for t in order.split()):
            if op in "qkv":
                t = "qkv".index(op)
                if heads:
                    y = part(j, t, PW, D) + heads.pop(0)
                else:
                    y = part(j, t, 0, D)
                qkv[t][j] = proj(j, t, y)
            elif op in "QKV":
                t = "QKV".index(op)
                done = tiles.setdefault((op, j), [])
                c = len(done) * LANES
                done.append(part(j, t, 0, D, c, c + LANES))
                if len(done) == 3:
                    qkv[t][j] = proj(j, t, jnp.concatenate(done, axis=1))
            elif op in "wm":
                due.extend(piece(op, j) or [])
            elif op == "s":
                p[j] = probs(j, qkv[0][j], qkv[1][j])
            elif op == "p":
                o[j] = jnp.dot(
                    p[j], values(qkv[2][j]), preferred_element_type=F32)
                if j == npair - 1:
                    xna_ref[nxt, :] = xn_next
            else:
                for rest in "wm":
                    while piece(rest, j):
                        pass
                if op == "O":
                    lo = tiles.get((op, j), 0)
                    hi = tiles[op, j] = lo + 1
                else:
                    lo, hi = {"a": (0, 3), "b": (3, 5), "o": (0, 5)}[op]
                lhs = jnp.concatenate(
                    [o[j][:M]] + mixed_rows[j] + [o[j][M:]], axis=0)
                w = _unpack(w_ref[j, D // 2:D // 2 + dh, lo * LANES:hi * LANES])
                y = jnp.dot(pin(lhs), w, preferred_element_type=F32)
                for n in range(lo, hi):
                    t = y[:, (n - lo) * LANES:(n - lo + 1) * LANES]
                    acc[n] = t if acc[n] is None else acc[n] + t
        acc = jnp.concatenate(acc, axis=1)
        xres_ref[rows, :] = xin_ref[rows, :].astype(F32) + acc[M:]
        return acc[:M]

    def a_steps(short, i, c):
        if short:
            pl.when(i == 1)(xt_copy.wait)
        mem = memf_ref[...]
        for u in range(UNROLL):
            mem = a_step(short, i * UNROLL + u, mem, u)
        memf_ref[...] = mem
        return c

    def layer_a(n):
        memf_ref[...] = mem_ref[...].astype(F32)
        nshort = jnp.where(n == 0, NPRE // UNROLL, 0)
        lax.fori_loop(0, nshort, functools.partial(a_steps, True), 0)
        lax.fori_loop(nshort, nseg // UNROLL, functools.partial(a_steps, False), 0)

    def b_proj(t, half, rows):
        w = _unpack(bwt_ref[t, half * (HR // 2):(half + 1) * (HR // 2), :])
        return lax.dot_general(
            w, xnb_ref[rows, :], NT, preferred_element_type=F32)

    def fold(vals, op):
        r = functools.reduce(op, vals)
        r = op(r, pltpu.roll(r, 4, 0))
        return op(r, pltpu.roll(r, 2, 0))

    def exps(a, g):
        slabs = [a[g * GR + 8 * i:g * GR + 8 * i + 8] for i in range(GR // 8)]
        mx = fold(slabs, jnp.maximum)
        mn = fold(slabs, jnp.minimum)
        ep = [jnp.exp2(u - mx) for u in slabs]
        en = [jnp.exp2(mn - u) for u in slabs]
        return ep, en, fold(ep, jnp.add), fold(en, jnp.add)

    def b_pass1(i, c):
        rows = pl.ds(pl.multiple_of(i * TB, TB), TB)

        def features(half):
            a = b_proj(1, half, rows)
            phi = []
            for g in range(NG):
                ep, en, sp, sn = exps(a, g)
                inv = 1.0 / (sp * sn)
                ip, im = sn * inv, sp * inv
                phi += [e * ip for e in ep] + [e * im for e in en]
            phi = jnp.concatenate(phi, axis=0)
            zsum = phi[:, :LANES]
            for n in range(1, TB // LANES):
                zsum = zsum + phi[:, n * LANES:(n + 1) * LANES]
            return phi.astype(BF16), zsum

        def outer(half, vt, phi):
            for n, (lo, hi) in enumerate(spans):
                y = lax.dot_general(
                    vt[lo:hi], phi[n * LANES:(n + 1) * LANES], NT,
                    preferred_element_type=F32)
                r = lax.broadcasted_iota(jnp.int32, (hi - lo, LANES), 0) + lo
                f = lax.broadcasted_iota(jnp.int32, (1, LANES), 1) + n * LANES
                first = (f & 1) * fb
                for g in range(lo // GR, hi // GR):
                    first = jnp.where(f >= g * 2 * GR, g * GR + (f & 1) * fb, first)
                keep = (r >= first) & (r < first + fb)
                blk = slice(offs[n], offs[n + 1])
                old = jnp.where(i > 0, kv_ref[half, blk, :], 0.0)
                kv_ref[half, blk, :] = jnp.where(keep, old + y, 0.0)

        phi0, z0 = features(0)
        phi1, z1 = features(1)
        for half, z in enumerate((z0, z1)):
            z_ref[half] = jnp.where(i > 0, z_ref[half], 0.0) + z
        vt0 = b_proj(2, 0, rows)
        vt1 = b_proj(2, 1, rows)
        outer(0, vt0, phi0)
        outer(1, vt1, phi1)
        xnb_ref[S - seg:S, :] = _layernorm(xres_ref[S - seg:S, :]).astype(BF16)
        return c

    def b_pass2(i, c):
        tu = TB // 2

        def unit_rows(u):
            return pl.ds(pl.multiple_of(i * TB + u * tu, tu), tu)

        def features(u, half):
            a = b_proj(0, half, unit_rows(u))
            phi = []
            for g in range(NG):
                ep, en, sp, sn = exps(a, g)

                def zdot(es, base):
                    terms = []
                    for n, e in enumerate(es):
                        z = z_ref[half, base + 8 * n:base + 8 * n + 8, :]
                        terms.append(e * jnp.concatenate([z] * (tu // LANES), axis=1))
                    return functools.reduce(jnp.add, terms)

                den = zdot(ep, 2 * GR * g) * sn + zdot(en, 2 * GR * g + GR) * sp
                inv = 1.0 / (fold([den], jnp.add) + 1e-6 * (sp * sn))
                ip, im = sn * inv, sp * inv
                phi += [e * ip for e in ep] + [e * im for e in en]
            return jnp.concatenate(phi, axis=0).astype(BF16)

        def mix(half, phi):
            parts = [None] * NG
            for n, (lo, hi) in enumerate(spans):
                y = jnp.dot(
                    kv_ref[half, offs[n]:offs[n + 1], :],
                    phi[n * LANES:(n + 1) * LANES], preferred_element_type=F32)
                for g in range(lo // GR, hi // GR):
                    piece = y[g * GR - lo:(g + 1) * GR - lo]
                    parts[g] = piece if parts[g] is None else parts[g] + piece
            return jnp.concatenate(parts, axis=0)

        def finish(u, cols, o):
            rows = unit_rows(u)
            y = jnp.dot(o, _unpack(bwo_ref[:, cols]), preferred_element_type=F32)
            y = xres_ref[rows, cols] + y
            xres_ref[rows, cols] = y
            xb_ref[rows, cols] = y.astype(BF16)
            return y[:seg]

        phi, ot, o = {}, {}, {}
        for op in B_ORDER.split():
            u = int(op[1])
            if op[0] == "f":
                phi[op[1:]] = features(u, int(op[2]))
            elif op[0] == "m":
                ot[op[1:]] = mix(int(op[2]), phi.pop(op[1:]))
                if op[2] == "1":
                    o[u] = jnp.concatenate(
                        [ot.pop(op[1] + "0"), ot.pop(op[1:])], axis=0).T
            else:
                cols = slice(0, PW) if op[0] == "a" else slice(PW, D)
                ot[op] = finish(u, cols, o[u])
                pltpu.make_async_copy(
                    xb_ref.at[unit_rows(u), cols], out_hbm.at[unit_rows(u), cols],
                    osem).start()
        xna_ref[pl.ds(pl.multiple_of(i * TB, TB), seg), :] = _layernorm(
            jnp.concatenate([ot["a0"], ot["b0"]], axis=1))
        return c

    nblk = S // TB
    out_copy = pltpu.make_async_copy(xb_ref, out_hbm, osem)

    def layer(n, c):
        layer_a(n)
        pl.when(n == 0)(b_weights)
        lax.fori_loop(0, nblk, b_pass1, 0)
        z_ref[...] = jnp.broadcast_to(
            jnp.sum(z_ref[...], axis=2, keepdims=True), z_ref.shape)
        pl.when(n == 1)(out_copy.wait)
        lax.fori_loop(0, nblk, b_pass2, 0)
        return c

    lax.fori_loop(0, 2, layer, 0)
    out_copy.wait()


@functools.partial(jax.jit, static_argnames=("A_seg_len",))
def pallas_interleave_layers__memory_aug_recurrent_mem_tr__linear_kernel_hedgehog__prompt_kernel(
    A_x: jax.Array,
    A_mem0: jax.Array,
    A_Wq: jax.Array,
    A_Wk: jax.Array,
    A_Wv: jax.Array,
    A_Wo: jax.Array,
    A_seg_len: int,
    B_x: jax.Array,
    B_wqkv: jax.Array,
    B_w_phi: jax.Array,
    B_wo: jax.Array,
):
    del B_x
    _, S, D = A_x.shape
    M = A_mem0.shape[1]
    _, H, dh = A_Wq.shape
    hb = B_w_phi.shape[0]
    seg = int(A_seg_len)
    npair, PW = H // 2, 2 * dh
    assert (A_x.shape[0], M, seg, H, dh, D, hb) == (1, 8, 32, 32, 192, 640, 32)
    assert S % TB == 0 and NPRE * seg <= S <= (2 * NPRE - UNROLL) * seg

    def rows_first(w):
        return jnp.transpose(w, (1, 2, 0)).reshape(H * dh, D)

    hbm = pl.BlockSpec(memory_space=pl.ANY)
    out = pl.pallas_call(
        functools.partial(_kernel, seg=seg, dh=dh, hb=hb),
        out_shape=jax.ShapeDtypeStruct((S, D), BF16),
        in_specs=[hbm] * 10,
        out_specs=hbm,
        scratch_shapes=[
            pltpu.VMEM((S, D), BF16),
            pltpu.VMEM((S, D), F32),
            pltpu.VMEM((S, D), F32),
            pltpu.VMEM((S, D), BF16),
            pltpu.VMEM((M, D), F32),
            pltpu.VMEM((NSLOT, 3, PW, D), BF16),
            pltpu.VMEM((H * dh, D), BF16),
            pltpu.VMEM((npair, D // 2 + dh, 3 * PW), U32),
            pltpu.VMEM((D, 3 * D), BF16),
            pltpu.VMEM((D, D), BF16),
            pltpu.VMEM((3, D // 2, D), U32),
            pltpu.VMEM((D // 2, D), U32),
            pltpu.VMEM((2, 480, LANES), F32),
            pltpu.VMEM((2, D, LANES), F32),
            pltpu.VMEM((NPRE, 8, D), BF16),
            pltpu.VMEM((NPRE * 4, D), U32),
            pltpu.VMEM((npair, NPRE * 8, 3 * PW), F32),
            pltpu.VMEM((M, D), BF16),
            pltpu.VMEM((D // hb, D // hb, hb), BF16),
            pltpu.VMEM((2 * D // hb, D), F32),
            pltpu.VMEM((npair, 4, M + 16, PW), F32),
            pltpu.SemaphoreType.DMA((NSLOT, 3)),
            pltpu.SemaphoreType.DMA((8,)),
            pltpu.SemaphoreType.DMA((6,)),
            pltpu.SemaphoreType.DMA,
        ],
        compiler_params=pltpu.CompilerParams(
            vmem_limit_bytes=112 * 1024 * 1024, disable_bounds_checks=True),
    )(
        A_x.reshape(S, D),
        A_x.reshape(S // seg, seg // 8, 8, D),
        A_mem0.reshape(M, D),
        rows_first(A_Wq),
        rows_first(A_Wk),
        rows_first(A_Wv),
        A_Wo.reshape(H * dh, D),
        B_wqkv,
        jnp.transpose(B_w_phi, (1, 2, 0)),
        B_wo,
    )
    return out.reshape(1, S, D)
```
